```python
import jax
import jax.numpy as jnp

def _softmax(x, axis=-1):
    return jax.nn.softmax(x, axis=axis)

def _gelu(x):
    return jax.nn.gelu(x, approximate=True)

def _silu(x):
    return jax.nn.silu(x)

def _sigmoid(x):
    return jax.nn.sigmoid(x)

def _layernorm(x, axis=-1, eps=1e-05):
    m = jnp.mean(x, axis=axis, keepdims=True)
    v = jnp.var(x, axis=axis, keepdims=True)
    return (x - m) / jnp.sqrt(v + eps)

def _scatter_add(tgt, idx, src, axis=0):
    return tgt.at[idx].add(src)

def _segment_sum(src, seg, n):
    return jax.ops.segment_sum(src, seg, n)

class _Rng:

    def __init__(self, key):
        self._k = key

    def _next(self):
        self._k, sub = jax.random.split(self._k)
        return sub

    def normal(self, shape):
        return jax.random.normal(self._next(), shape, dtype=jnp.bfloat16)

    def randint(self, lo, hi, shape):
        return jax.random.randint(self._next(), shape, lo, hi, dtype=jnp.int32)

    def uniform(self, shape, lo=0.0, hi=1.0):
        return jax.random.uniform(self._next(), shape, jnp.bfloat16, lo, hi)

    def permutation(self, n):
        return jax.random.permutation(self._next(), n)
kernel_name = 'standalone__conformer_family_conformer__speech'

def setup_inputs():
    _rng = _Rng(jax.random.key(int.from_bytes(__import__("os").urandom(4), "little")))
    _w = lambda a: (lambda t: t.astype(jnp.bfloat16) if jnp.issubdtype(t.dtype, jnp.floating) else t)(jnp.asarray(a))
    B, T, D, K = (2, 4000, 512, 15)
    F = 4 * D
    s = D ** (-0.5)
    sf = F ** (-0.5)
    return {'x': _w((lambda *s: _rng.normal(s) * 0.05)(B, T, D)), 'w_ff1_a': _w((lambda *s: _rng.normal(s) * 0.05)(D, F) * s), 'w_ff1_b': _w((lambda *s: _rng.normal(s) * 0.05)(F, D) * sf), 'w_q': _w((lambda *s: _rng.normal(s) * 0.05)(D, D) * s), 'w_k': _w((lambda *s: _rng.normal(s) * 0.05)(D, D) * s), 'w_v': _w((lambda *s: _rng.normal(s) * 0.05)(D, D) * s), 'w_o': _w((lambda *s: _rng.normal(s) * 0.05)(D, D) * s), 'w_pw1': _w((lambda *s: _rng.normal(s) * 0.05)(D, 2 * D) * s), 'dw': _w((lambda *s: _rng.normal(s) * 0.05)(K, D) * K ** (-0.5)), 'w_pw2': _w((lambda *s: _rng.normal(s) * 0.05)(D, D) * s), 'w_ff2_a': _w((lambda *s: _rng.normal(s) * 0.05)(D, F) * s), 'w_ff2_b': _w((lambda *s: _rng.normal(s) * 0.05)(F, D) * sf)}

def reference(x, w_ff1_a, w_ff1_b, w_q, w_k, w_v, w_o, w_pw1, dw, w_pw2, w_ff2_a, w_ff2_b):
    B, T, D = x.shape
    K = dw.shape[0]
    scale = D ** (-0.5)
    h = _layernorm(x, axis=-1)
    h = _silu(h @ w_ff1_a) @ w_ff1_b
    x1 = x + 0.5 * h
    h = _layernorm(x1, axis=-1)
    q = h @ w_q
    k = h @ w_k
    v = h @ w_v
    scores = jnp.einsum('btd,bsd->bts', q, k) * scale
    p = _softmax(scores, axis=-1)
    attn = jnp.einsum('bts,bsd->btd', p, v) @ w_o
    x2 = x1 + attn
    h = _layernorm(x2, axis=-1)
    h = h @ w_pw1
    a = h[..., :D].copy()
    b = h[..., D:].copy()
    h = a * _sigmoid(b)
    pad = K // 2
    hp = jnp.pad(h, ((0, 0), (pad, K - 1 - pad), (0, 0)))
    dc = jnp.zeros_like(h)
    for i in range(K):
        dc = dc + hp[:, i:i + T, :] * dw[i][None, None, :]
    flat = dc.reshape(-1, D)
    mu = flat.mean(0)
    var = ((flat - mu) ** 2).mean(0)
    dc = (dc - mu[None, None, :]) / jnp.sqrt(var[None, None, :] + 1e-05)
    h = _silu(dc) @ w_pw2
    x3 = x2 + h
    h = _layernorm(x3, axis=-1)
    h = _silu(h @ w_ff2_a) @ w_ff2_b
    x4 = x3 + 0.5 * h
    return _layernorm(x4, axis=-1)
```

```python
import functools
import jax
import jax.numpy as jnp
import numpy as np
from jax import lax
from jax.experimental import pallas as pl
from jax.experimental.pallas import tpu as pltpu

B, T, D, F, KW = 2, 4000, 512, 2048, 15
TP = 4096
TM = 400
NT = T // TM
NTILE = B * NT
EPS = 1e-5
LOG2E = 1.4426950408889634
BF = jnp.bfloat16
F32 = jnp.float32
HALO = 8


def _ln(x):
    m = jnp.mean(x, axis=-1, keepdims=True)
    xc = x - m
    v = jnp.mean(xc * xc, axis=-1, keepdims=True)
    return xc * lax.rsqrt(v + EPS)


def _dot(a, b):
    return jnp.dot(a, b, preferred_element_type=F32)


def _dot_nt(a, b):
    return lax.dot_general(a, b, (((1,), (1,)), ((), ())), preferred_element_type=F32)


def _ffn(h_bf, wa_ref, wb_ref):
    u = _dot(h_bf, wa_ref[...])
    u = jax.nn.silu(u).astype(BF)
    return _dot(u, wb_ref[...])


def kernel(x_ref, w1a, w1b, wq, wk, wv, wo, wp1, dw_ref, wp2, w2a, w2b, o_ref,
           xs, hs, gs, dcs, mq, nv, st):
    s = pl.program_id(0)

    @pl.when(s == 0)
    def _init():
        m = _dot_nt(wq[...], wk[...]) * (D ** -0.5 * LOG2E)
        mq[...] = m.astype(BF)
        nv[...] = _dot(wv[...], wo[...]).astype(BF)
        for b in range(B):
            hs[b, T:TP, :] = jnp.zeros((TP - T, D), BF)
            gs[b, 0:HALO, :] = jnp.zeros((HALO, D), F32)
            gs[b, HALO + T:HALO + T + HALO, :] = jnp.zeros((HALO, D), F32)
        st[...] = jnp.zeros(st.shape, F32)

    @pl.when(s < NTILE)
    def _phase_a():
        b = s // NT
        t0 = pl.multiple_of((s % NT) * TM, 16)
        x = x_ref[...].astype(F32)
        h = _ln(x).astype(BF)
        x1 = x + 0.5 * _ffn(h, w1a, w1b)
        xs[b, pl.ds(t0, TM), :] = x1
        hs[b, pl.ds(t0, TM), :] = _ln(x1).astype(BF)

    @pl.when((s >= NTILE) & (s < 2 * NTILE))
    def _phase_b():
        i = s - NTILE
        b = i // NT
        t0 = pl.multiple_of((i % NT) * TM, 16)
        hq = hs[b, pl.ds(t0, TM), :]
        q = _dot(hq, mq[...]).astype(BF)
        hb = hs[b]
        sc = _dot_nt(q, hb)
        col = lax.broadcasted_iota(jnp.int32, (TM, TP), 1)
        sc = jnp.where(col < T, sc, -jnp.inf)
        mx = jnp.max(sc, axis=-1, keepdims=True)
        p = jnp.exp2(sc - mx)
        l = jnp.sum(p, axis=-1, keepdims=True)
        o = _dot(p.astype(BF), hb) / l
        attn = _dot(o.astype(BF), nv[...])
        x2 = xs[b, pl.ds(t0, TM), :] + attn
        xs[b, pl.ds(t0, TM), :] = x2
        y = _dot(_ln(x2).astype(BF), wp1[...])
        g = y[:, :D] * jax.nn.sigmoid(y[:, D:])
        gs[b, pl.ds(pl.multiple_of(t0 + HALO, 8), TM), :] = g

    @pl.when(s == 2 * NTILE)
    def _conv():
        def body(i, carry):
            b = i // NT
            t0 = pl.multiple_of((i % NT) * TM, 8)
            acc = jnp.zeros((TM, D), F32)
            blk = gs[b, pl.ds(t0, TM + 2 * HALO), :]
            for k in range(KW):
                acc = acc + blk[k + 1:k + 1 + TM, :] * dw_ref[k:k + 1, :].astype(F32)
            dcs[b, pl.ds(t0, TM), :] = acc
            return carry + jnp.sum(acc, axis=0, keepdims=True)
        tot = lax.fori_loop(0, NTILE, body, jnp.zeros((1, D), F32))
        mu = tot * (1.0 / (B * T))

        def body2(i, carry):
            b = i // NT
            t0 = pl.multiple_of((i % NT) * TM, 8)
            d = dcs[b, pl.ds(t0, TM), :] - mu
            return carry + jnp.sum(d * d, axis=0, keepdims=True)
        var = lax.fori_loop(0, NTILE, body2, jnp.zeros((1, D), F32)) * (1.0 / (B * T))
        st[0:1, :] = mu
        st[1:2, :] = lax.rsqrt(var + EPS)

    @pl.when(s >= 2 * NTILE)
    def _phase_c():
        i = s - 2 * NTILE
        b = i // NT
        t0 = pl.multiple_of((i % NT) * TM, 16)
        dc = (dcs[b, pl.ds(t0, TM), :] - st[0:1, :]) * st[1:2, :]
        x3 = xs[b, pl.ds(t0, TM), :] + _dot(jax.nn.silu(dc).astype(BF), wp2[...])
        x4 = x3 + 0.5 * _ffn(_ln(x3).astype(BF), w2a, w2b)
        o_ref[...] = _ln(x4).astype(o_ref.dtype)


@jax.jit
def pallas_standalone__conformer_family_conformer__speech_kernel(x, w_ff1_a, w_ff1_b, w_q, w_k, w_v, w_o, w_pw1, dw, w_pw2, w_ff2_a, w_ff2_b):
    w1a, w1b, wq, wk, wv, wo, wp1, wp2, w2a, w2b = w_ff1_a, w_ff1_b, w_q, w_k, w_v, w_o, w_pw1, w_pw2, w_ff2_a, w_ff2_b
    xf = x.reshape(B * T, D)
    full = lambda a: pl.BlockSpec(a.shape, lambda s: (0,) * a.ndim, pipeline_mode=pl.Buffered(1))
    ws = (w1a, w1b, wq, wk, wv, wo, wp1, dw, wp2, w2a, w2b)
    out = pl.pallas_call(
        kernel,
        grid=(3 * NTILE,),
        in_specs=[pl.BlockSpec((TM, D), lambda s: (jnp.minimum(s, NTILE - 1), 0))] + [full(w) for w in ws],
        out_specs=pl.BlockSpec((TM, D), lambda s: (jnp.maximum(s - 2 * NTILE, 0), 0)),
        out_shape=jax.ShapeDtypeStruct((B * T, D), x.dtype),
        scratch_shapes=[
            pltpu.VMEM((B, T, D), F32),
            pltpu.VMEM((B, TP, D), BF),
            pltpu.VMEM((B, T + 2 * HALO, D), F32),
            pltpu.VMEM((B, T, D), F32),
            pltpu.VMEM((D, D), BF),
            pltpu.VMEM((D, D), BF),
            pltpu.VMEM((8, D), F32),
        ],
        compiler_params=pltpu.CompilerParams(
            dimension_semantics=("arbitrary",), vmem_limit_bytes=120 * 1024 * 1024),
    )(xf, *ws)
    return out.reshape(B, T, D)
```

```python
import functools
import jax
import jax.numpy as jnp
import numpy as np
from jax import lax
from jax.experimental import pallas as pl
from jax.experimental.pallas import tpu as pltpu

B, T, D, F, KW = 2, 4000, 512, 2048, 15
TP = 4096
TM = 400
NT = T // TM
NTILE = B * NT
KC = 512
NKC = TP // KC
EPS = 1e-5
LOG2E = 1.4426950408889634
BF = jnp.bfloat16
F32 = jnp.float32
HALO = 8


def _ln(x):
    m = jnp.mean(x, axis=-1, keepdims=True)
    xc = x - m
    v = jnp.mean(xc * xc, axis=-1, keepdims=True)
    return xc * lax.rsqrt(v + EPS)


def _dot(a, b):
    return jnp.dot(a, b, preferred_element_type=F32)


def _dot_nt(a, b):
    return lax.dot_general(a, b, (((1,), (1,)), ((), ())), preferred_element_type=F32)


def _sigmoid(x):
    return 0.5 * jnp.tanh(0.5 * x) + 0.5


def _silu(x):
    hx = 0.5 * x
    return hx * jnp.tanh(hx) + hx


def _mult(v, n):
    return v if isinstance(v, int) else pl.multiple_of(v, n)


def _rows(i):
    return pl.ds(_mult(i * TM, 16), TM)


def _krow(i):
    return _mult((i // NT) * TP + (i % NT) * TM, 16)


def _grow(i):
    return _mult((i // NT) * (T + 2 * HALO) + (i % NT) * TM, 8)


def kernel(x_hbm, w1a_h, w1b_h, wq_h, wk_h, wv_h, wo_h, wp1_h, dw_h, wp2_h, w2a_h, w2b_h, o_hbm,
           w1a, w1b, wq, wk, wv, wo, wp1, dw_ref, wp2, w2a, w2b,
           xs, hs, qs, vs, gs, dcs, us, ss, accs, ls, zs, mqv, st,
           wsem, xsem, osem):
    def wcopy(k):
        srcs = (w1a_h, w1b_h, wq_h, wk_h, wv_h, wo_h, wp1_h, dw_h, wp2_h, w2a_h, w2b_h)
        dsts = (w1a, w1b, wq, wk, wv, wo, wp1, dw_ref, wp2, w2a, w2b)
        return pltpu.make_async_copy(srcs[k], dsts[k], wsem.at[k])

    def xcopy(i):
        return pltpu.make_async_copy(x_hbm.at[_rows(i), :], qs.at[_rows(i), :], xsem.at[i])

    def ocopy(i):
        return pltpu.make_async_copy(qs.at[_rows(i), :], o_hbm.at[_rows(i), :], osem.at[0])

    def ffa(h_bf, wa):
        for c in range(F // 512):
            u = _dot(h_bf, wa[:, c * 512:(c + 1) * 512])
            us[:, c * 512:(c + 1) * 512] = _silu(u).astype(BF)

    def a_step(i, do_prev, do_cur):
        if do_prev:
            y = _dot(us[...], w1b[...])
        if do_cur:
            x = qs[_rows(i), :].astype(F32)
            xs[_rows(i), :] = x
            h0 = _ln(x).astype(BF)
        if do_prev:
            x1 = xs[_rows(i - 1), :] + 0.5 * y
            xs[_rows(i - 1), :] = x1
            h1 = _ln(x1).astype(BF)
            hs[pl.ds(_krow(i - 1), TM), :] = h1
        if do_cur:
            ffa(h0, w1a)
        if do_prev:
            qv = _dot(h1, mqv[...])
            qs[_rows(i - 1), :] = qv[:, :D].astype(BF)
            vs[pl.ds(_krow(i - 1), TM), :] = qv[:, D:].astype(BF)

    def conv(i):
        g0 = _grow(i)
        r0 = _mult(i * TM, 8)
        sub = lax.broadcasted_iota(jnp.int32, (8, 128), 0)
        NV = TM // 8
        for cb in range(D // 128):
            cols = slice(cb * 128, (cb + 1) * 128)
            w = [jnp.broadcast_to(dw_ref[k:k + 1, cols].astype(F32), (8, 128)) for k in range(KW)]
            ld = lambda j: gs[pl.ds(g0 + 8 * j, 8), cols]
            cur = ld(0)
            rcur = [cur] + [pltpu.roll(cur, 8 - r, 0) for r in range(1, 8)]
            part = None
            tot = None
            for j in range(NV + 1):
                nxt = ld(j + 1)
                rnxt = [nxt] + [pltpu.roll(nxt, 8 - r, 0) for r in range(1, 8)]
                g = [cur] + [jnp.where(sub < 8 - r, rcur[r], rnxt[r]) for r in range(1, 8)]
                if j >= 1:
                    t = [g[r] * w[7 + r] for r in range(8)]
                    o = part + (((t[0] + t[1]) + (t[2] + t[3])) + ((t[4] + t[5]) + (t[6] + t[7])))
                    dcs[pl.ds(r0 + 8 * (j - 1), 8), cols] = o
                    tot = o if tot is None else tot + o
                if j < NV:
                    t = [g[r] * w[r - 1] for r in range(1, 8)]
                    part = ((t[0] + t[1]) + (t[2] + t[3])) + ((t[4] + t[5]) + t[6])
                cur, rcur = nxt, rnxt
            tm = jnp.sum(tot, axis=0, keepdims=True) * (1.0 / TM)
            tmb = jnp.broadcast_to(tm, (8, 128))
            m2 = None
            for j in range(NV):
                d = dcs[pl.ds(r0 + 8 * j, 8), cols] - tmb
                m2 = d * d if m2 is None else m2 + d * d
            m2 = jnp.sum(m2, axis=0, keepdims=True)
            n = jnp.zeros((1, 128), F32) + jnp.asarray(i, F32)
            mean_old = st[0:1, cols]
            delta = tm - mean_old
            st[0:1, cols] = mean_old + delta / (n + 1.0)
            st[1:2, cols] = st[1:2, cols] + m2 + delta * delta * (n * TM / (n + 1.0))

    def b_step(i, do_prev, do_cur, conv_tiles, a_tail=False):
        if a_tail:
            y = _dot(us[...], w1b[...])
        if do_cur:
            kb = _mult((i // NT) * TP, TP)
            q = qs[_rows(i), :]
            m128 = None
            for c in range(NKC):
                sc = _dot_nt(q, hs[pl.ds(kb + c * KC, KC), :])
                parts = [sc[:, j * 128:(j + 1) * 128] for j in range(KC // 128)]
                lo = c * KC
                for j in range(KC // 128):
                    if lo + (j + 1) * 128 > T:
                        lane = lax.broadcasted_iota(jnp.int32, (TM, 128), 1)
                        parts[j] = jnp.where(lane < T - (lo + j * 128), parts[j], -jnp.inf)
                    ss[:, lo + j * 128:lo + (j + 1) * 128] = parts[j]
                    m128 = parts[j] if m128 is None else jnp.maximum(m128, parts[j])
        if a_tail:
            x1 = xs[_rows(NTILE - 1), :] + 0.5 * y
            xs[_rows(NTILE - 1), :] = x1
            h1 = _ln(x1).astype(BF)
            hs[pl.ds(_krow(NTILE - 1), TM), :] = h1
        if do_prev:
            x2 = xs[_rows(i - 1), :] + accs[...] * (1.0 / jnp.sum(ls[...], axis=-1, keepdims=True))
            xs[_rows(i - 1), :] = x2
            h2 = _ln(x2).astype(BF)
        for t in conv_tiles[0]:
            conv(t)
        if a_tail:
            qv = _dot(h1, mqv[...])
            qs[_rows(NTILE - 1), :] = qv[:, :D].astype(BF)
            vs[pl.ds(_krow(NTILE - 1), TM), :] = qv[:, D:].astype(BF)
        if do_prev:
            y2 = _dot(h2, wp1[...])
            g = y2[:, :D] * _sigmoid(y2[:, D:])
            gs[pl.ds(_grow(i - 1) + HALO, TM), :] = g
        if do_cur:
            mx = jnp.max(m128, axis=-1, keepdims=True)
            acc = None
            l128 = None
            for c in range(NKC):
                p = jnp.exp2(ss[:, c * KC:(c + 1) * KC] - mx)
                for j in range(KC // 128):
                    pj = p[:, j * 128:(j + 1) * 128]
                    l128 = pj if l128 is None else l128 + pj
                pv = _dot(p.astype(BF), vs[pl.ds(kb + c * KC, KC), :])
                acc = pv if acc is None else acc + pv
            accs[...] = acc
            ls[...] = l128
        for t in conv_tiles[1]:
            conv(t)

    def bn_silu(i):
        dc = (dcs[_rows(i), :] - st[0:1, :]) * st[2:3, :]
        zs[...] = _silu(dc).astype(BF)

    def c_step(i, do_prev, do_cur, do_next):
        if do_cur:
            y3 = _dot(zs[...], wp2[...])
        if do_prev:
            y = _dot(us[...], w2b[...])
        if do_cur:
            x3 = xs[_rows(i), :] + y3
            xs[_rows(i), :] = x3
            h3 = _ln(x3).astype(BF)
            ffa(h3, w2a)
        if do_prev:
            x4 = xs[_rows(i - 1), :] + 0.5 * y
            qs[_rows(i - 1), :] = _ln(x4).astype(BF)
            ocopy(i - 1).start()
        if do_next:
            bn_silu(jnp.minimum(i + 1, NTILE - 1))

    W1A, W1B, WQ, WK, WV, WO, WP1, DW, WP2, W2A, W2B = range(11)
    xcopy(0).start()
    wcopy(W1A).start()
    for b in range(B):
        hs[b * TP + T:(b + 1) * TP, :] = jnp.zeros((TP - T, D), BF)
        vs[b * TP + T:(b + 1) * TP, :] = jnp.zeros((TP - T, D), BF)
        g0 = b * (T + 2 * HALO)
        gs[g0:g0 + HALO, :] = jnp.zeros((HALO, D), F32)
        gs[g0 + HALO + T:g0 + T + 2 * HALO, :] = jnp.zeros((HALO, D), F32)
    st[...] = jnp.zeros(st.shape, F32)
    xcopy(0).wait()
    wcopy(W1A).wait()
    for k in (WQ, WK, WV, WO, W1B):
        wcopy(k).start()
    xcopy(1).start()
    a_step(0, False, True)
    for k in (WQ, WK, WV, WO):
        wcopy(k).wait()
    for t in range(2, NTILE):
        xcopy(t).start()
    for k in (WP1, DW, WP2, W2A, W2B):
        wcopy(k).start()
    mqv[:, :D] = (_dot_nt(wq[...], wk[...]) * (D ** -0.5 * LOG2E)).astype(BF)
    mqv[:, D:] = _dot(wv[...], wo[...]).astype(BF)
    wcopy(W1B).wait()

    def a_body(i, c):
        xcopy(i).wait()
        a_step(i, True, True)
        return c
    lax.fori_loop(1, NTILE, a_body, 0)

    for k in (WP1, DW, WP2, W2A, W2B):
        wcopy(k).wait()
    b_step(0, False, True, ((), ()), a_tail=True)
    b_step(1, True, True, ((), ()))

    def b_body(i, c):
        b_step(i, True, True, ((), (i - 2,)))
        return c
    lax.fori_loop(2, NTILE, b_body, 0)

    b_step(NTILE, True, False, ((), (NTILE - 2, NTILE - 1)))
    st[2:3, :] = lax.rsqrt(st[1:2, :] * (1.0 / (B * T)) + EPS)
    bn_silu(0)
    c_step(0, False, True, True)

    def c_body(i, c):
        c_step(i, True, True, True)
        return c
    lax.fori_loop(1, NTILE, c_body, 0)
    c_step(NTILE, True, False, False)
    for t in range(NTILE):
        ocopy(t).wait()


@jax.jit
def pallas_standalone__conformer_family_conformer__speech_kernel(x, w_ff1_a, w_ff1_b, w_q, w_k, w_v, w_o, w_pw1, dw, w_pw2, w_ff2_a, w_ff2_b):
    xf = x.reshape(B * T, D)
    ws = (w_ff1_a, w_ff1_b, w_q, w_k, w_v, w_o, w_pw1, dw, w_pw2, w_ff2_a, w_ff2_b)
    hbm = pl.BlockSpec(memory_space=pl.ANY)
    out = pl.pallas_call(
        kernel,
        in_specs=[hbm] * 12,
        out_specs=hbm,
        out_shape=jax.ShapeDtypeStruct((B * T, D), x.dtype),
        scratch_shapes=[pltpu.VMEM(w.shape, BF) for w in ws] + [
            pltpu.VMEM((B * T, D), F32),
            pltpu.VMEM((B * TP, D), BF),
            pltpu.VMEM((B * T, D), BF),
            pltpu.VMEM((B * TP, D), BF),
            pltpu.VMEM((B * (T + 2 * HALO), D), F32),
            pltpu.VMEM((B * T, D), F32),
            pltpu.VMEM((TM, F), BF),
            pltpu.VMEM((TM, TP), F32),
            pltpu.VMEM((TM, D), F32),
            pltpu.VMEM((TM, 128), F32),
            pltpu.VMEM((TM, D), BF),
            pltpu.VMEM((D, 2 * D), BF),
            pltpu.VMEM((8, D), F32),
            pltpu.SemaphoreType.DMA((11,)),
            pltpu.SemaphoreType.DMA((NTILE,)),
            pltpu.SemaphoreType.DMA((1,)),
        ],
        compiler_params=pltpu.CompilerParams(vmem_limit_bytes=124 * 1024 * 1024),
    )(xf, *ws)
    return out.reshape(B, T, D)
```

```python
import jax
import jax.numpy as jnp
from jax import lax
from jax.experimental import pallas as pl
from jax.experimental.pallas import tpu as pltpu

B, T, D, F, KW = 2, 4000, 512, 2048, 15
TP = 4096
TM = 400
NT = T // TM
NTILE = B * NT
KC = 512
NKC = TP // KC
RU = 80
NRB = TM // RU
NV = TM // 8
EPS = 1e-5
LOG2E = 1.4426950408889634
BF = jnp.bfloat16
F32 = jnp.float32
HALO = 8


def _ln(x):
    m = jnp.mean(x, axis=-1, keepdims=True)
    xc = x - m
    v = jnp.mean(xc * xc, axis=-1, keepdims=True)
    return xc * lax.rsqrt(v + EPS)


def _dot(a, b):
    return jnp.dot(a, b, preferred_element_type=F32)


def _dot_nt(a, b):
    return lax.dot_general(a, b, (((1,), (1,)), ((), ())), preferred_element_type=F32)


def _sigmoid(x):
    return 0.5 * jnp.tanh(0.5 * x) + 0.5


def _silu(x):
    hx = 0.5 * x
    return hx * jnp.tanh(hx) + hx


def _mult(v, n):
    return v if isinstance(v, int) else pl.multiple_of(v, n)


def _rows(i, rb=None):
    if rb is None:
        return pl.ds(_mult(i * TM, 16), TM)
    return pl.ds(_mult(i * TM + rb * RU, 16), RU)


def _krows(i):
    return pl.ds(_mult((i // NT) * TP + (i % NT) * TM, 16), TM)


def _grow(i):
    return _mult((i // NT) * (T + 2 * HALO) + (i % NT) * TM, 8)


def rsl(rb):
    return slice(rb * RU, (rb + 1) * RU)


def csl(n):
    return slice(n * 128, (n + 1) * 128)


def kernel(x_hbm, w1a_h, w1b_h, wq_h, wk_h, wv_h, wo_h, wp1_h, dw_h, wp2_h, w2a_h, w2b_h, o_hbm,
           w1a, w1b, wq, wk, wv, wo, wp1, dw_ref, wp2, w2a, w2b,
           xs, hs, qs, vs, gs, dcs, us, ss, accs, ls, zs, mqv, st, bn,
           wsem, xsem, osem):
    def wcopy(k):
        srcs = (w1a_h, w1b_h, wq_h, wk_h, wv_h, wo_h, wp1_h, dw_h, wp2_h, w2a_h, w2b_h)
        dsts = (w1a, w1b, wq, wk, wv, wo, wp1, dw_ref, wp2, w2a, w2b)
        return pltpu.make_async_copy(srcs[k], dsts[k], wsem.at[k])

    def xcopy(i):
        return pltpu.make_async_copy(x_hbm.at[_rows(i), :], qs.at[_rows(i), :], xsem.at[i])

    def ocopy(i):
        return pltpu.make_async_copy(qs.at[_rows(i), :], o_hbm.at[_rows(i), :], osem.at[0])

    def make_pin():
        nv = jnp.abs(w1a[0:16, 0:128].astype(F32)[0:1, :])

        def pin(val, dep):
            never = jnp.broadcast_to(nv, val.shape) < 0.0
            return jnp.where(never, dep, val)
        return pin

    def acc_matmul(lhs_ref, w_ref, pin, deadlines):
        acc = {}
        for kg in range(lhs_ref.shape[1] // 512):
            part = _dot(lhs_ref[:, kg * 512:(kg + 1) * 512], w_ref[kg * 512:(kg + 1) * 512, :])
            for n in range(4):
                for rb in range(NRB):
                    blk = part[rsl(rb), csl(n)]
                    if kg == 0:
                        acc[n, rb] = blk
                        continue
                    a = acc[n, rb]
                    if (kg, n, rb) in deadlines:
                        a = pin(a, deadlines[kg, n, rb]())
                    acc[n, rb] = a + blk
        return acc

    def spread(first, count, unit_blocks):
        return {(first + rb * count // NRB, n, rb): (lambda rb=rb, n=n: unit_blocks(rb)[:, csl(n)])
                for rb in range(NRB) for n in range(4)}

    def memo(fn):
        cache = {}

        def get(rb):
            if rb not in cache:
                cache[rb] = fn(rb)
            return cache[rb]
        return get

    def ffa(h_bf, wa, pin, deadlines):
        for c in range(F // 512):
            u = _dot(h_bf, wa[:, c * 512:(c + 1) * 512])
            if not any(k[0] == c for k in deadlines):
                us[:, c * 512:(c + 1) * 512] = _silu(u).astype(BF)
                continue
            for rb in range(NRB):
                cols = []
                for n in range(4):
                    blk = u[rsl(rb), csl(n)]
                    if (c, n, rb) in deadlines:
                        blk = pin(blk, deadlines[c, n, rb]())
                    cols.append(blk)
                us[rsl(rb), c * 512:(c + 1) * 512] = _silu(jnp.concatenate(cols, axis=1)).astype(BF)

    def cat_rows(get):
        return jnp.concatenate([get(rb) for rb in range(NRB)], axis=0)

    def ff1_tail_unit(i, yacc):
        def unit(rb):
            y = jnp.concatenate([yacc[n, rb] for n in range(4)], axis=1)
            x1 = xs[_rows(i, rb), :] + 0.5 * y
            xs[_rows(i, rb), :] = x1
            return _ln(x1)
        return memo(unit)

    def store_qv(i, h1):
        h1 = h1.astype(BF)
        hs[_krows(i), :] = h1
        return _dot(h1, mqv[...])

    def a_step(i, do_prev):
        pin = make_pin()

        def lnx(rb):
            x = qs[_rows(i, rb), :].astype(F32)
            xs[_rows(i, rb), :] = x
            return _ln(x)
        lnx = memo(lnx)
        dl = {}
        if do_prev:
            yacc = acc_matmul(us, w1b, pin, spread(1, 3, lnx))
            tail = ff1_tail_unit(i - 1, yacc)
            dl = spread(1, 3, tail)
        ffa(cat_rows(lnx).astype(BF), w1a, pin, dl)
        if do_prev:
            qv = store_qv(i - 1, cat_rows(tail))
            qs[_rows(i - 1), :] = qv[:, :D].astype(BF)
            vs[_krows(i - 1), :] = qv[:, D:].astype(BF)

    def conv_stream(t, pin):
        g0 = _grow(t)
        r0 = _mult(t * TM, 8)
        sub = lax.broadcasted_iota(jnp.int32, (8, 128), 0)
        cs = {}

        def rot(v):
            return [v] + [pltpu.roll(v, 8 - s, 0) for s in range(1, 8)]

        def shift(ra, rb_):
            return [ra[0]] + [jnp.where(sub < 8 - s, ra[s], rb_[s]) for s in range(1, 8)]

        def step(k, dep):
            cb, j = divmod(k, NV)
            cols = csl(cb)
            rel = (lambda v: v) if dep is None else (lambda v: pin(v, dep))
            ld = lambda jj: rel(gs[pl.ds(_mult(g0 + 8 * jj, 8), 8), cols])
            if j == 0:
                cs["w"] = [rel(jnp.broadcast_to(dw_ref[kk:kk + 1, cols].astype(F32), (8, 128))) for kk in range(KW)]
                ra, rb_ = rot(ld(0)), rot(ld(1))
                cs["g"], cs["r"] = shift(ra, rb_), rb_
            w = cs["w"]
            rn = rot(ld(j + 2))
            gn = shift(cs["r"], rn)
            terms = [cs["g"][s] * w[s - 1] for s in range(1, 8)] + [gn[s] * w[7 + s] for s in range(8)]
            while len(terms) > 1:
                terms = [terms[q] + terms[q + 1] for q in range(0, len(terms) - 1, 2)] + ([terms[-1]] if len(terms) % 2 else [])
            o = terms[0]
            dcs[pl.ds(_mult(r0 + 8 * j, 8), 8), cols] = o
            cs["g"], cs["r"] = gn, rn
            if j == 0:
                cs["c"] = o
            else:
                d = o - cs["c"]
                cs["s1"] = d if j == 1 else cs["s1"] + d
                cs["s2"] = d * d if j == 1 else cs["s2"] + d * d
            if j == NV - 1:
                tmean = cs["c"] + cs["s1"] * (1.0 / NV)
                tm2 = cs["s2"] - cs["s1"] * cs["s1"] * (1.0 / NV)
                n = jnp.zeros((8, 128), F32) + jnp.asarray(t, F32)
                mean_old = st[0, :, cols]
                delta = tmean - mean_old
                st[0, :, cols] = mean_old + delta / (n + 1.0)
                st[1, :, cols] = st[1, :, cols] + tm2 + delta * delta * (n * NV / (n + 1.0))
            return o
        return step

    def attn_tail_unit(i):
        def unit(rb):
            inv = 1.0 / jnp.sum(ls[rsl(rb), :], axis=-1, keepdims=True)
            x2 = xs[_rows(i, rb), :] + accs[rsl(rb), :] * inv
            xs[_rows(i, rb), :] = x2
            return _ln(x2)
        return memo(unit)

    def glu_block(i, y2, n):
        g = y2[:, csl(n)] * _sigmoid(y2[:, D + n * 128:D + (n + 1) * 128])
        gs[pl.ds(_mult(_grow(i) + HALO, 8), TM), csl(n)] = g
        return g

    def b_step(i, prev, do_conv):
        pin = make_pin()
        kb = _mult((i // NT) * TP, TP)
        if prev == "ff1":
            tail = ff1_tail_unit(NTILE - 1, acc_matmul(us, w1b, pin, {}))
        else:
            tail = attn_tail_unit(i - 1)
        q = qs[_rows(i), :]
        m = [None] * NRB
        mhist = []
        sp = {}
        MD = 2
        for c in range(NKC):
            kt = hs[pl.ds(kb + c * KC, KC), :]
            if c >= MD:
                d = None
                for rb in range(NRB):
                    for v in range(RU // 8):
                        t_ = mhist[c - MD][rb][v * 8:(v + 1) * 8, :]
                        d = t_ if d is None else jnp.maximum(d, t_)
                top = [kt[0:16, csl(j)] for j in range(4)]
                top[2] = pin(top[2], jnp.concatenate([d, d], axis=0).astype(BF))
                kt = jnp.concatenate([jnp.concatenate(top, axis=1), kt[16:, :]], axis=0)
            sc = _dot_nt(q, kt)
            for rb in range(NRB):
                parts = [sc[rsl(rb), csl(j)] for j in range(4)]
                if c == NKC - 1:
                    lane = lax.broadcasted_iota(jnp.int32, (RU, 128), 1)
                    parts[3] = jnp.where(lane < T - (c * KC + 384), parts[3], -jnp.inf)
                if c == 1 + rb:
                    hf = tail(rb)
                    parts = [pin(parts[j], hf[:, csl(j)]) for j in range(4)]
                mm = jnp.maximum(jnp.maximum(parts[0], parts[1]), jnp.maximum(parts[2], parts[3]))
                m[rb] = mm if m[rb] is None else jnp.maximum(m[rb], mm)
                for j in range(4):
                    sp[c, rb, j] = parts[j]
            mhist.append(list(m))
        if prev == "ff1":
            mid = store_qv(NTILE - 1, cat_rows(tail))
        else:
            mid = _dot(cat_rows(tail).astype(BF), wp1[...])
        mxb = [jnp.broadcast_to(jnp.max(m[rb], axis=-1, keepdims=True), (RU, 128)) for rb in range(NRB)]
        C0, RL = 2, 25
        nslots = (NKC - C0) * 4 * NV
        where = {C0 * 4 * NV + k * nslots // (4 * NV): k for k in range(4 * NV)} if do_conv else {}
        conv = conv_stream(i - 2, pin) if do_conv else None
        acc, l128, pvs = {}, [None] * NRB, []
        for c in range(NKC):
            pbl = []
            for rb in range(NRB):
                mb = mxb[rb]
                if c == 1:
                    mb = pin(mb, mid[rsl(rb), D:D + 128])
                elif c >= 2:
                    mb = pin(mb, pvs[c - 1][rsl(rb), 0:128])
                pj = [jnp.exp2(sp[c, rb, j] - mb) for j in range(4)]
                lsum = (pj[0] + pj[1]) + (pj[2] + pj[3])
                l128[rb] = lsum if l128[rb] is None else l128[rb] + lsum
                pbl.append(jnp.concatenate(pj, axis=1).astype(BF))
            pv = _dot(jnp.concatenate(pbl, axis=0), vs[pl.ds(kb + c * KC, KC), :])
            pvs.append(pv)
            for n in range(4):
                side = None
                if c == 1:
                    if prev == "ff1":
                        qb, vb = mid[:, csl(n)].astype(BF), mid[:, D + n * 128:D + (n + 1) * 128].astype(BF)
                        qs[_rows(NTILE - 1), csl(n)] = qb
                        vs[_krows(NTILE - 1), csl(n)] = vb
                        side = qb.astype(F32) + vb.astype(F32)
                    else:
                        side = glu_block(i - 1, mid, n)
                for v in range(NV):
                    blk = pv[v * 8:(v + 1) * 8, csl(n)]
                    if c == 0:
                        acc[n, v] = blk
                        continue
                    a = acc[n, v]
                    if side is not None:
                        a = pin(a, side[v * 8:(v + 1) * 8, :])
                    slot = (c * 4 + n) * NV + v
                    if slot in where:
                        s0 = slot - RL
                        dep = pvs[s0 // (4 * NV)][(s0 % NV) * 8:(s0 % NV) * 8 + 8, csl((s0 // NV) % 4)]
                        a = pin(a, conv(where[slot], dep))
                    if n == 2:
                        rb, vv = divmod(v, RU // 8)
                        a = pin(a, l128[rb][vv * 8:(vv + 1) * 8, :])
                    acc[n, v] = a + blk
        for n in range(4):
            for v in range(NV):
                accs[v * 8:(v + 1) * 8, csl(n)] = acc[n, v]
        for rb in range(NRB):
            ls[rsl(rb), :] = l128[rb]

    def bn_silu_unit(i):
        def unit(rb):
            z = _silu((dcs[_rows(i, rb), :] - bn[0:1, :]) * bn[1:2, :])
            zs[rsl(rb), :] = z.astype(BF)
            return z
        return memo(unit)

    def c_step(i, do_prev, do_cur, do_next):
        pin = make_pin()
        if do_cur:
            y3 = _dot(zs[...], wp2[...])

            def x3u(rb):
                x3 = xs[_rows(i, rb), :] + y3[rsl(rb), :]
                xs[_rows(i, rb), :] = x3
                return _ln(x3)
            x3u = memo(x3u)
        if do_prev:
            yacc = acc_matmul(us, w2b, pin, spread(1, 3, x3u) if do_cur else {})

            def out_unit(rb):
                y = jnp.concatenate([yacc[n, rb] for n in range(4)], axis=1)
                o = _ln(xs[_rows(i - 1, rb), :] + 0.5 * y)
                qs[_rows(i - 1, rb), :] = o.astype(BF)
                return o
            out_unit = memo(out_unit)
        if do_cur:
            dl = {}
            if do_prev:
                dl.update(spread(1, 2, out_unit))
            if do_next:
                dl.update(spread(3, 1, bn_silu_unit(jnp.minimum(i + 1, NTILE - 1))))
            ffa(cat_rows(x3u).astype(BF), w2a, pin, dl)
        elif do_prev:
            cat_rows(out_unit)
        if do_prev:
            ocopy(i - 1).start()

    W1A, W1B, WQ, WK, WV, WO, WP1, DW, WP2, W2A, W2B = range(11)
    xcopy(0).start()
    wcopy(W1A).start()
    for b in range(B):
        hs[b * TP + T:(b + 1) * TP, :] = jnp.zeros((TP - T, D), BF)
        vs[b * TP + T:(b + 1) * TP, :] = jnp.zeros((TP - T, D), BF)
        g0 = b * (T + 2 * HALO)
        gs[g0:g0 + HALO, :] = jnp.zeros((HALO, D), F32)
        gs[g0 + HALO + T:g0 + T + 2 * HALO, :] = jnp.zeros((HALO, D), F32)
    st[...] = jnp.zeros(st.shape, F32)
    xcopy(0).wait()
    wcopy(W1A).wait()
    for k in (WQ, WK, WV, WO, W1B):
        wcopy(k).start()
    xcopy(1).start()
    a_step(0, False)
    for k in (WQ, WK, WV, WO):
        wcopy(k).wait()
    for t in range(2, NTILE):
        xcopy(t).start()
    for k in (WP1, DW, WP2, W2A, W2B):
        wcopy(k).start()
    mqv[:, :D] = (_dot_nt(wq[...], wk[...]) * (D ** -0.5 * LOG2E)).astype(BF)
    mqv[:, D:] = _dot(wv[...], wo[...]).astype(BF)
    wcopy(W1B).wait()

    def a_body(i, c):
        xcopy(i).wait()
        a_step(i, True)
        return c
    lax.fori_loop(1, NTILE, a_body, 0)

    for k in (WP1, DW, WP2, W2A, W2B):
        wcopy(k).wait()
    b_step(0, "ff1", False)
    b_step(1, "attn", False)

    def b_body(i, c):
        b_step(i, "attn", True)
        return c
    lax.fori_loop(2, NTILE, b_body, 0)

    pin = make_pin()
    y2 = _dot(cat_rows(attn_tail_unit(NTILE - 1)).astype(BF), wp1[...])
    for n in range(4):
        glu_block(NTILE - 1, y2, n)
    for t in (NTILE - 2, NTILE - 1):
        conv = conv_stream(t, pin)
        for k in range(4 * NV):
            conv(k, None)
    mean8, m28 = st[0], st[1]
    mu = jnp.mean(mean8, axis=0, keepdims=True)
    dm = mean8 - mu
    var = (jnp.sum(m28, axis=0, keepdims=True) + (B * T // 8) * jnp.sum(dm * dm, axis=0, keepdims=True)) * (1.0 / (B * T))
    bn[0:1, :] = mu
    bn[1:2, :] = lax.rsqrt(var + EPS)
    cat_rows(bn_silu_unit(0))
    c_step(0, False, True, True)

    def c_body(i, c):
        c_step(i, True, True, True)
        return c
    lax.fori_loop(1, NTILE, c_body, 0)
    c_step(NTILE, True, False, False)
    for t in range(NTILE):
        ocopy(t).wait()


@jax.jit
def pallas_standalone__conformer_family_conformer__speech_kernel(x, w_ff1_a, w_ff1_b, w_q, w_k, w_v, w_o, w_pw1, dw, w_pw2, w_ff2_a, w_ff2_b):
    xf = x.reshape(B * T, D)
    ws = (w_ff1_a, w_ff1_b, w_q, w_k, w_v, w_o, w_pw1, dw, w_pw2, w_ff2_a, w_ff2_b)
    hbm = pl.BlockSpec(memory_space=pl.ANY)
    out = pl.pallas_call(
        kernel,
        in_specs=[hbm] * 12,
        out_specs=hbm,
        out_shape=jax.ShapeDtypeStruct((B * T, D), x.dtype),
        scratch_shapes=[pltpu.VMEM(w.shape, BF) for w in ws] + [
            pltpu.VMEM((B * T, D), F32),
            pltpu.VMEM((B * TP, D), BF),
            pltpu.VMEM((B * T, D), BF),
            pltpu.VMEM((B * TP, D), BF),
            pltpu.VMEM((B * (T + 2 * HALO), D), F32),
            pltpu.VMEM((B * T, D), F32),
            pltpu.VMEM((TM, F), BF),
            pltpu.VMEM((TM, TP), F32),
            pltpu.VMEM((TM, D), F32),
            pltpu.VMEM((TM, 128), F32),
            pltpu.VMEM((TM, D), BF),
            pltpu.VMEM((D, 2 * D), BF),
            pltpu.VMEM((2, 8, D), F32),
            pltpu.VMEM((8, D), F32),
            pltpu.SemaphoreType.DMA((11,)),
            pltpu.SemaphoreType.DMA((NTILE,)),
            pltpu.SemaphoreType.DMA((1,)),
        ],
        compiler_params=pltpu.CompilerParams(vmem_limit_bytes=124 * 1024 * 1024),
    )(xf, *ws)
    return out.reshape(B, T, D)
```

```python
import jax
import jax.numpy as jnp
from jax import lax
from jax.experimental import pallas as pl
from jax.experimental.pallas import tpu as pltpu

B, T, D, F, KW = 2, 4000, 512, 2048, 15
TP = 4096
TM = 400
NT = T // TM
NTILE = B * NT
KC = 512
NKC = TP // KC
RU = 80
NRB = TM // RU
NV = TM // 8
EPS = 1e-5
LOG2E = 1.4426950408889634
BF = jnp.bfloat16
F32 = jnp.float32
U32 = jnp.uint32
HALO = 8
GR = B * (T + 2 * HALO)


def _ln(x):
    m = jnp.mean(x, axis=-1, keepdims=True)
    xc = x - m
    v = jnp.mean(xc * xc, axis=-1, keepdims=True)
    return xc * lax.rsqrt(v + EPS)


def pack(x):
    return pltpu.bitcast(x.astype(BF), U32)


def unpack(w):
    return pltpu.bitcast(w, BF)


def _dot(a32, b32):
    return jnp.dot(unpack(a32), unpack(b32), preferred_element_type=F32)


def _dot_nt(a32, b32):
    return lax.dot_general(unpack(a32), unpack(b32), (((1,), (1,)), ((), ())), preferred_element_type=F32)


def _sigmoid(x):
    return 0.5 * jnp.tanh(0.5 * x) + 0.5


def _silu(x):
    hx = 0.5 * x
    return hx * jnp.tanh(hx) + hx


def _mult(v, n):
    return v if isinstance(v, int) else pl.multiple_of(v, n)


def _rows(i, rb=None):
    if rb is None:
        return pl.ds(_mult(i * TM, 8), TM)
    return pl.ds(_mult(i * TM + rb * RU, 8), RU)


def _prows(i, rb=None):
    if rb is None:
        return pl.ds(_mult(i * (TM // 2), 8), TM // 2)
    return pl.ds(_mult(i * (TM // 2) + rb * (RU // 2), 8), RU // 2)


def _pkrows(i):
    return pl.ds(_mult((i // NT) * (TP // 2) + (i % NT) * (TM // 2), 8), TM // 2)


def _grow(i):
    return (i // NT) * (T + 2 * HALO) + (i % NT) * TM


def rsl(rb):
    return slice(rb * RU, (rb + 1) * RU)


def csl(n):
    return slice(n * 128, (n + 1) * 128)


def kernel(x_hbm, w1a_h, w1b_h, wq_h, wk_h, wv_h, wo_h, wp1_h, dw_h, wp2_h, w2a_h, w2b_h, o_hbm,
           w1a, w1b, wq, wk, wv, wo, wp1, wp2, w2a, w2b, dw_ref,
           xs, hs, qs, vs, gs, dcs, us, accs, ls, zs, mqv, dwt, st, bn,
           wsem, csem, xsem, osem):
    def wcopy(k):
        srcs = (w1a_h, w1b_h, wq_h, wk_h, wv_h, wo_h, wp1_h, wp2_h, w2a_h, w2b_h, dw_h)
        dsts = (w1a, w1b, wq, wk, wv, wo, wp1, wp2, w2a, w2b)
        dst = dw_ref if k == 10 else dsts[k].bitcast(BF)
        return pltpu.make_async_copy(srcs[k], dst, wsem.at[k])

    def w1a_copy(c):
        return pltpu.make_async_copy(w1a_h.at[:, c * 512:(c + 1) * 512], w1a.bitcast(BF).at[:, c * 512:(c + 1) * 512], csem.at[c])

    def w1b_copy(c):
        return pltpu.make_async_copy(w1b_h.at[c * 512:(c + 1) * 512, :], w1b.bitcast(BF).at[c * 512:(c + 1) * 512, :], csem.at[4 + c])

    def xcopy(i):
        rows = pl.ds(_mult(i * TM, 16), TM)
        return pltpu.make_async_copy(x_hbm.at[rows, :], qs.bitcast(BF).at[rows, :], xsem.at[i])

    def ocopy(i):
        rows = pl.ds(_mult(i * TM, 16), TM)
        return pltpu.make_async_copy(qs.bitcast(BF).at[rows, :], o_hbm.at[rows, :], osem.at[0])

    def make_pin():
        nv = jnp.abs(bn[2:3, :])

        def pin(val, dep):
            never = jnp.broadcast_to(nv[:, :val.shape[1]], val.shape) < 0.0
            return jnp.where(never, dep, val)
        return pin

    def memo(fn):
        cache = {}

        def get(rb, rel=None):
            if rb not in cache:
                cache[rb] = fn(rb, rel)
            return cache[rb]
        return get

    def cat_rows(get):
        return jnp.concatenate([get(rb) for rb in range(NRB)], axis=0)

    def pin_rhs(w32, pin, tokens):
        if not tokens:
            return w32
        cols = []
        for n in range(4):
            col = w32[:, csl(n)]
            if n in tokens:
                tk = tokens[n]()
                k = tk.shape[0]
                col = jnp.concatenate([pin(col[:k], tk), col[k:]], axis=0)
            cols.append(col)
        return jnp.concatenate(cols, axis=1)

    def spread(first, count, unit, res, lead):
        out = {}
        for rb in range(NRB):
            p = first + rb * count // NRB
            pr = min(p - lead, 4 * (p // 4) - 1)

            def token(rb=rb, pr=pr):
                rel = None
                if pr >= 0 and lead < 90:
                    rel = jnp.concatenate([res[pr // 4][rsl(rb), csl(pr % 4)]] * 4, axis=1)
                u_ = unit(rb, rel)
                return jnp.concatenate([u_[:, csl(n)] for n in range(4)], axis=0)
            assert (p // 4, p % 4) not in out
            out[p // 4, p % 4] = token
        return out

    def tok(deadlines, c):
        return {n: f for (cc, n), f in deadlines.items() if cc == c}

    def acc_matmul(lhs, w, pin, deadlines, res, pre=None):
        acc = None
        for kg in range(4):
            if pre:
                pre(kg)
            part = _dot(lhs[:, kg * 512:(kg + 1) * 512], pin_rhs(w[kg * 256:(kg + 1) * 256, :], pin, tok(deadlines, kg)))
            res.append(part)
            if acc is None:
                acc = [part[rsl(rb), :] for rb in range(NRB)]
            else:
                acc = [acc[rb] + part[rsl(rb), :] for rb in range(NRB)]
        return acc

    def ffa(h32, wa, pin, deadlines, res, pre=None):
        for c in range(F // 512):
            if pre:
                pre(c)
            u = _dot(h32, pin_rhs(wa[:, c * 512:(c + 1) * 512], pin, tok(deadlines, c)))
            res.append(u)
            us[:, c * 512:(c + 1) * 512] = pack(_silu(u))

    def held(val, rel, pin):
        if rel is None:
            return val
        if val.dtype == U32:
            return pin(val, pltpu.bitcast(rel[:val.shape[0]], U32))
        return pin(val, rel)

    def ff1_tail_unit(i, yacc, pin):
        def unit(rb, rel):
            x1 = unpack(held(qs[_prows(i, rb), :], rel, pin)).astype(F32) + 0.5 * yacc[rb]
            xs[_rows(i, rb), :] = x1
            return pack(_ln(x1))
        return memo(unit)

    def store_qv(i, h1):
        hs[_pkrows(i), :] = h1
        return _dot(h1, mqv[...])

    def a_step(i, do_prev, pre_a=None, pre_b=None, pre_qv=None):
        pin = make_pin()
        lnx = memo(lambda rb, rel: pack(_ln(unpack(held(qs[_prows(i, rb), :], rel, pin)).astype(F32))))
        dl, r1, r2 = {}, [], []
        if do_prev:
            yacc = acc_matmul(us, w1b, pin, spread(4, 10, lnx, r1, 3), r1, pre_b)
            tail = ff1_tail_unit(i - 1, yacc, pin)
            dl = spread(5, 10, tail, r2, 3)
        ffa(cat_rows(lnx), w1a, pin, dl, r2, pre_a)
        if do_prev:
            if pre_qv:
                pre_qv()
            qv = store_qv(i - 1, cat_rows(tail))
            qs[_prows(i - 1), :] = pack(qv[:, :D])
            vs[_pkrows(i - 1), :] = pack(qv[:, D:])

    def conv_stream(t, pin):
        g0 = _grow(t)
        cs = [dict() for _ in range(4)]
        sub = lax.broadcasted_iota(jnp.int32, (8, 128), 0)

        def rot(v):
            return [v] + [pltpu.roll(v, 8 - s_, 0) for s_ in range(1, 8)]

        def shift(ra, rb_):
            return [ra[0]] + [jnp.where(sub < 8 - s_, ra[s_], rb_[s_]) for s_ in range(1, 8)]

        def step(cb, j, dep):
            c_ = cs[cb]
            rel = (lambda v: v) if dep is None else (lambda v: pin(v, dep))
            ld = lambda jj: rel(gs[pl.ds(_mult(g0 + cb * GR + 8 * jj, 8), 8), :])
            if c_.get("next") != j:
                ra, rb_ = rot(ld(j)), rot(ld(j + 1))
                c_["G"], c_["R"] = shift(ra, rb_), rb_
                c_["w"] = [dwt[(kk * 4 + cb) * 8:(kk * 4 + cb + 1) * 8, :] for kk in range(KW)]
            rn = rot(ld(j + 2))
            gn = shift(c_["R"], rn)
            terms = [c_["G"][s_] * c_["w"][s_ - 1] for s_ in range(1, 8)] + [gn[s_] * c_["w"][7 + s_] for s_ in range(8)]
            c_["G"], c_["R"], c_["next"] = gn, rn, j + 1
            while len(terms) > 1:
                terms = [terms[q] + terms[q + 1] for q in range(0, len(terms) - 1, 2)] + ([terms[-1]] if len(terms) % 2 else [])
            o = terms[0]
            dcs[pl.ds(_mult(t * TM + 8 * j, 8), 8), csl(cb)] = o
            if j == 0:
                c_["c"] = o
            else:
                d = o - c_["c"]
                c_["s1"] = d if j == 1 else c_["s1"] + d
                c_["s2"] = d * d if j == 1 else c_["s2"] + d * d
            if j == NV - 1:
                cols = csl(cb)
                tmean = c_["c"] + c_["s1"] * (1.0 / NV)
                tm2 = c_["s2"] - c_["s1"] * c_["s1"] * (1.0 / NV)
                n = jnp.zeros((8, 128), F32) + jnp.asarray(t, F32)
                mean_old = st[0, :, cols]
                delta = tmean - mean_old
                st[0, :, cols] = mean_old + delta / (n + 1.0)
                st[1, :, cols] = st[1, :, cols] + tm2 + delta * delta * (n * NV / (n + 1.0))
            return o
        return step

    def attn_tail_unit(i, pin):
        def unit(rb, rel):
            lsum = ls[rsl(rb), :]
            if rel is not None:
                lsum = pin(lsum, rel[:, 0:128])
            inv = 1.0 / jnp.sum(lsum, axis=-1, keepdims=True)
            x2 = held(xs[_rows(i, rb), :], rel, pin) + accs[rsl(rb), :] * inv
            xs[_rows(i, rb), :] = x2
            return pack(_ln(x2))
        return memo(unit)

    def glu_block(i, y2, n):
        g = y2[:, csl(n)] * _sigmoid(y2[:, D + n * 128:D + (n + 1) * 128])
        gs[pl.ds(_mult(_grow(i) + (n * GR + HALO), 8), TM), :] = g
        return g

    def b_step(i, prev, do_conv):
        pin = make_pin()
        kb = _mult((i // NT) * (TP // 2), TP // 2)
        if prev == "ff1":
            tail = ff1_tail_unit(NTILE - 1, acc_matmul(us, w1b, pin, {}, []), pin)
        else:
            tail = attn_tail_unit(i - 1, pin)
        q = qs[_prows(i), :]
        m = [None] * NRB
        mhist = []
        sp = {}
        MD, LN0, LNL = 2, 2, 0
        scs = []
        JS = 0 if do_conv else 0
        conv = conv_stream(i - 2, pin) if do_conv else None
        early = [(cb, j) for cb in range(4) for j in range(JS)]
        late = [(cb, j) for cb in range(4) for j in range(JS, NV)] if do_conv else []
        eslots = [(c, n) for c in range(1, NKC) for n in (0, 3)]
        emap = {}
        for k, u_ in enumerate(early):
            emap.setdefault(eslots[k * len(eslots) // len(early)], []).append(u_)
        for c in range(NKC):
            kt = hs[pl.ds(kb + c * (KC // 2), KC // 2), :]
            rowsets = [kt[n * 64:(n + 1) * 64, :] for n in range(4)]
            if c >= MD:
                d = None
                for rb in range(NRB):
                    for v in range(RU // 8):
                        t_ = mhist[c - MD][rb][v * 8:(v + 1) * 8, :]
                        d = t_ if d is None else jnp.maximum(d, t_)
                r2 = rowsets[2]
                rowsets[2] = jnp.concatenate(
                    [jnp.concatenate([pin(r2[0:8, 0:128], pltpu.bitcast(d, U32)), r2[0:8, 128:]], axis=1), r2[8:]], axis=0)
            if LN0 <= c < LN0 + NRB:
                r1 = rowsets[1]
                rel = None
                if c >= 1 and LNL:
                    rel = jnp.concatenate([scs[c - 1][rsl(c - LN0), csl(LNL - 1)]] * 4, axis=1)
                rowsets[1] = jnp.concatenate([pin(r1[:RU // 2], tail(c - LN0, rel)), r1[RU // 2:]], axis=0)
            for n in (0, 3):
                if (c, n) in emap:
                    dn = 0 if n == 3 else 1
                    cells = [[rowsets[n][r * 8:(r + 1) * 8, csl(q_)] for q_ in range(4)] for r in range(8)]
                    for e_, (cb, j) in enumerate(emap[c, n]):
                        dep = scs[c - 1][(e_ % NV) * 8:(e_ % NV) * 8 + 8, csl(dn + 1 if n == 3 else dn)] if c >= 1 else None
                        cells[e_ % 8][e_ // 8] = pin(cells[e_ % 8][e_ // 8], pltpu.bitcast(conv(cb, j, dep), U32))
                    rowsets[n] = jnp.concatenate([jnp.concatenate(r_, axis=1) for r_ in cells], axis=0)
            kt = jnp.concatenate(rowsets, axis=0)
            sc = _dot_nt(q, kt)
            scs.append(sc)
            for rb in range(NRB):
                parts = [sc[rsl(rb), csl(j)] for j in range(4)]
                if c == NKC - 1:
                    lane = lax.broadcasted_iota(jnp.int32, (RU, 128), 1)
                    parts[3] = jnp.where(lane < T - (c * KC + 384), parts[3], -jnp.inf)
                mm = jnp.maximum(jnp.maximum(parts[0], parts[1]), jnp.maximum(parts[2], parts[3]))
                m[rb] = mm if m[rb] is None else jnp.maximum(m[rb], mm)
                for j in range(4):
                    sp[c, rb, j] = parts[j]
            mhist.append(list(m))
        if prev == "ff1":
            mid = store_qv(NTILE - 1, cat_rows(tail))
        else:
            mid = _dot(cat_rows(tail), wp1[...])
        mxb = [jnp.broadcast_to(jnp.max(m[rb], axis=-1, keepdims=True), (RU, 128)) for rb in range(NRB)]
        C0, RL = 2, 25
        nslots = (NKC - C0) * 4 * NV
        where = {C0 * 4 * NV + k * nslots // max(len(late), 1): u_ for k, u_ in enumerate(late)}
        acc, l128, pvs = {}, [None] * NRB, []
        for c in range(NKC):
            pbl = []
            for rb in range(NRB):
                mb = mxb[rb]
                if c == 1:
                    mb = pin(mb, mid[rsl(rb), D:D + 128])
                elif c >= 2:
                    mb = pin(mb, pvs[c - 1][rsl(rb), 0:128])
                pj = [jnp.exp2(sp[c, rb, j] - mb) for j in range(4)]
                lsum = (pj[0] + pj[1]) + (pj[2] + pj[3])
                l128[rb] = lsum if l128[rb] is None else l128[rb] + lsum
                pbl.append(pack(jnp.concatenate(pj, axis=1)))
            pv = _dot(jnp.concatenate(pbl, axis=0), vs[pl.ds(kb + c * (KC // 2), KC // 2), :])
            pvs.append(pv)
            for n in range(4):
                side = None
                if c == 1:
                    if prev == "ff1":
                        qs[_prows(NTILE - 1), csl(n)] = pack(mid[:, csl(n)])
                        vs[_pkrows(NTILE - 1), csl(n)] = pack(mid[:, D + n * 128:D + (n + 1) * 128])
                    else:
                        side = glu_block(i - 1, mid, n)
                for v in range(NV):
                    blk = pv[v * 8:(v + 1) * 8, csl(n)]
                    if c == 0:
                        acc[n, v] = blk
                        continue
                    a = acc[n, v]
                    if side is not None:
                        a = pin(a, side[v * 8:(v + 1) * 8, :])
                    slot = (c * 4 + n) * NV + v
                    if slot in where:
                        s0 = slot - RL
                        dep = pvs[s0 // (4 * NV)][(s0 % NV) * 8:(s0 % NV) * 8 + 8, csl((s0 // NV) % 4)]
                        a = pin(a, conv(*where[slot], dep))
                    if n == 2:
                        rb, vv = divmod(v, RU // 8)
                        a = pin(a, l128[rb][vv * 8:(vv + 1) * 8, :])
                    acc[n, v] = a + blk
        for n in range(4):
            for v in range(NV):
                accs[v * 8:(v + 1) * 8, csl(n)] = acc[n, v]
        for rb in range(NRB):
            ls[rsl(rb), :] = l128[rb]

    def bn_silu_unit(i, pin):
        def unit(rb, rel):
            z = pack(_silu((held(dcs[_rows(i, rb), :], rel, pin) - bn[0:1, :]) * bn[1:2, :]))
            zs[rb * (RU // 2):(rb + 1) * (RU // 2), :] = z
            return z
        return memo(unit)

    def c_step(i, do_prev, do_cur, do_next):
        pin = make_pin()
        if do_cur:
            y3 = _dot(zs[...], wp2[...])

            def x3u(rb, rel):
                x3 = held(xs[_rows(i, rb), :], rel, pin) + y3[rsl(rb), :]
                xs[_rows(i, rb), :] = x3
                return pack(_ln(x3))
            x3u = memo(x3u)
        if do_prev:
            r1 = []
            yacc = acc_matmul(us, w2b, pin, spread(5, 10, x3u, r1, 3) if do_cur else {}, r1)

            def out_unit(rb, rel):
                o = pack(_ln(held(xs[_rows(i - 1, rb), :], rel, pin) + 0.5 * yacc[rb]))
                qs[_prows(i - 1, rb), :] = o
                return o
            out_unit = memo(out_unit)
        if do_cur:
            dl, r2 = {}, []
            if do_prev:
                dl.update(spread(5, 10, out_unit, r2, 3))
            if do_next:
                dl.update(spread(6, 10, bn_silu_unit(jnp.minimum(i + 1, NTILE - 1), pin), r2, 5))
            ffa(cat_rows(x3u), w2a, pin, dl, r2)
        elif do_prev:
            cat_rows(out_unit)

    W1A, W1B, WQ, WK, WV, WO, WP1, WP2, W2A, W2B, DW = range(11)
    xcopy(0).start()
    w1a_copy(0).start()
    w1a_copy(1).start()
    wcopy(DW).start()
    for b in range(B):
        hs[(b * TP + T) // 2:(b + 1) * TP // 2, :] = jnp.zeros(((TP - T) // 2, D), U32)
        vs[(b * TP + T) // 2:(b + 1) * TP // 2, :] = jnp.zeros(((TP - T) // 2, D), U32)
        for cb in range(4):
            g0 = cb * GR + b * (T + 2 * HALO)
            gs[g0:g0 + HALO, :] = jnp.zeros((HALO, 128), F32)
            gs[g0 + HALO + T:g0 + T + 2 * HALO, :] = jnp.zeros((HALO, 128), F32)
    st[...] = jnp.zeros(st.shape, F32)
    wcopy(DW).wait()
    bn[2:3, :] = dw_ref[0:1, :].astype(F32)
    for kk in range(KW):
        for cb in range(4):
            dwt[(kk * 4 + cb) * 8:(kk * 4 + cb + 1) * 8, :] = jnp.broadcast_to(
                dw_ref[kk:kk + 1, csl(cb)].astype(F32), (8, 128))
    xcopy(0).wait()

    def first_a(c):
        w1a_copy(c).wait()
        nxt = (lambda: w1a_copy(2), lambda: w1a_copy(3), lambda: w1b_copy(0), lambda: w1b_copy(1))[c]
        nxt().start()
        if c == 1:
            xcopy(1).start()
    a_step(0, False, pre_a=first_a)

    def first_b(kg):
        w1b_copy(kg).wait()
        if kg < 2:
            w1b_copy(kg + 2).start()
        else:
            for k in ((WQ, WK), (WV, WO))[kg - 2]:
                wcopy(k).start()

    def rest(c):
        if c == 0:
            xcopy(2).start()
            xcopy(3).start()
        elif c == 1:
            for t in range(4, NTILE):
                xcopy(t).start()
            for k in (WP1, WP2, W2A, W2B):
                wcopy(k).start()

    def fold_weights():
        for k in (WQ, WK, WV, WO):
            wcopy(k).wait()
        mqv[:, :D] = pack(_dot_nt(wq[...], wk[...]) * (D ** -0.5 * LOG2E))
        mqv[:, D:] = pack(_dot(wv[...], wo[...]))
    xcopy(1).wait()
    a_step(1, True, pre_a=rest, pre_b=first_b, pre_qv=fold_weights)


    def a_body(j, c):
        xcopy(2 * j).wait()
        xcopy(2 * j + 1).wait()
        a_step(2 * j, True)
        a_step(2 * j + 1, True)
        return c
    lax.fori_loop(1, NTILE // 2, a_body, 0)

    for k in (WP1, WP2, W2A, W2B):
        wcopy(k).wait()
    b_step(0, "ff1", False)
    b_step(1, "attn", False)

    def b_body(i, c):
        b_step(i, "attn", True)
        return c
    lax.fori_loop(2, NTILE, b_body, 0)

    pin = make_pin()
    y2 = _dot(cat_rows(attn_tail_unit(NTILE - 1, pin)), wp1[...])
    for n in range(4):
        glu_block(NTILE - 1, y2, n)
    for t in (NTILE - 2, NTILE - 1):
        conv = conv_stream(t, pin)
        for cb in range(4):
            for j in range(NV):
                conv(cb, j, None)
    mean8, m28 = st[0], st[1]
    mu = jnp.mean(mean8, axis=0, keepdims=True)
    dm = mean8 - mu
    var = (jnp.sum(m28, axis=0, keepdims=True) + (B * T // 8) * jnp.sum(dm * dm, axis=0, keepdims=True)) * (1.0 / (B * T))
    bn[0:1, :] = mu
    bn[1:2, :] = lax.rsqrt(var + EPS)
    cat_rows(bn_silu_unit(0, pin))
    c_step(0, False, True, True)

    c_step(1, True, True, True)
    ocopy(0).start()

    def c_body(j, c):
        c_step(2 * j, True, True, True)
        c_step(2 * j + 1, True, True, True)
        ocopy(2 * j - 1).start()
        ocopy(2 * j).start()
        return c
    lax.fori_loop(1, NTILE // 2, c_body, 0)
    c_step(NTILE, True, False, False)
    ocopy(NTILE - 1).start()
    for t in range(NTILE):
        ocopy(t).wait()


@jax.jit
def pallas_standalone__conformer_family_conformer__speech_kernel(x, w_ff1_a, w_ff1_b, w_q, w_k, w_v, w_o, w_pw1, dw, w_pw2, w_ff2_a, w_ff2_b):
    xf = x.reshape(B * T, D)
    ws = (w_ff1_a, w_ff1_b, w_q, w_k, w_v, w_o, w_pw1, dw, w_pw2, w_ff2_a, w_ff2_b)
    packed = lambda w: pltpu.VMEM((w.shape[0] // 2, w.shape[1]), U32)
    hbm = pl.BlockSpec(memory_space=pl.ANY)
    out = pl.pallas_call(
        kernel,
        in_specs=[hbm] * 12,
        out_specs=hbm,
        out_shape=jax.ShapeDtypeStruct((B * T, D), x.dtype),
        scratch_shapes=[packed(w) for w in (w_ff1_a, w_ff1_b, w_q, w_k, w_v, w_o, w_pw1, w_pw2, w_ff2_a, w_ff2_b)] + [
            pltpu.VMEM((KW, D), BF),
            pltpu.VMEM((B * T, D), F32),
            pltpu.VMEM((B * TP // 2, D), U32),
            pltpu.VMEM((B * T // 2, D), U32),
            pltpu.VMEM((B * TP // 2, D), U32),
            pltpu.VMEM((4 * GR, 128), F32),
            pltpu.VMEM((B * T, D), F32),
            pltpu.VMEM((TM // 2, F), U32),
            pltpu.VMEM((TM, D), F32),
            pltpu.VMEM((TM, 128), F32),
            pltpu.VMEM((TM // 2, D), U32),
            pltpu.VMEM((D // 2, 2 * D), U32),
            pltpu.VMEM((KW * 4 * 8, 128), F32),
            pltpu.VMEM((2, 8, D), F32),
            pltpu.VMEM((8, D), F32),
            pltpu.SemaphoreType.DMA((11,)),
            pltpu.SemaphoreType.DMA((8,)),
            pltpu.SemaphoreType.DMA((NTILE,)),
            pltpu.SemaphoreType.DMA((1,)),
        ],
        compiler_params=pltpu.CompilerParams(vmem_limit_bytes=124 * 1024 * 1024),
    )(xf, *ws)
    return out.reshape(B, T, D)
```

```python
import jax
import jax.numpy as jnp
from jax import lax
from jax.experimental import pallas as pl
from jax.experimental.pallas import tpu as pltpu

B, T, D, F, KW = 2, 4000, 512, 2048, 15
TP = 4096
TM = 400
NT = T // TM
NTILE = B * NT
KC = 512
NKC = TP // KC
RU = 80
NRB = TM // RU
NV = TM // 8
EPS = 1e-5
LOG2E = 1.4426950408889634
BF = jnp.bfloat16
F32 = jnp.float32
U32 = jnp.uint32
HALO = 8
GR = B * (T + 2 * HALO)


def _ln(x):
    m = jnp.mean(x, axis=-1, keepdims=True)
    xc = x - m
    v = jnp.mean(xc * xc, axis=-1, keepdims=True)
    return xc * lax.rsqrt(v + EPS)


def pack(x):
    return pltpu.bitcast(x.astype(BF), U32)


def unpack(w):
    return pltpu.bitcast(w, BF)


def _dot(a32, b32):
    return jnp.dot(unpack(a32), unpack(b32), preferred_element_type=F32)


def _dot_nt(a32, b32):
    return lax.dot_general(unpack(a32), unpack(b32), (((1,), (1,)), ((), ())), preferred_element_type=F32)


def _sigmoid(x):
    return 0.5 * jnp.tanh(0.5 * x) + 0.5


def _silu(x):
    hx = 0.5 * x
    return hx * jnp.tanh(hx) + hx


def _mult(v, n):
    return v if isinstance(v, int) else pl.multiple_of(v, n)


def _rows(i, rb=None):
    if rb is None:
        return pl.ds(_mult(i * TM, 8), TM)
    return pl.ds(_mult(i * TM + rb * RU, 8), RU)


def _prows(i, rb=None):
    if rb is None:
        return pl.ds(_mult(i * (TM // 2), 8), TM // 2)
    return pl.ds(_mult(i * (TM // 2) + rb * (RU // 2), 8), RU // 2)


def _pkrows(i):
    return pl.ds(_mult((i // NT) * (TP // 2) + (i % NT) * (TM // 2), 8), TM // 2)


def _grow(i):
    return (i // NT) * (T + 2 * HALO) + (i % NT) * TM


def rsl(rb):
    return slice(rb * RU, (rb + 1) * RU)


def csl(n):
    return slice(n * 128, (n + 1) * 128)


def kernel(x_hbm, w1a_h, w1b_h, wq_h, wk_h, wv_h, wo_h, wp1_h, dw_h, wp2_h, w2a_h, w2b_h, o_hbm,
           w1a, w1b, wq, wk, wv, wo, wp1, wp2, w2a, w2b, dw_ref,
           xs, hs, qs, vs, gs, dcs, us, accs, ls, zs, mqv, dwt, st, bn,
           wsem, csem, xsem, osem):
    def wcopy(k):
        srcs = (w1a_h, w1b_h, wq_h, wk_h, wv_h, wo_h, wp1_h, wp2_h, w2a_h, w2b_h, dw_h)
        dsts = (w1a, w1b, wq, wk, wv, wo, wp1, wp2, w2a, w2b)
        dst = dw_ref if k == 10 else dsts[k].bitcast(BF)
        return pltpu.make_async_copy(srcs[k], dst, wsem.at[k])

    def w1a_copy(c):
        return pltpu.make_async_copy(w1a_h.at[:, c * 512:(c + 1) * 512], w1a.bitcast(BF).at[:, c * 512:(c + 1) * 512], csem.at[c])

    def w1b_copy(c):
        return pltpu.make_async_copy(w1b_h.at[c * 512:(c + 1) * 512, :], w1b.bitcast(BF).at[c * 512:(c + 1) * 512, :], csem.at[4 + c])

    def xcopy(i):
        rows = pl.ds(_mult(i * TM, 16), TM)
        return pltpu.make_async_copy(x_hbm.at[rows, :], qs.bitcast(BF).at[rows, :], xsem.at[i])

    def ocopy(i):
        rows = pl.ds(_mult(i * TM, 16), TM)
        return pltpu.make_async_copy(qs.bitcast(BF).at[rows, :], o_hbm.at[rows, :], osem.at[0])

    def make_pin():
        nv = jnp.abs(bn[2:3, :])

        def pin(val, dep):
            never = jnp.broadcast_to(nv[:, :val.shape[1]], val.shape) < 0.0
            return jnp.where(never, dep, val)
        return pin

    def memo(fn):
        cache = {}

        def get(rb, rel=None):
            if rb not in cache:
                cache[rb] = fn(rb, rel)
            return cache[rb]
        return get

    def cat_rows(get):
        return jnp.concatenate([get(rb) for rb in range(NRB)], axis=0)

    def pin_rhs(w32, pin, tokens):
        if not tokens:
            return w32
        cols = []
        for n in range(4):
            col = w32[:, csl(n)]
            if n in tokens:
                tk = tokens[n]()
                k = tk.shape[0]
                col = jnp.concatenate([pin(col[:k], tk), col[k:]], axis=0)
            cols.append(col)
        return jnp.concatenate(cols, axis=1)

    def spread(first, count, unit, res, lead):
        out = {}
        for rb in range(NRB):
            p = first + rb * count // NRB
            pr = min(p - lead, 4 * (p // 4) - 1)

            def token(rb=rb, pr=pr):
                rel = None
                if pr >= 0 and lead < 90:
                    rel = jnp.concatenate([res[pr // 4][rsl(rb), csl(pr % 4)]] * 4, axis=1)
                u_ = unit(rb, rel)
                return jnp.concatenate([u_[:, csl(n)] for n in range(4)], axis=0)
            assert (p // 4, p % 4) not in out
            out[p // 4, p % 4] = token
        return out

    def tok(deadlines, c):
        return {n: f for (cc, n), f in deadlines.items() if cc == c}

    def acc_matmul(lhs, w, pin, deadlines, res, pre=None):
        acc = None
        for kg in range(4):
            if pre:
                pre(kg)
            part = _dot(lhs[:, kg * 512:(kg + 1) * 512], pin_rhs(w[kg * 256:(kg + 1) * 256, :], pin, tok(deadlines, kg)))
            res.append(part)
            if acc is None:
                acc = [part[rsl(rb), :] for rb in range(NRB)]
            else:
                acc = [acc[rb] + part[rsl(rb), :] for rb in range(NRB)]
        return acc

    def ffa(h32, wa, pin, deadlines, res, pre=None):
        for c in range(F // 512):
            if pre:
                pre(c)
            u = _dot(h32, pin_rhs(wa[:, c * 512:(c + 1) * 512], pin, tok(deadlines, c)))
            res.append(u)
            us[:, c * 512:(c + 1) * 512] = pack(_silu(u))

    def held(val, rel, pin):
        if rel is None:
            return val
        if val.dtype == U32:
            return pin(val, pltpu.bitcast(rel[:val.shape[0]], U32))
        return pin(val, rel)

    def ff1_tail_unit(i, yacc, pin):
        def unit(rb, rel):
            x1 = unpack(held(qs[_prows(i, rb), :], rel, pin)).astype(F32) + 0.5 * yacc[rb]
            xs[_rows(i, rb), :] = x1
            return pack(_ln(x1))
        return memo(unit)

    def store_qv(i, h1):
        hs[_pkrows(i), :] = h1
        return _dot(h1, mqv[...])

    def a_step(i, do_prev, pre_a=None, pre_b=None, pre_qv=None):
        pin = make_pin()
        lnx = memo(lambda rb, rel: pack(_ln(unpack(held(qs[_prows(i, rb), :], rel, pin)).astype(F32))))
        dl, r1, r2 = {}, [], []
        if do_prev:
            yacc = acc_matmul(us, w1b, pin, spread(4, 10, lnx, r1, 3), r1, pre_b)
            tail = ff1_tail_unit(i - 1, yacc, pin)
            dl = spread(5, 10, tail, r2, 3)
        ffa(cat_rows(lnx), w1a, pin, dl, r2, pre_a)
        if do_prev:
            if pre_qv:
                pre_qv()
            qv = store_qv(i - 1, cat_rows(tail))
            qs[_prows(i - 1), :] = pack(qv[:, :D])
            vs[_pkrows(i - 1), :] = pack(qv[:, D:])

    def conv_stream(n_old, pin):
        cs = [dict(cnt=0) for _ in range(4)]
        sub = lax.broadcasted_iota(jnp.int32, (8, 128), 0)

        def rot(v):
            return [v] + [pltpu.roll(v, 8 - s_, 0) for s_ in range(1, 8)]

        def shift(ra, rb_):
            return [ra[0]] + [jnp.where(sub < 8 - s_, ra[s_], rb_[s_]) for s_ in range(1, 8)]

        def step(cb, t, j, dep, key, valid=None):
            c_ = cs[cb]
            g0 = _grow(t)
            rel = (lambda v: v) if dep is None else (lambda v: pin(v, dep))
            ld = lambda jj: rel(gs[pl.ds(_mult(g0 + cb * GR + 8 * jj, 8), 8), :])
            if c_.get("next") != (key, j):
                ra, rb_ = rot(ld(j)), rot(ld(j + 1))
                c_["G"], c_["R"] = shift(ra, rb_), rb_
            if "w" not in c_:
                c_["w"] = [dwt[(kk * 4 + cb) * 8:(kk * 4 + cb + 1) * 8, :] for kk in range(KW)]
            rn = rot(ld(j + 2))
            gn = shift(c_["R"], rn)
            terms = [c_["G"][s_] * c_["w"][s_ - 1] for s_ in range(1, 8)] + [gn[s_] * c_["w"][7 + s_] for s_ in range(8)]
            c_["G"], c_["R"], c_["next"] = gn, rn, (key, j + 1)
            while len(terms) > 1:
                terms = [terms[q] + terms[q + 1] for q in range(0, len(terms) - 1, 2)] + ([terms[-1]] if len(terms) % 2 else [])
            o = terms[0]
            dcs[pl.ds(_mult(t * TM + 8 * j, 8), 8), csl(cb)] = o
            if c_["cnt"] == 0:
                c_["c"] = o
            else:
                d = o - c_["c"]
                if valid is not None:
                    d = jnp.where(valid, d, 0.0)
                c_["s1"] = d if c_["cnt"] == 1 else c_["s1"] + d
                c_["s2"] = d * d if c_["cnt"] == 1 else c_["s2"] + d * d
            c_["cnt"] += 1
            return o

        def flush(cb, valid=None):
            c_ = cs[cb]
            k = jnp.full((8, 128), c_["cnt"], F32)
            if valid is not None:
                k = jnp.where(valid, k, k - 1.0)
            cols = csl(cb)
            rk = 1.0 / k
            tmean = c_["c"] + c_["s1"] * rk
            tm2 = c_["s2"] - c_["s1"] * c_["s1"] * rk
            n = jnp.zeros((8, 128), F32) + jnp.asarray(n_old, F32)
            f = k / (n + k)
            mean_old = st[0, :, cols]
            delta = tmean - mean_old
            st[0, :, cols] = mean_old + delta * f
            st[1, :, cols] = st[1, :, cols] + tm2 + delta * delta * (n * f)
            c_["cnt"] = 0
        return step, flush

    def attn_tail_unit(i, pin):
        def unit(rb, rel):
            lsum = ls[rsl(rb), :]
            if rel is not None:
                lsum = pin(lsum, rel[:, 0:128])
            inv = 1.0 / jnp.sum(lsum, axis=-1, keepdims=True)
            x2 = held(xs[_rows(i, rb), :], rel, pin) + accs[rsl(rb), :] * inv
            xs[_rows(i, rb), :] = x2
            return pack(_ln(x2))
        return memo(unit)

    def glu_block(i, y2, n):
        g = y2[:, csl(n)] * _sigmoid(y2[:, D + n * 128:D + (n + 1) * 128])
        gs[pl.ds(_mult(_grow(i) + (n * GR + HALO), 8), TM), :] = g
        return g

    def b_step(i, prev, conv_mode):
        pin = make_pin()
        kb = _mult((i // NT) * (TP // 2), TP // 2)
        if prev == "ff1":
            tail = ff1_tail_unit(NTILE - 1, acc_matmul(us, w1b, pin, {}, []), pin)
        else:
            tail = attn_tail_unit(i - 1, pin)
        q = qs[_prows(i), :]
        m = [None] * NRB
        mhist = []
        sp = {}
        MD, LN0, LNL = 2, 2, 0
        scs = []
        late = []
        if conv_mode:
            has_old = i >= 2
            conv, flush = conv_stream(jnp.where(has_old, (NV - 1) + NV * (i - 2), 0), pin)
            for cb in range(4):
                late += [(cb, i - 1, j, 1) for j in range(NV - 1)]
                late.append((cb, jnp.maximum(i - 2, 0), NV - 1, 0))
        for c in range(NKC):
            kt = hs[pl.ds(kb + c * (KC // 2), KC // 2), :]
            rowsets = [kt[n * 64:(n + 1) * 64, :] for n in range(4)]
            if c >= MD:
                d = None
                for rb in range(NRB):
                    for v in range(RU // 8):
                        t_ = mhist[c - MD][rb][v * 8:(v + 1) * 8, :]
                        d = t_ if d is None else jnp.maximum(d, t_)
                r2 = rowsets[2]
                rowsets[2] = jnp.concatenate(
                    [jnp.concatenate([pin(r2[0:8, 0:128], pltpu.bitcast(d, U32)), r2[0:8, 128:]], axis=1), r2[8:]], axis=0)
            if LN0 <= c < LN0 + NRB:
                r1 = rowsets[1]
                rel = None
                if c >= 1 and LNL:
                    rel = jnp.concatenate([scs[c - 1][rsl(c - LN0), csl(LNL - 1)]] * 4, axis=1)
                rowsets[1] = jnp.concatenate([pin(r1[:RU // 2], tail(c - LN0, rel)), r1[RU // 2:]], axis=0)
            kt = jnp.concatenate(rowsets, axis=0)
            sc = _dot_nt(q, kt)
            scs.append(sc)
            for rb in range(NRB):
                parts = [sc[rsl(rb), csl(j)] for j in range(4)]
                if c == NKC - 1:
                    lane = lax.broadcasted_iota(jnp.int32, (RU, 128), 1)
                    parts[3] = jnp.where(lane < T - (c * KC + 384), parts[3], -jnp.inf)
                mm = jnp.maximum(jnp.maximum(parts[0], parts[1]), jnp.maximum(parts[2], parts[3]))
                m[rb] = mm if m[rb] is None else jnp.maximum(m[rb], mm)
                for j in range(4):
                    sp[c, rb, j] = parts[j]
            mhist.append(list(m))
        if prev == "ff1":
            mid = store_qv(NTILE - 1, cat_rows(tail))
        else:
            mid = _dot(cat_rows(tail), wp1[...])
        mxb = [jnp.broadcast_to(jnp.max(m[rb], axis=-1, keepdims=True), (RU, 128)) for rb in range(NRB)]
        C0, RL = 2, 25
        nslots = (NKC - C0) * 4 * NV
        where = {C0 * 4 * NV + k * nslots // max(len(late), 1): u_ for k, u_ in enumerate(late)}
        acc, l128, pvs = {}, [None] * NRB, []
        for c in range(NKC):
            pbl = []
            for rb in range(NRB):
                mb = mxb[rb]
                if c == 1:
                    mb = pin(mb, mid[rsl(rb), D:D + 128])
                elif c >= 2:
                    mb = pin(mb, pvs[c - 1][rsl(rb), 0:128])
                pj = [jnp.exp2(sp[c, rb, j] - mb) for j in range(4)]
                lsum = (pj[0] + pj[1]) + (pj[2] + pj[3])
                l128[rb] = lsum if l128[rb] is None else l128[rb] + lsum
                pbl.append(pack(jnp.concatenate(pj, axis=1)))
            pv = _dot(jnp.concatenate(pbl, axis=0), vs[pl.ds(kb + c * (KC // 2), KC // 2), :])
            pvs.append(pv)
            for n in range(4):
                side = None
                if c == 1:
                    if prev == "ff1":
                        qs[_prows(NTILE - 1), csl(n)] = pack(mid[:, csl(n)])
                        vs[_pkrows(NTILE - 1), csl(n)] = pack(mid[:, D + n * 128:D + (n + 1) * 128])
                    else:
                        side = glu_block(i - 1, mid, n)
                for v in range(NV):
                    blk = pv[v * 8:(v + 1) * 8, csl(n)]
                    if c == 0:
                        acc[n, v] = blk
                        continue
                    a = acc[n, v]
                    if side is not None:
                        a = pin(a, side[v * 8:(v + 1) * 8, :])
                    slot = (c * 4 + n) * NV + v
                    if slot in where:
                        s0 = slot - RL
                        dep = pvs[s0 // (4 * NV)][(s0 % NV) * 8:(s0 % NV) * 8 + 8, csl((s0 // NV) % 4)]
                        cb_, t_, j_, key_ = where[slot]
                        a = pin(a, conv(cb_, t_, j_, dep, key_, has_old if key_ == 0 else None))
                        if key_ == 0:
                            flush(cb_, has_old)
                    if n == 2:
                        rb, vv = divmod(v, RU // 8)
                        a = pin(a, l128[rb][vv * 8:(vv + 1) * 8, :])
                    acc[n, v] = a + blk
        for n in range(4):
            for v in range(NV):
                accs[v * 8:(v + 1) * 8, csl(n)] = acc[n, v]
        for rb in range(NRB):
            ls[rsl(rb), :] = l128[rb]

    def bn_silu_unit(i, pin):
        def unit(rb, rel):
            z = pack(_silu((held(dcs[_rows(i, rb), :], rel, pin) - bn[0:1, :]) * bn[1:2, :]))
            zs[rb * (RU // 2):(rb + 1) * (RU // 2), :] = z
            return z
        return memo(unit)

    def c_step(i, do_prev, do_cur, do_next):
        pin = make_pin()
        if do_cur:
            y3 = _dot(zs[...], wp2[...])

            def x3u(rb, rel):
                x3 = held(xs[_rows(i, rb), :], rel, pin) + y3[rsl(rb), :]
                xs[_rows(i, rb), :] = x3
                return pack(_ln(x3))
            x3u = memo(x3u)
        if do_prev:
            r1 = []
            yacc = acc_matmul(us, w2b, pin, spread(5, 10, x3u, r1, 3) if do_cur else {}, r1)

            def out_unit(rb, rel):
                o = pack(_ln(held(xs[_rows(i - 1, rb), :], rel, pin) + 0.5 * yacc[rb]))
                qs[_prows(i - 1, rb), :] = o
                return o
            out_unit = memo(out_unit)
        if do_cur:
            dl, r2 = {}, []
            if do_prev:
                dl.update(spread(5, 10, out_unit, r2, 3))
            if do_next:
                dl.update(spread(6, 10, bn_silu_unit(i + 1, pin), r2, 5))
            ffa(cat_rows(x3u), w2a, pin, dl, r2)
        elif do_prev:
            cat_rows(out_unit)

    W1A, W1B, WQ, WK, WV, WO, WP1, WP2, W2A, W2B, DW = range(11)
    xcopy(0).start()
    w1a_copy(0).start()
    for b in range(B):
        hs[(b * TP + T) // 2:(b + 1) * TP // 2, :] = jnp.zeros(((TP - T) // 2, D), U32)
        vs[(b * TP + T) // 2:(b + 1) * TP // 2, :] = jnp.zeros(((TP - T) // 2, D), U32)
        for cb in range(4):
            g0 = cb * GR + b * (T + 2 * HALO)
            gs[g0:g0 + HALO, :] = jnp.zeros((HALO, 128), F32)
            gs[g0 + HALO + T:g0 + T + 2 * HALO, :] = jnp.zeros((HALO, 128), F32)
    for cb in range(4):
        gs[cb * GR + HALO + TM:cb * GR + HALO + TM + 16, :] = jnp.zeros((16, 128), F32)
    st[...] = jnp.zeros(st.shape, F32)
    bn[...] = jnp.zeros(bn.shape, F32)
    xcopy(0).wait()
    w1a_copy(1).start()

    def first_a(c):
        w1a_copy(c).wait()
        nxt = (lambda: w1a_copy(2), lambda: w1a_copy(3), lambda: w1b_copy(0), lambda: w1b_copy(1))[c]
        nxt().start()
        if c == 1:
            xcopy(1).start()
            wcopy(DW).start()
    a_step(0, False, pre_a=first_a)
    wcopy(DW).wait()
    bn[2:3, :] = dw_ref[0:1, :].astype(F32)
    for kk in range(KW):
        for cb in range(4):
            dwt[(kk * 4 + cb) * 8:(kk * 4 + cb + 1) * 8, :] = jnp.broadcast_to(
                dw_ref[kk:kk + 1, csl(cb)].astype(F32), (8, 128))

    def first_b(kg):
        w1b_copy(kg).wait()
        if kg < 2:
            w1b_copy(kg + 2).start()
        else:
            for k in ((WQ, WK), (WV, WO))[kg - 2]:
                wcopy(k).start()

    def rest(c):
        if c == 0:
            xcopy(2).start()
            xcopy(3).start()
        elif c == 1:
            for t in range(4, NTILE):
                xcopy(t).start()
            for k in (WP1, WP2, W2A, W2B):
                wcopy(k).start()

    def fold_weights():
        for k in (WQ, WK, WV, WO):
            wcopy(k).wait()
        mqv[:, :D] = pack(_dot_nt(wq[...], wk[...]) * (D ** -0.5 * LOG2E))
        mqv[:, D:] = pack(_dot(wv[...], wo[...]))
    xcopy(1).wait()
    a_step(1, True, pre_a=rest, pre_b=first_b, pre_qv=fold_weights)


    def a_body(j, c):
        xcopy(2 * j).wait()
        xcopy(2 * j + 1).wait()
        a_step(2 * j, True)
        a_step(2 * j + 1, True)
        return c
    lax.fori_loop(1, NTILE // 2 - 1, a_body, 0)
    if 1:
        a_body(NTILE // 2 - 1, 0)

    for k in (WP1, WP2, W2A, W2B):
        wcopy(k).wait()
    b_step(0, "ff1", 0)

    def b_body(i, c):
        b_step(i, "attn", 2)
        return c
    lax.fori_loop(1, NTILE, b_body, 0)

    pin = make_pin()
    h2 = cat_rows(attn_tail_unit(NTILE - 1, pin))
    conv, flush = conv_stream((NV - 1) + NV * (NTILE - 2), pin)
    for n in range(4):
        wab = jnp.concatenate([wp1[:, csl(n)], wp1[:, D + n * 128:D + (n + 1) * 128]], axis=1)
        yab = _dot(h2, wab)
        gs[pl.ds(_grow(NTILE - 1) + n * GR + HALO, TM), :] = yab[:, :128] * _sigmoid(yab[:, 128:])
        conv(n, NTILE - 2, NV - 1, None, 0)
        for j in range(NV):
            conv(n, NTILE - 1, j, None, 1)
        flush(n)
    mean8, m28 = st[0], st[1]
    mu = jnp.mean(mean8, axis=0, keepdims=True)
    dm = mean8 - mu
    var = (jnp.sum(m28, axis=0, keepdims=True) + (B * T // 8) * jnp.sum(dm * dm, axis=0, keepdims=True)) * (1.0 / (B * T))
    bn[0:1, :] = mu
    bn[1:2, :] = lax.rsqrt(var + EPS)
    cat_rows(bn_silu_unit(0, pin))
    c_step(0, False, True, True)


    def c_body(j, c):
        c_step(2 * j - 1, True, True, True)
        c_step(2 * j, True, True, True)
        ocopy(2 * j - 2).start()
        ocopy(2 * j - 1).start()
        return c
    lax.fori_loop(1, NTILE // 2, c_body, 0)
    c_step(NTILE - 1, True, True, False)
    ocopy(NTILE - 2).start()
    c_step(NTILE, True, False, False)
    ocopy(NTILE - 1).start()
    for t in range(NTILE):
        ocopy(t).wait()


@jax.jit
def pallas_standalone__conformer_family_conformer__speech_kernel(x, w_ff1_a, w_ff1_b, w_q, w_k, w_v, w_o, w_pw1, dw, w_pw2, w_ff2_a, w_ff2_b):
    xf = x.reshape(B * T, D)
    ws = (w_ff1_a, w_ff1_b, w_q, w_k, w_v, w_o, w_pw1, dw, w_pw2, w_ff2_a, w_ff2_b)
    packed = lambda w: pltpu.VMEM((w.shape[0] // 2, w.shape[1]), U32)
    hbm = pl.BlockSpec(memory_space=pl.ANY)
    out = pl.pallas_call(
        kernel,
        in_specs=[hbm] * 12,
        out_specs=hbm,
        out_shape=jax.ShapeDtypeStruct((B * T, D), x.dtype),
        scratch_shapes=[packed(w) for w in (w_ff1_a, w_ff1_b, w_q, w_k, w_v, w_o, w_pw1, w_pw2, w_ff2_a, w_ff2_b)] + [
            pltpu.VMEM((KW, D), BF),
            pltpu.VMEM((B * T, D), F32),
            pltpu.VMEM((B * TP // 2, D), U32),
            pltpu.VMEM((B * T // 2, D), U32),
            pltpu.VMEM((B * TP // 2, D), U32),
            pltpu.VMEM((4 * GR, 128), F32),
            pltpu.VMEM((B * T, D), F32),
            pltpu.VMEM((TM // 2, F), U32),
            pltpu.VMEM((TM, D), F32),
            pltpu.VMEM((TM, 128), F32),
            pltpu.VMEM((TM // 2, D), U32),
            pltpu.VMEM((D // 2, 2 * D), U32),
            pltpu.VMEM((KW * 4 * 8, 128), F32),
            pltpu.VMEM((2, 8, D), F32),
            pltpu.VMEM((8, D), F32),
            pltpu.SemaphoreType.DMA((11,)),
            pltpu.SemaphoreType.DMA((8,)),
            pltpu.SemaphoreType.DMA((NTILE,)),
            pltpu.SemaphoreType.DMA((1,)),
        ],
        compiler_params=pltpu.CompilerParams(vmem_limit_bytes=124 * 1024 * 1024),
    )(xf, *ws)
    return out.reshape(B, T, D)
```

```python
import jax
import jax.numpy as jnp
from jax import lax
from jax.experimental import pallas as pl
from jax.experimental.pallas import tpu as pltpu

B, T, D, F, KW = 2, 4000, 512, 2048, 15
TP = 4096
TM = 400
NT = T // TM
NTILE = B * NT
KC = 512
NKC = TP // KC
RU = 80
NRB = TM // RU
NV = TM // 8
EPS = 1e-5
LOG2E = 1.4426950408889634
BF = jnp.bfloat16
F32 = jnp.float32
U32 = jnp.uint32
HALO = 8
GR = B * (T + 2 * HALO)


def _ln(x):
    m = jnp.mean(x, axis=-1, keepdims=True)
    xc = x - m
    v = jnp.mean(xc * xc, axis=-1, keepdims=True)
    return xc * lax.rsqrt(v + EPS)


def pack(x):
    return pltpu.bitcast(x.astype(BF), U32)


def unpack(w):
    return pltpu.bitcast(w, BF)


def _dot(a32, b32):
    return jnp.dot(unpack(a32), unpack(b32), preferred_element_type=F32)


def _dot_nt(a32, b32):
    return lax.dot_general(unpack(a32), unpack(b32), (((1,), (1,)), ((), ())), preferred_element_type=F32)


def _sigmoid(x):
    return 0.5 * jnp.tanh(0.5 * x) + 0.5


def _silu(x):
    hx = 0.5 * x
    return hx * jnp.tanh(hx) + hx


def _mult(v, n):
    return v if isinstance(v, int) else pl.multiple_of(v, n)


def _rows(i, rb=None):
    if rb is None:
        return pl.ds(_mult(i * TM, 8), TM)
    return pl.ds(_mult(i * TM + rb * RU, 8), RU)


def _prows(i, rb=None):
    if rb is None:
        return pl.ds(_mult(i * (TM // 2), 8), TM // 2)
    return pl.ds(_mult(i * (TM // 2) + rb * (RU // 2), 8), RU // 2)


def _pk0(i):
    return (i // NT) * (TP // 2) + (i % NT) * (TM // 2)


def _pkrows(i):
    return pl.ds(_mult(_pk0(i), 8), TM // 2)


def _grow(i):
    return (i // NT) * (T + 2 * HALO) + (i % NT) * TM


def rsl(rb):
    return slice(rb * RU, (rb + 1) * RU)


def csl(n):
    return slice(n * 128, (n + 1) * 128)


def kernel(x_hbm, w1a_h, w1b_h, wq_h, wk_h, wv_h, wo_h, wp1_h, dw_h, wp2_h, w2a_h, w2b_h, o_hbm,
           w1a, w1b, wq, wk, wv, wo, wp1, wp2, w2a, w2b, dw_ref,
           xs, hs, qs, vs, gs, dcs, us, hb, accs, ls, zs, mqv, dwt, st, bn,
           wsem, csem, xsem, osem):
    def wcopy(k):
        srcs = (w1a_h, w1b_h, wq_h, wk_h, wv_h, wo_h, wp1_h, wp2_h, w2a_h, w2b_h, dw_h)
        dsts = (w1a, w1b, wq, wk, wv, wo, wp1, wp2, w2a, w2b)
        dst = dw_ref if k == 10 else dsts[k].bitcast(BF)
        return pltpu.make_async_copy(srcs[k], dst, wsem.at[k])

    def w1a_copy(c):
        return pltpu.make_async_copy(w1a_h.at[:, c * 512:(c + 1) * 512], w1a.bitcast(BF).at[:, c * 512:(c + 1) * 512], csem.at[c])

    def w1b_copy(c):
        return pltpu.make_async_copy(w1b_h.at[c * 512:(c + 1) * 512, :], w1b.bitcast(BF).at[c * 512:(c + 1) * 512, :], csem.at[4 + c])

    def xcopy(i):
        rows = pl.ds(_mult(i * TM, 16), TM)
        return pltpu.make_async_copy(x_hbm.at[rows, :], qs.bitcast(BF).at[rows, :], xsem.at[i])

    def ocopy(i):
        rows = pl.ds(_mult(i * TM, 16), TM)
        return pltpu.make_async_copy(qs.bitcast(BF).at[rows, :], o_hbm.at[rows, :], osem.at[0])

    def make_pin():
        nv = jnp.abs(bn[2:3, :])

        def pin(val, dep):
            never = jnp.broadcast_to(nv[:, :val.shape[1]], val.shape) < 0.0
            return jnp.where(never, dep, val)
        return pin

    def memo(fn):
        cache = {}

        def get(rb, rel=None):
            if rb not in cache:
                cache[rb] = fn(rb, rel)
            return cache[rb]
        return get

    def stash(rb, h32):
        hb[rb * (RU // 2):(rb + 1) * (RU // 2), :] = h32
        return hb[rb * (RU // 2):(rb + 1) * (RU // 2), :]

    def all_units(get):
        for rb in range(NRB):
            get(rb)

    def pin_rhs(w32, pin, tokens):
        if not tokens:
            return w32
        cols = []
        for n in range(4):
            col = w32[:, csl(n)]
            if n in tokens:
                tk = tokens[n]()
                k = tk.shape[0]
                col = jnp.concatenate([pin(col[:k], tk), col[k:]], axis=0)
            cols.append(col)
        return jnp.concatenate(cols, axis=1)

    def spread(first, count, unit, res, lead):
        out = {}
        for rb in range(NRB):
            p = first + rb * count // NRB
            pr = min(p - lead, 4 * (p // 4) - 1)

            def token(rb=rb, pr=pr):
                rel = None
                if pr >= 0 and lead < 90:
                    rel = jnp.concatenate([res[pr // 4][rsl(rb), csl(pr % 4)]] * 4, axis=1)
                u_ = unit(rb, rel)
                return jnp.concatenate([u_[:, csl(n)] for n in range(4)], axis=0)
            assert p < 16 and (p // 4, p % 4) not in out
            out[p // 4, p % 4] = token
        return out

    def tok(deadlines, c):
        return {n: f for (cc, n), f in deadlines.items() if cc == c}

    def acc_matmul(lhs, w, pin, deadlines, res, pre=None):
        acc = None
        for kg in range(4):
            if pre:
                pre(kg)
            part = _dot(lhs[:, kg * 512:(kg + 1) * 512], pin_rhs(w[kg * 256:(kg + 1) * 256, :], pin, tok(deadlines, kg)))
            res.append(part)
            if acc is None:
                acc = [part[rsl(rb), :] for rb in range(NRB)]
            else:
                acc = [acc[rb] + part[rsl(rb), :] for rb in range(NRB)]
        return acc

    def ffa(h32, wa, pin, deadlines, res, pre=None):
        for c in range(F // 512):
            if pre:
                pre(c)
            u = _dot(h32, pin_rhs(wa[:, c * 512:(c + 1) * 512], pin, tok(deadlines, c)))
            res.append(u)
            us[:, c * 512:(c + 1) * 512] = pack(_silu(u))

    def held(val, rel, pin):
        if rel is None:
            return val
        if val.dtype == U32:
            return pin(val, pltpu.bitcast(rel[:val.shape[0]], U32))
        return pin(val, rel)

    def ff1_tail_unit(i, yacc, pin):
        def unit(rb, rel):
            x1 = unpack(held(qs[_prows(i, rb), :], rel, pin)).astype(F32) + 0.5 * yacc[rb]
            xs[_rows(i, rb), :] = x1
            h1 = pack(_ln(x1))
            rows = pl.ds(_mult(_pk0(i) + rb * (RU // 2), 8), RU // 2)
            hs[rows, :] = h1
            return hs[rows, :]
        return memo(unit)

    def qv_matmul(i):
        return _dot(hs[_pkrows(i), :], mqv[...])

    def a_step(i, do_prev, pre_a=None, pre_b=None, pre_qv=None):
        pin = make_pin()
        lnx = memo(lambda rb, rel: stash(rb, pack(_ln(unpack(held(qs[_prows(i, rb), :], rel, pin)).astype(F32)))))
        dl, r1, r2 = {}, [], []
        if do_prev:
            yacc = acc_matmul(us, w1b, pin, spread(4, 10, lnx, r1, 3), r1, pre_b)
            tail = ff1_tail_unit(i - 1, yacc, pin)
            dl = spread(2, 10, tail, r2, 4)
        all_units(lnx)
        ffa(hb[...], w1a, pin, dl, r2, pre_a)
        if do_prev:
            if pre_qv:
                pre_qv()
            all_units(tail)
            qv = qv_matmul(i - 1)
            qs[_prows(i - 1), :] = pack(qv[:, :D])
            vs[_pkrows(i - 1), :] = pack(qv[:, D:])

    def conv_stream(n_old, pin):
        cs = [dict(cnt=0) for _ in range(4)]
        sub = lax.broadcasted_iota(jnp.int32, (8, 128), 0)

        def rot(v):
            return [v] + [pltpu.roll(v, 8 - s_, 0) for s_ in range(1, 8)]

        def shift(ra, rb_):
            return [ra[0]] + [jnp.where(sub < 8 - s_, ra[s_], rb_[s_]) for s_ in range(1, 8)]

        def step(cb, t, j, dep, key, valid=None):
            c_ = cs[cb]
            g0 = _grow(t)
            rel = (lambda v: v) if dep is None else (lambda v: pin(v, dep))
            ld = lambda jj: rel(gs[pl.ds(_mult(g0 + cb * GR + 8 * jj, 8), 8), :])
            if c_.get("next") != (key, j):
                ra, rb_ = rot(ld(j)), rot(ld(j + 1))
                c_["G"], c_["R"] = shift(ra, rb_), rb_
            if "w" not in c_:
                c_["w"] = [dwt[(kk * 4 + cb) * 8:(kk * 4 + cb + 1) * 8, :] for kk in range(KW)]
            rn = rot(ld(j + 2))
            gn = shift(c_["R"], rn)
            terms = [c_["G"][s_] * c_["w"][s_ - 1] for s_ in range(1, 8)] + [gn[s_] * c_["w"][7 + s_] for s_ in range(8)]
            c_["G"], c_["R"], c_["next"] = gn, rn, (key, j + 1)
            while len(terms) > 1:
                terms = [terms[q] + terms[q + 1] for q in range(0, len(terms) - 1, 2)] + ([terms[-1]] if len(terms) % 2 else [])
            o = terms[0]
            dcs[pl.ds(_mult(t * TM + 8 * j, 8), 8), csl(cb)] = o
            if c_["cnt"] == 0:
                c_["c"] = o
            else:
                d = o - c_["c"]
                if valid is not None:
                    d = jnp.where(valid, d, 0.0)
                c_["s1"] = d if c_["cnt"] == 1 else c_["s1"] + d
                c_["s2"] = d * d if c_["cnt"] == 1 else c_["s2"] + d * d
            c_["cnt"] += 1
            return o

        def flush(cb, valid=None):
            c_ = cs[cb]
            k = jnp.full((8, 128), c_["cnt"], F32)
            if valid is not None:
                k = jnp.where(valid, k, k - 1.0)
            cols = csl(cb)
            rk = 1.0 / k
            tmean = c_["c"] + c_["s1"] * rk
            tm2 = c_["s2"] - c_["s1"] * c_["s1"] * rk
            n = jnp.zeros((8, 128), F32) + jnp.asarray(n_old, F32)
            f = k / (n + k)
            mean_old = st[0, :, cols]
            delta = tmean - mean_old
            st[0, :, cols] = mean_old + delta * f
            st[1, :, cols] = st[1, :, cols] + tm2 + delta * delta * (n * f)
            c_["cnt"] = 0
        return step, flush

    def attn_tail_unit(i, pin):
        def unit(rb, rel):
            lsum = ls[rsl(rb), :]
            if rel is not None:
                lsum = pin(lsum, rel[:, 0:128])
            inv = 1.0 / jnp.sum(lsum, axis=-1, keepdims=True)
            x2 = held(xs[_rows(i, rb), :], rel, pin) + accs[rsl(rb), :] * inv
            xs[_rows(i, rb), :] = x2
            return stash(rb, pack(_ln(x2)))
        return memo(unit)

    def glu_block(i, y2, n):
        g = y2[:, csl(n)] * _sigmoid(y2[:, D + n * 128:D + (n + 1) * 128])
        gs[pl.ds(_mult(_grow(i) + (n * GR + HALO), 8), TM), :] = g
        return g

    def b_step(i, prev, conv_mode):
        pin = make_pin()
        kb = _mult((i // NT) * (TP // 2), TP // 2)
        if prev == "ff1":
            tail = ff1_tail_unit(NTILE - 1, acc_matmul(us, w1b, pin, {}, []), pin)
        else:
            tail = attn_tail_unit(i - 1, pin)
        q = qs[_prows(i), :]
        m = [None] * NRB
        mhist = []
        sp = {}
        MD, LN0, LNL = 2, 3, 0
        scs = []
        late = []
        if conv_mode:
            has_old = i >= 2
            conv, flush = conv_stream(jnp.where(has_old, (NV - 1) + NV * (i - 2), 0), pin)
            for cb in range(4):
                late += [(cb, i - 1, j, 1) for j in range(NV - 1)]
                late.append((cb, jnp.maximum(i - 2, 0), NV - 1, 0))
        for c in range(NKC):
            kt = hs[pl.ds(kb + c * (KC // 2), KC // 2), :]
            rowsets = [kt[n * 64:(n + 1) * 64, :] for n in range(4)]
            if c >= MD:
                d = None
                for rb in range(NRB):
                    for v in range(RU // 8):
                        t_ = mhist[c - MD][rb][v * 8:(v + 1) * 8, :]
                        d = t_ if d is None else jnp.maximum(d, t_)
                r2 = rowsets[2]
                rowsets[2] = jnp.concatenate(
                    [jnp.concatenate([pin(r2[0:8, 0:128], pltpu.bitcast(d, U32)), r2[0:8, 128:]], axis=1), r2[8:]], axis=0)
            if LN0 <= c < LN0 + NRB:
                r1 = rowsets[1]
                rel = None
                if c >= 1 and LNL:
                    rel = jnp.concatenate([scs[c - 1][rsl(c - LN0), csl(LNL - 1)]] * 4, axis=1)
                rowsets[1] = jnp.concatenate([pin(r1[:RU // 2], tail(c - LN0, rel)), r1[RU // 2:]], axis=0)
            kt = jnp.concatenate(rowsets, axis=0)
            sc = _dot_nt(q, kt)
            scs.append(sc)
            for rb in range(NRB):
                parts = [sc[rsl(rb), csl(j)] for j in range(4)]
                if c == NKC - 1:
                    lane = lax.broadcasted_iota(jnp.int32, (RU, 128), 1)
                    parts[3] = jnp.where(lane < T - (c * KC + 384), parts[3], -jnp.inf)
                mm = jnp.maximum(jnp.maximum(parts[0], parts[1]), jnp.maximum(parts[2], parts[3]))
                m[rb] = mm if m[rb] is None else jnp.maximum(m[rb], mm)
                for j in range(4):
                    sp[c, rb, j] = parts[j]
            mhist.append(list(m))
        all_units(tail)
        if prev == "ff1":
            mid = qv_matmul(NTILE - 1)
        else:
            mid = _dot(hb[...], wp1[...])
        mxb = [jnp.broadcast_to(jnp.max(m[rb], axis=-1, keepdims=True), (RU, 128)) for rb in range(NRB)]
        C0, RL = 2, 25
        CN = 15
        slots = [(c * 4 + n) * NV + v for c in range(C0, NKC) for n in range(4) if CN >> n & 1 for v in range(NV)]
        where = {slots[k * len(slots) // max(len(late), 1)]: u_ for k, u_ in enumerate(late)}
        acc, l128, pvs = {}, [None] * NRB, []
        for c in range(NKC):
            pbl = []
            for rb in range(NRB):
                mb = mxb[rb]
                if c == 1:
                    mb = pin(mb, mid[rsl(rb), D:D + 128])
                elif c >= 2:
                    mb = pin(mb, pvs[c - 1][rsl(rb), 0:128])
                pj = [jnp.exp2(sp[c, rb, j] - mb) for j in range(4)]
                lsum = (pj[0] + pj[1]) + (pj[2] + pj[3])
                l128[rb] = lsum if l128[rb] is None else l128[rb] + lsum
                pbl.append(jnp.concatenate(pj, axis=1))
            pv = jnp.dot(jnp.concatenate(pbl, axis=0).astype(BF), unpack(vs[pl.ds(kb + c * (KC // 2), KC // 2), :]),
                         preferred_element_type=F32)
            pvs.append(pv)
            for n in range(4):
                side = None
                if c == 1:
                    if prev == "ff1":
                        qs[_prows(NTILE - 1), csl(n)] = pack(mid[:, csl(n)])
                        vs[_pkrows(NTILE - 1), csl(n)] = pack(mid[:, D + n * 128:D + (n + 1) * 128])
                    else:
                        side = glu_block(i - 1, mid, n)
                for v in range(NV):
                    blk = pv[v * 8:(v + 1) * 8, csl(n)]
                    if c == 0:
                        acc[n, v] = blk
                        continue
                    a = acc[n, v]
                    if side is not None:
                        a = pin(a, side[v * 8:(v + 1) * 8, :])
                    slot = (c * 4 + n) * NV + v
                    if slot in where:
                        s0 = slot - RL
                        dep = pvs[s0 // (4 * NV)][(s0 % NV) * 8:(s0 % NV) * 8 + 8, csl((s0 // NV) % 4)]
                        cb_, t_, j_, key_ = where[slot]
                        a = pin(a, conv(cb_, t_, j_, dep, key_, has_old if key_ == 0 else None))
                        if key_ == 0:
                            flush(cb_, has_old)
                    if n == 2:
                        rb, vv = divmod(v, RU // 8)
                        a = pin(a, l128[rb][vv * 8:(vv + 1) * 8, :])
                    acc[n, v] = a + blk
        for n in range(4):
            for v in range(NV):
                accs[v * 8:(v + 1) * 8, csl(n)] = acc[n, v]
        for rb in range(NRB):
            ls[rsl(rb), :] = l128[rb]

    def bn_silu_unit(i, pin):
        def unit(rb, rel):
            z = pack(_silu((held(dcs[_rows(i, rb), :], rel, pin) - bn[0:1, :]) * bn[1:2, :]))
            zs[rb * (RU // 2):(rb + 1) * (RU // 2), :] = z
            return zs[rb * (RU // 2):(rb + 1) * (RU // 2), :]
        return memo(unit)

    def c_step(i, do_prev, do_cur, do_next):
        pin = make_pin()
        if do_cur:
            y3 = _dot(zs[...], wp2[...])

            def x3u(rb, rel):
                x3 = held(xs[_rows(i, rb), :], rel, pin) + y3[rsl(rb), :]
                xs[_rows(i, rb), :] = x3
                return stash(rb, pack(_ln(x3)))
            x3u = memo(x3u)
        if do_prev:
            r1 = []
            yacc = acc_matmul(us, w2b, pin, spread(5, 10, x3u, r1, 3) if do_cur else {}, r1)

            def out_unit(rb, rel):
                o = pack(_ln(held(xs[_rows(i - 1, rb), :], rel, pin) + 0.5 * yacc[rb]))
                qs[_prows(i - 1, rb), :] = o
                return qs[_prows(i - 1, rb), :]
            out_unit = memo(out_unit)
        if do_cur:
            dl, r2 = {}, []
            if do_prev:
                dl.update(spread(6, 5, out_unit, r2, 4))
            if do_next:
                nd = len(dl)
                dl.update(spread(11, 5, bn_silu_unit(jnp.minimum(i + 1, NTILE - 1), pin), r2, 90))
                assert len(dl) == nd + NRB
            all_units(x3u)
            ffa(hb[...], w2a, pin, dl, r2)
        elif do_prev:
            all_units(out_unit)

    W1A, W1B, WQ, WK, WV, WO, WP1, WP2, W2A, W2B, DW = range(11)
    xcopy(0).start()
    for c in range(4):
        w1a_copy(c).start()
    xcopy(1).start()
    for c in range(4):
        w1b_copy(c).start()
    for k in (DW, WQ, WK, WV, WO):
        wcopy(k).start()
    for t in range(2, NTILE):
        xcopy(t).start()
    for k in (WP1, WP2, W2A, W2B):
        wcopy(k).start()
    for b in range(B):
        hs[(b * TP + T) // 2:(b + 1) * TP // 2, :] = jnp.zeros(((TP - T) // 2, D), U32)
        vs[(b * TP + T) // 2:(b + 1) * TP // 2, :] = jnp.zeros(((TP - T) // 2, D), U32)
        for cb in range(4):
            g0 = cb * GR + b * (T + 2 * HALO)
            gs[g0:g0 + HALO, :] = jnp.zeros((HALO, 128), F32)
            gs[g0 + HALO + T:g0 + T + 2 * HALO, :] = jnp.zeros((HALO, 128), F32)
    for cb in range(4):
        gs[cb * GR + HALO + TM:cb * GR + HALO + TM + 16, :] = jnp.zeros((16, 128), F32)
    st[...] = jnp.zeros(st.shape, F32)
    bn[...] = jnp.zeros(bn.shape, F32)
    xcopy(0).wait()

    def first_a(c):
        for cc in ((0,), (1,), (2, 3), ())[c]:
            w1a_copy(cc).wait()
    a_step(0, False, pre_a=first_a)

    def first_b(kg):
        if kg == 2:
            w1b_copy(2).wait()
            w1b_copy(3).wait()

    def fold_weights(c):
        if c != 0:
            return
        for k in (DW, WQ, WK, WV, WO):
            wcopy(k).wait()
        for kk in range(KW):
            for cb in range(4):
                dwt[(kk * 4 + cb) * 8:(kk * 4 + cb + 1) * 8, :] = jnp.broadcast_to(
                    dw_ref[kk:kk + 1, csl(cb)].astype(F32), (8, 128))
        mqv[:, :D] = pack(_dot_nt(wq[...], wk[...]) * (D ** -0.5 * LOG2E))
        mqv[:, D:] = pack(_dot(wv[...], wo[...]))
    xcopy(1).wait()
    w1b_copy(0).wait()
    w1b_copy(1).wait()
    bn[2:3, :] = unpack(w1a[0:8, 0:D]).astype(F32)[0:1, :]
    a_step(1, True, pre_a=fold_weights, pre_b=first_b)


    def a_body(j, c):
        xcopy(2 * j).wait()
        xcopy(2 * j + 1).wait()
        a_step(2 * j, True)
        a_step(2 * j + 1, True)
        return c
    lax.fori_loop(1, NTILE // 2 - 1, a_body, 0)
    if 1:
        a_body(NTILE // 2 - 1, 0)

    for k in (WP1, WP2, W2A, W2B):
        wcopy(k).wait()
    b_step(0, "ff1", 0)

    def b_body(i, c):
        b_step(i, "attn", 2)
        return c
    lax.fori_loop(1, NTILE, b_body, 0)

    pin = make_pin()
    all_units(attn_tail_unit(NTILE - 1, pin))
    conv, flush = conv_stream((NV - 1) + NV * (NTILE - 2), pin)
    for n in range(4):
        wab = jnp.concatenate([wp1[:, csl(n)], wp1[:, D + n * 128:D + (n + 1) * 128]], axis=1)
        yab = _dot(hb[...], wab)
        gs[pl.ds(_grow(NTILE - 1) + n * GR + HALO, TM), :] = yab[:, :128] * _sigmoid(yab[:, 128:])
        conv(n, NTILE - 2, NV - 1, None, 0)
        for j in range(NV):
            conv(n, NTILE - 1, j, None, 1)
        flush(n)
    mean8, m28 = st[0], st[1]
    mu = jnp.mean(mean8, axis=0, keepdims=True)
    dm = mean8 - mu
    var = (jnp.sum(m28, axis=0, keepdims=True) + (B * T // 8) * jnp.sum(dm * dm, axis=0, keepdims=True)) * (1.0 / (B * T))
    bn[0:1, :] = mu
    bn[1:2, :] = lax.rsqrt(var + EPS)
    all_units(bn_silu_unit(0, pin))
    c_step(0, False, True, True)

    c_step(1, True, True, True)
    ocopy(0).start()

    def c_body(j, c):
        c_step(2 * j, True, True, True)
        c_step(2 * j + 1, True, True, True)
        ocopy(2 * j - 1).start()
        ocopy(2 * j).start()
        return c
    lax.fori_loop(1, NTILE // 2, c_body, 0)
    c_step(NTILE, True, False, False)
    ocopy(NTILE - 1).start()
    for t in range(NTILE):
        ocopy(t).wait()


@jax.jit
def pallas_standalone__conformer_family_conformer__speech_kernel(x, w_ff1_a, w_ff1_b, w_q, w_k, w_v, w_o, w_pw1, dw, w_pw2, w_ff2_a, w_ff2_b):
    xf = x.reshape(B * T, D)
    ws = (w_ff1_a, w_ff1_b, w_q, w_k, w_v, w_o, w_pw1, dw, w_pw2, w_ff2_a, w_ff2_b)
    packed = lambda w: pltpu.VMEM((w.shape[0] // 2, w.shape[1]), U32)
    hbm = pl.BlockSpec(memory_space=pl.ANY)
    out = pl.pallas_call(
        kernel,
        in_specs=[hbm] * 12,
        out_specs=hbm,
        out_shape=jax.ShapeDtypeStruct((B * T, D), x.dtype),
        scratch_shapes=[packed(w) for w in (w_ff1_a, w_ff1_b, w_q, w_k, w_v, w_o, w_pw1, w_pw2, w_ff2_a, w_ff2_b)] + [
            pltpu.VMEM((KW, D), BF),
            pltpu.VMEM((B * T, D), F32),
            pltpu.VMEM((B * TP // 2, D), U32),
            pltpu.VMEM((B * T // 2, D), U32),
            pltpu.VMEM((B * TP // 2, D), U32),
            pltpu.VMEM((4 * GR, 128), F32),
            pltpu.VMEM((B * T, D), F32),
            pltpu.VMEM((TM // 2, F), U32),
            pltpu.VMEM((TM // 2, D), U32),
            pltpu.VMEM((TM, D), F32),
            pltpu.VMEM((TM, 128), F32),
            pltpu.VMEM((TM // 2, D), U32),
            pltpu.VMEM((D // 2, 2 * D), U32),
            pltpu.VMEM((KW * 4 * 8, 128), F32),
            pltpu.VMEM((2, 8, D), F32),
            pltpu.VMEM((8, D), F32),
            pltpu.SemaphoreType.DMA((11,)),
            pltpu.SemaphoreType.DMA((8,)),
            pltpu.SemaphoreType.DMA((NTILE,)),
            pltpu.SemaphoreType.DMA((1,)),
        ],
        compiler_params=pltpu.CompilerParams(vmem_limit_bytes=124 * 1024 * 1024),
    )(xf, *ws)
    return out.reshape(B, T, D)
```

```python
import jax
import jax.numpy as jnp
from jax import lax
from jax.experimental import pallas as pl
from jax.experimental.pallas import tpu as pltpu

B, T, D, F, KW = 2, 4000, 512, 2048, 15
TP = 4096
TM = 400
NT = T // TM
NTILE = B * NT
KC = 512
NKC = TP // KC
RU = 80
NRB = TM // RU
NV = TM // 8
EPS = 1e-5
LOG2E = 1.4426950408889634
BF = jnp.bfloat16
F32 = jnp.float32
U32 = jnp.uint32
HALO = 8
GR = B * (T + 2 * HALO)


def _ln(x):
    m = jnp.mean(x, axis=-1, keepdims=True)
    xc = x - m
    v = jnp.mean(xc * xc, axis=-1, keepdims=True)
    return xc * lax.rsqrt(v + EPS)


def pack(x):
    return pltpu.bitcast(x.astype(BF), U32)


def unpack(w):
    return pltpu.bitcast(w, BF)


def _dot(a32, b32):
    return jnp.dot(unpack(a32), unpack(b32), preferred_element_type=F32)


def _dot_nt(a32, b32):
    return lax.dot_general(unpack(a32), unpack(b32), (((1,), (1,)), ((), ())), preferred_element_type=F32)


def _sigmoid(x):
    return 0.5 * jnp.tanh(0.5 * x) + 0.5


def _silu(x):
    hx = 0.5 * x
    return hx * jnp.tanh(hx) + hx


def _mult(v, n):
    return v if isinstance(v, int) else pl.multiple_of(v, n)


def _rows(i, rb=None):
    if rb is None:
        return pl.ds(_mult(i * TM, 8), TM)
    return pl.ds(_mult(i * TM + rb * RU, 8), RU)


def _prows(i, rb=None):
    if rb is None:
        return pl.ds(_mult(i * (TM // 2), 8), TM // 2)
    return pl.ds(_mult(i * (TM // 2) + rb * (RU // 2), 8), RU // 2)


def _pk0(i):
    return (i // NT) * (TP // 2) + (i % NT) * (TM // 2)


def _pkrows(i):
    return pl.ds(_mult(_pk0(i), 8), TM // 2)


def _grow(i):
    return (i // NT) * (T + 2 * HALO) + (i % NT) * TM


def rsl(rb):
    return slice(rb * RU, (rb + 1) * RU)


def csl(n):
    return slice(n * 128, (n + 1) * 128)


def kernel(x_hbm, w1a_h, w1b_h, wq_h, wk_h, wv_h, wo_h, wp1_h, dw_h, wp2_h, w2a_h, w2b_h, o_hbm,
           w1a, w1b, wq, wk, wv, wo, wp1, wp2, w2a, w2b, dw_ref,
           xs, hs, qs, vs, gs, dcs, us, hb, accs, ls, zs, mqv, dwt, st, bn,
           wsem, csem, xsem, osem):
    def wcopy(k):
        srcs = (w1a_h, w1b_h, wq_h, wk_h, wv_h, wo_h, wp1_h, wp2_h, w2a_h, w2b_h, dw_h)
        dsts = (w1a, w1b, wq, wk, wv, wo, wp1, wp2, w2a, w2b)
        dst = dw_ref if k == 10 else dsts[k].bitcast(BF)
        return pltpu.make_async_copy(srcs[k], dst, wsem.at[k])

    def w1a_copy(c):
        return pltpu.make_async_copy(w1a_h.at[:, c * 512:(c + 1) * 512], w1a.bitcast(BF).at[:, c * 512:(c + 1) * 512], csem.at[c])

    def w1b_copy(c):
        return pltpu.make_async_copy(w1b_h.at[c * 512:(c + 1) * 512, :], w1b.bitcast(BF).at[c * 512:(c + 1) * 512, :], csem.at[4 + c])

    def xcopy(i):
        rows = pl.ds(_mult(i * TM, 16), TM)
        return pltpu.make_async_copy(x_hbm.at[rows, :], qs.bitcast(BF).at[rows, :], xsem.at[i])

    def ocopy(i):
        rows = pl.ds(_mult(i * TM, 16), TM)
        return pltpu.make_async_copy(qs.bitcast(BF).at[rows, :], o_hbm.at[rows, :], osem.at[0])

    def make_pin():
        nv = jnp.abs(bn[2:3, :])

        def pin(val, dep):
            never = jnp.broadcast_to(nv[:, :val.shape[1]], val.shape) < 0.0
            return jnp.where(never, dep, val)
        return pin

    def memo(fn):
        cache = {}

        def get(rb, rel=None):
            if rb not in cache:
                cache[rb] = fn(rb, rel)
            return cache[rb]
        return get

    def stash(rb, h32):
        hb[rb * (RU // 2):(rb + 1) * (RU // 2), :] = h32
        return hb[rb * (RU // 2):(rb + 1) * (RU // 2), :]

    def all_units(get):
        for rb in range(NRB):
            get(rb)

    def pin_rhs(w32, pin, tokens):
        if not tokens:
            return w32
        cols = []
        for n in range(4):
            col = w32[:, csl(n)]
            if n in tokens:
                tk = tokens[n]()
                k = tk.shape[0]
                col = jnp.concatenate([pin(col[:k], tk), col[k:]], axis=0)
            cols.append(col)
        return jnp.concatenate(cols, axis=1)

    def spread(first, count, unit, res, lead):
        out = {}
        for rb in range(NRB):
            p = first + rb * count // NRB
            pr = min(p - lead, 4 * (p // 4) - 1)

            def token(rb=rb, pr=pr):
                rel = None
                if pr >= 0 and lead < 90:
                    rel = jnp.concatenate([res[pr // 4][rsl(rb), csl(pr % 4)]] * 4, axis=1)
                u_ = unit(rb, rel)
                return jnp.concatenate([u_[:, csl(n)] for n in range(4)], axis=0)
            assert p < 16 and (p // 4, p % 4) not in out
            out[p // 4, p % 4] = token
        return out

    def tok(deadlines, c):
        return {n: f for (cc, n), f in deadlines.items() if cc == c}

    def acc_matmul(lhs, w, pin, deadlines, res, pre=None):
        acc = None
        for kg in range(4):
            if pre:
                pre(kg)
            part = _dot(lhs[:, kg * 512:(kg + 1) * 512], pin_rhs(w[kg * 256:(kg + 1) * 256, :], pin, tok(deadlines, kg)))
            res.append(part)
            if acc is None:
                acc = [part[rsl(rb), :] for rb in range(NRB)]
            else:
                acc = [acc[rb] + part[rsl(rb), :] for rb in range(NRB)]
        return acc

    def ffa(h32, wa, pin, deadlines, res, pre=None):
        for c in range(F // 512):
            if pre:
                pre(c)
            u = _dot(h32, pin_rhs(wa[:, c * 512:(c + 1) * 512], pin, tok(deadlines, c)))
            res.append(u)
            us[:, c * 512:(c + 1) * 512] = pack(_silu(u))

    def held(val, rel, pin):
        if rel is None:
            return val
        if val.dtype == U32:
            return pin(val, pltpu.bitcast(rel[:val.shape[0]], U32))
        return pin(val, rel)

    def ff1_tail_unit(i, yacc, pin):
        def unit(rb, rel):
            x1 = unpack(held(qs[_prows(i, rb), :], rel, pin)).astype(F32) + 0.5 * yacc[rb]
            xs[_rows(i, rb), :] = x1
            h1 = pack(_ln(x1))
            rows = pl.ds(_mult(_pk0(i) + rb * (RU // 2), 8), RU // 2)
            hs[rows, :] = h1
            return hs[rows, :]
        return memo(unit)

    def qv_matmul(i):
        return _dot(hs[_pkrows(i), :], mqv[...])

    def a_step(i, do_prev, pre_a=None, pre_b=None, pre_qv=None, mode="steady"):
        pin = make_pin()
        lnx = memo(lambda rb, rel: stash(rb, pack(_ln(unpack(held(qs[_prows(i, rb), :], rel, pin)).astype(F32)))))
        dl, r1, r2 = {}, [], []
        lhs = hb
        if mode == "first":
            def nxt(rb, rel):
                rows = slice(rb * (RU // 2), (rb + 1) * (RU // 2))
                zs[rows, :] = pack(_ln(unpack(held(qs[_prows(i + 1, rb), :], rel, pin)).astype(F32)))
                return zs[rows, :]
            dl = spread(9, 5, memo(nxt), r2, 4)
        if do_prev:
            yacc = acc_matmul(us, w1b, pin, {} if mode == "second" else spread(4, 10, lnx, r1, 3), r1, pre_b)
            tail = ff1_tail_unit(i - 1, yacc, pin)
            dl = spread(2, 10, tail, r2, 4)
        if mode == "second":
            lhs = zs
        else:
            all_units(lnx)
        ffa(lhs[...], w1a, pin, dl, r2, pre_a)
        if do_prev:
            if pre_qv:
                pre_qv()
            all_units(tail)
            qv = qv_matmul(i - 1)
            qs[_prows(i - 1), :] = pack(qv[:, :D])
            vs[_pkrows(i - 1), :] = pack(qv[:, D:])

    def conv_stream(n_old, pin):
        cs = [dict(cnt=0) for _ in range(4)]
        sub = lax.broadcasted_iota(jnp.int32, (8, 128), 0)

        def rot(v):
            return [v] + [pltpu.roll(v, 8 - s_, 0) for s_ in range(1, 8)]

        def shift(ra, rb_):
            return [ra[0]] + [jnp.where(sub < 8 - s_, ra[s_], rb_[s_]) for s_ in range(1, 8)]

        def step(cb, t, j, dep, key, valid=None):
            c_ = cs[cb]
            g0 = _grow(t)
            rel = (lambda v: v) if dep is None else (lambda v: pin(v, dep))
            ld = lambda jj: rel(gs[pl.ds(_mult(g0 + cb * GR + 8 * jj, 8), 8), :])
            if c_.get("next") != (key, j):
                ra, rb_ = rot(ld(j)), rot(ld(j + 1))
                c_["G"], c_["R"] = shift(ra, rb_), rb_
            if "w" not in c_:
                c_["w"] = [dwt[(kk * 4 + cb) * 8:(kk * 4 + cb + 1) * 8, :] for kk in range(KW)]
            rn = rot(ld(j + 2))
            gn = shift(c_["R"], rn)
            terms = [c_["G"][s_] * c_["w"][s_ - 1] for s_ in range(1, 8)] + [gn[s_] * c_["w"][7 + s_] for s_ in range(8)]
            c_["G"], c_["R"], c_["next"] = gn, rn, (key, j + 1)
            while len(terms) > 1:
                terms = [terms[q] + terms[q + 1] for q in range(0, len(terms) - 1, 2)] + ([terms[-1]] if len(terms) % 2 else [])
            o = terms[0]
            dcs[pl.ds(_mult(t * TM + 8 * j, 8), 8), csl(cb)] = o
            if c_["cnt"] == 0:
                c_["c"] = o
            else:
                d = o - c_["c"]
                if valid is not None:
                    d = jnp.where(valid, d, 0.0)
                c_["s1"] = d if c_["cnt"] == 1 else c_["s1"] + d
                c_["s2"] = d * d if c_["cnt"] == 1 else c_["s2"] + d * d
            c_["cnt"] += 1
            return o

        def flush(cb, valid=None):
            c_ = cs[cb]
            k = jnp.full((8, 128), c_["cnt"], F32)
            if valid is not None:
                k = jnp.where(valid, k, k - 1.0)
            cols = csl(cb)
            rk = 1.0 / k
            tmean = c_["c"] + c_["s1"] * rk
            tm2 = c_["s2"] - c_["s1"] * c_["s1"] * rk
            n = jnp.zeros((8, 128), F32) + jnp.asarray(n_old, F32)
            f = k / (n + k)
            mean_old = st[0, :, cols]
            delta = tmean - mean_old
            st[0, :, cols] = mean_old + delta * f
            st[1, :, cols] = st[1, :, cols] + tm2 + delta * delta * (n * f)
            c_["cnt"] = 0
        return step, flush

    def attn_tail_unit(i, pin):
        def unit(rb, rel):
            lsum = ls[rsl(rb), :]
            if rel is not None:
                lsum = pin(lsum, rel[:, 0:128])
            inv = 1.0 / jnp.sum(lsum, axis=-1, keepdims=True)
            x2 = held(xs[_rows(i, rb), :], rel, pin) + accs[rsl(rb), :] * inv
            xs[_rows(i, rb), :] = x2
            return stash(rb, pack(_ln(x2)))
        return memo(unit)

    def glu_block(i, y2, n):
        g = y2[:, csl(n)] * _sigmoid(y2[:, D + n * 128:D + (n + 1) * 128])
        gs[pl.ds(_mult(_grow(i) + (n * GR + HALO), 8), TM), :] = g
        return g

    def b_step(i, prev, conv_mode):
        pin = make_pin()
        kb = _mult((i // NT) * (TP // 2), TP // 2)
        if prev == "ff1":
            tail = ff1_tail_unit(NTILE - 1, acc_matmul(us, w1b, pin, {}, []), pin)
        else:
            tail = attn_tail_unit(i - 1, pin)
        q = qs[_prows(i), :]
        m = [None] * NRB
        mhist = []
        sp = {}
        MD, LN0, LNL = 2, 2, 0
        scs = []
        late = []
        if conv_mode:
            has_old = i >= 2
            conv, flush = conv_stream(jnp.where(has_old, (NV - 1) + NV * (i - 2), 0), pin)
            for cb in range(4):
                late += [(cb, i - 1, j, 1) for j in range(NV - 1)]
                late.append((cb, jnp.maximum(i - 2, 0), NV - 1, 0))
        for c in range(NKC):
            kt = hs[pl.ds(kb + c * (KC // 2), KC // 2), :]
            rowsets = [kt[n * 64:(n + 1) * 64, :] for n in range(4)]
            if c >= MD:
                d = None
                for rb in range(NRB):
                    for v in range(RU // 8):
                        t_ = mhist[c - MD][rb][v * 8:(v + 1) * 8, :]
                        d = t_ if d is None else jnp.maximum(d, t_)
                MP = 3
                r2 = rowsets[MP]
                rowsets[MP] = jnp.concatenate(
                    [jnp.concatenate([pin(r2[0:8, 0:128], pltpu.bitcast(d, U32)), r2[0:8, 128:]], axis=1), r2[8:]], axis=0)
            if LN0 <= c < LN0 + NRB:
                LP = 0
                r1 = rowsets[LP]
                rel = None
                if c >= 1 and LNL:
                    rel = jnp.concatenate([scs[c - 1][rsl(c - LN0), csl(LNL - 1)]] * 4, axis=1)
                rowsets[LP] = jnp.concatenate([pin(r1[:RU // 2], tail(c - LN0, rel)), r1[RU // 2:]], axis=0)
            kt = jnp.concatenate(rowsets, axis=0)
            sc = _dot_nt(q, kt)
            scs.append(sc)
            for rb in range(NRB):
                parts = [sc[rsl(rb), csl(j)] for j in range(4)]
                if c == NKC - 1:
                    lane = lax.broadcasted_iota(jnp.int32, (RU, 128), 1)
                    parts[3] = jnp.where(lane < T - (c * KC + 384), parts[3], -jnp.inf)
                mm = jnp.maximum(jnp.maximum(parts[0], parts[1]), jnp.maximum(parts[2], parts[3]))
                m[rb] = mm if m[rb] is None else jnp.maximum(m[rb], mm)
                for j in range(4):
                    sp[c, rb, j] = parts[j]
            mhist.append(list(m))
        all_units(tail)
        if prev == "ff1":
            mid = qv_matmul(NTILE - 1)
        else:
            mid = _dot(hb[...], wp1[...])
        mxb = [jnp.broadcast_to(jnp.max(m[rb], axis=-1, keepdims=True), (RU, 128)) for rb in range(NRB)]
        C0, RL = 2, 31
        CN = 15
        slots = [(c * 4 + n) * NV + v for c in range(C0, NKC) for n in range(4) if CN >> n & 1 for v in range(NV)]
        slots = slots[0:len(slots) - 0]
        where = {slots[k * len(slots) // max(len(late), 1)]: u_ for k, u_ in enumerate(late)}
        acc, l128, pvs = {}, [None] * NRB, []
        for c in range(NKC):
            pbl = []
            for rb in range(NRB):
                mb = mxb[rb]
                if c == 1:
                    mb = pin(mb, mid[rsl(rb), csl(4)])
                elif c >= 2:
                    mb = pin(mb, pvs[c - 1][rsl(rb), csl(1)])
                pj = [jnp.exp2(sp[c, rb, j] - mb) for j in range(4)]
                lsum = (pj[0] + pj[1]) + (pj[2] + pj[3])
                l128[rb] = lsum if l128[rb] is None else l128[rb] + lsum
                pbl.append(jnp.concatenate(pj, axis=1))
            pv = jnp.dot(jnp.concatenate(pbl, axis=0).astype(BF), unpack(vs[pl.ds(kb + c * (KC // 2), KC // 2), :]),
                         preferred_element_type=F32)
            pvs.append(pv)
            for n in range(4):
                side = None
                if c == 1:
                    if prev == "ff1":
                        qs[_prows(NTILE - 1), csl(n)] = pack(mid[:, csl(n)])
                        vs[_pkrows(NTILE - 1), csl(n)] = pack(mid[:, D + n * 128:D + (n + 1) * 128])
                    else:
                        side = glu_block(i - 1, mid, n)
                for v in range(NV):
                    blk = pv[v * 8:(v + 1) * 8, csl(n)]
                    if c == 0:
                        acc[n, v] = blk
                        continue
                    a = acc[n, v]
                    if side is not None:
                        a = pin(a, side[v * 8:(v + 1) * 8, :])
                    slot = (c * 4 + n) * NV + v
                    if slot in where:
                        s0 = slot - RL
                        dep = pvs[s0 // (4 * NV)][(s0 % NV) * 8:(s0 % NV) * 8 + 8, csl((s0 // NV) % 4)]
                        cb_, t_, j_, key_ = where[slot]
                        a = pin(a, conv(cb_, t_, j_, dep, key_, has_old if key_ == 0 else None))
                        if key_ == 0:
                            flush(cb_, has_old)
                    if n == 1:
                        rb, vv = divmod(v, RU // 8)
                        a = pin(a, l128[rb][vv * 8:(vv + 1) * 8, :])
                    acc[n, v] = a + blk
        for n in range(4):
            for v in range(NV):
                accs[v * 8:(v + 1) * 8, csl(n)] = acc[n, v]
        for rb in range(NRB):
            ls[rsl(rb), :] = l128[rb]

    def bn_silu_unit(i, pin):
        def unit(rb, rel):
            z = pack(_silu((held(dcs[_rows(i, rb), :], rel, pin) - bn[0:1, :]) * bn[1:2, :]))
            zs[rb * (RU // 2):(rb + 1) * (RU // 2), :] = z
            return zs[rb * (RU // 2):(rb + 1) * (RU // 2), :]
        return memo(unit)

    def c_step(i, do_prev, do_cur, do_next):
        pin = make_pin()
        if do_cur:
            y3 = _dot(zs[...], wp2[...])

            def x3u(rb, rel):
                x3 = held(xs[_rows(i, rb), :], rel, pin) + y3[rsl(rb), :]
                xs[_rows(i, rb), :] = x3
                return stash(rb, pack(_ln(x3)))
            x3u = memo(x3u)
        if do_prev:
            r1 = []
            yacc = acc_matmul(us, w2b, pin, spread(5, 10, x3u, r1, 3) if do_cur else {}, r1)

            def out_unit(rb, rel):
                o = pack(_ln(held(xs[_rows(i - 1, rb), :], rel, pin) + 0.5 * yacc[rb]))
                qs[_prows(i - 1, rb), :] = o
                return qs[_prows(i - 1, rb), :]
            out_unit = memo(out_unit)
        if do_cur:
            dl, r2 = {}, []
            if do_prev:
                dl.update(spread(6, 5, out_unit, r2, 4))
            if do_next:
                nd = len(dl)
                dl.update(spread(11, 5, bn_silu_unit(jnp.minimum(i + 1, NTILE - 1), pin), r2, 90 if do_prev else 3))
                assert len(dl) == nd + NRB
            all_units(x3u)
            ffa(hb[...], w2a, pin, dl, r2)
        elif do_prev:
            all_units(out_unit)

    W1A, W1B, WQ, WK, WV, WO, WP1, WP2, W2A, W2B, DW = range(11)
    xcopy(0).start()
    for c in range(4):
        w1a_copy(c).start()
    xcopy(1).start()
    for c in range(4):
        w1b_copy(c).start()
    for k in (DW, WQ, WK, WV, WO):
        wcopy(k).start()
    for t in range(2, NTILE):
        xcopy(t).start()
    for k in (WP1, WP2, W2A, W2B):
        wcopy(k).start()
    for b in range(B):
        hs[(b * TP + T) // 2:(b + 1) * TP // 2, :] = jnp.zeros(((TP - T) // 2, D), U32)
        vs[(b * TP + T) // 2:(b + 1) * TP // 2, :] = jnp.zeros(((TP - T) // 2, D), U32)
        for cb in range(4):
            g0 = cb * GR + b * (T + 2 * HALO)
            gs[g0:g0 + HALO, :] = jnp.zeros((HALO, 128), F32)
            gs[g0 + HALO + T:g0 + T + 2 * HALO, :] = jnp.zeros((HALO, 128), F32)
    for cb in range(4):
        gs[cb * GR + HALO + TM:cb * GR + HALO + TM + 16, :] = jnp.zeros((16, 128), F32)
    st[...] = jnp.zeros(st.shape, F32)
    bn[...] = jnp.zeros(bn.shape, F32)
    xcopy(0).wait()
    bn[2:3, :] = unpack(qs[0:8, :]).astype(F32)[0:1, :]

    def first_a(c):
        for cc in ((0,), (1,), (2, 3), ())[c]:
            w1a_copy(cc).wait()
        if c == 2:
            xcopy(1).wait()
    a_step(0, False, pre_a=first_a, mode="first")

    def first_b(kg):
        if kg == 2:
            w1b_copy(2).wait()
            w1b_copy(3).wait()

    def fold_weights(c):
        if c != 0:
            return
        for k in (DW, WQ, WK, WV, WO):
            wcopy(k).wait()
        for kk in range(KW):
            for cb in range(4):
                dwt[(kk * 4 + cb) * 8:(kk * 4 + cb + 1) * 8, :] = jnp.broadcast_to(
                    dw_ref[kk:kk + 1, csl(cb)].astype(F32), (8, 128))
        mqv[:, :D] = pack(_dot_nt(wq[...], wk[...]) * (D ** -0.5 * LOG2E))
        mqv[:, D:] = pack(_dot(wv[...], wo[...]))
    w1b_copy(0).wait()
    w1b_copy(1).wait()
    a_step(1, True, pre_a=fold_weights, pre_b=first_b, mode="second")


    def a_body(j, c):
        xcopy(2 * j).wait()
        xcopy(2 * j + 1).wait()
        a_step(2 * j, True)
        a_step(2 * j + 1, True)
        return c
    lax.fori_loop(1, NTILE // 2 - 1, a_body, 0)
    if 1:
        a_body(NTILE // 2 - 1, 0)

    for k in (WP1, WP2, W2A, W2B):
        wcopy(k).wait()
    b_step(0, "ff1", 0)

    def b_body(i, c):
        b_step(i, "attn", 2)
        return c
    lax.fori_loop(1, NTILE, b_body, 0)

    pin = make_pin()
    all_units(attn_tail_unit(NTILE - 1, pin))
    conv, flush = conv_stream((NV - 1) + NV * (NTILE - 2), pin)
    for n in range(4):
        wab = jnp.concatenate([wp1[:, csl(n)], wp1[:, D + n * 128:D + (n + 1) * 128]], axis=1)
        yab = _dot(hb[...], wab)
        gs[pl.ds(_grow(NTILE - 1) + n * GR + HALO, TM), :] = yab[:, :128] * _sigmoid(yab[:, 128:])
        conv(n, NTILE - 2, NV - 1, None, 0)
        for j in range(NV):
            conv(n, NTILE - 1, j, None, 1)
        flush(n)
    mean8, m28 = st[0], st[1]
    mu = jnp.mean(mean8, axis=0, keepdims=True)
    dm = mean8 - mu
    var = (jnp.sum(m28, axis=0, keepdims=True) + (B * T // 8) * jnp.sum(dm * dm, axis=0, keepdims=True)) * (1.0 / (B * T))
    bn[0:1, :] = mu
    bn[1:2, :] = lax.rsqrt(var + EPS)
    all_units(bn_silu_unit(0, pin))
    c_step(0, False, True, True)

    c_step(1, True, True, True)
    ocopy(0).start()

    def c_body(j, c):
        c_step(2 * j, True, True, True)
        c_step(2 * j + 1, True, True, True)
        ocopy(2 * j - 1).start()
        ocopy(2 * j).start()
        return c
    lax.fori_loop(1, NTILE // 2, c_body, 0)
    c_step(NTILE, True, False, False)
    ocopy(NTILE - 1).start()
    for t in range(NTILE):
        ocopy(t).wait()


@jax.jit
def pallas_standalone__conformer_family_conformer__speech_kernel(x, w_ff1_a, w_ff1_b, w_q, w_k, w_v, w_o, w_pw1, dw, w_pw2, w_ff2_a, w_ff2_b):
    xf = x.reshape(B * T, D)
    ws = (w_ff1_a, w_ff1_b, w_q, w_k, w_v, w_o, w_pw1, dw, w_pw2, w_ff2_a, w_ff2_b)
    packed = lambda w: pltpu.VMEM((w.shape[0] // 2, w.shape[1]), U32)
    hbm = pl.BlockSpec(memory_space=pl.ANY)
    out = pl.pallas_call(
        kernel,
        in_specs=[hbm] * 12,
        out_specs=hbm,
        out_shape=jax.ShapeDtypeStruct((B * T, D), x.dtype),
        scratch_shapes=[packed(w) for w in (w_ff1_a, w_ff1_b, w_q, w_k, w_v, w_o, w_pw1, w_pw2, w_ff2_a, w_ff2_b)] + [
            pltpu.VMEM((KW, D), BF),
            pltpu.VMEM((B * T, D), F32),
            pltpu.VMEM((B * TP // 2, D), U32),
            pltpu.VMEM((B * T // 2, D), U32),
            pltpu.VMEM((B * TP // 2, D), U32),
            pltpu.VMEM((4 * GR, 128), F32),
            pltpu.VMEM((B * T, D), F32),
            pltpu.VMEM((TM // 2, F), U32),
            pltpu.VMEM((TM // 2, D), U32),
            pltpu.VMEM((TM, D), F32),
            pltpu.VMEM((TM, 128), F32),
            pltpu.VMEM((TM // 2, D), U32),
            pltpu.VMEM((D // 2, 2 * D), U32),
            pltpu.VMEM((KW * 4 * 8, 128), F32),
            pltpu.VMEM((2, 8, D), F32),
            pltpu.VMEM((8, D), F32),
            pltpu.SemaphoreType.DMA((11,)),
            pltpu.SemaphoreType.DMA((8,)),
            pltpu.SemaphoreType.DMA((NTILE,)),
            pltpu.SemaphoreType.DMA((1,)),
        ],
        compiler_params=pltpu.CompilerParams(vmem_limit_bytes=124 * 1024 * 1024),
    )(xf, *ws)
    return out.reshape(B, T, D)
```

```python
import jax
import jax.numpy as jnp
from jax import lax
from jax.experimental import pallas as pl
from jax.experimental.pallas import tpu as pltpu

B, T, D, F, KW = 2, 4000, 512, 2048, 15
TP = 4096
TM = 400
NT = T // TM
NTILE = B * NT
KC = 512
NKC = TP // KC
RU = 80
NRB = TM // RU
NV = TM // 8
EPS = 1e-5
LOG2E = 1.4426950408889634
BF = jnp.bfloat16
F32 = jnp.float32
U32 = jnp.uint32
HALO = 8
GR = B * (T + 2 * HALO)


def _ln(x):
    m = jnp.mean(x, axis=-1, keepdims=True)
    xc = x - m
    v = jnp.mean(xc * xc, axis=-1, keepdims=True)
    return xc * lax.rsqrt(v + EPS)


def pack(x):
    return pltpu.bitcast(x.astype(BF), U32)


def unpack(w):
    return pltpu.bitcast(w, BF)


def _dot(a32, b32):
    return jnp.dot(unpack(a32), unpack(b32), preferred_element_type=F32)


def _dot_nt(a32, b32):
    return lax.dot_general(unpack(a32), unpack(b32), (((1,), (1,)), ((), ())), preferred_element_type=F32)


def _sigmoid(x):
    return 0.5 * jnp.tanh(0.5 * x) + 0.5


def _silu(x):
    hx = 0.5 * x
    return hx * jnp.tanh(hx) + hx


def _mult(v, n):
    return v if isinstance(v, int) else pl.multiple_of(v, n)


def _rows(i, rb=None):
    if rb is None:
        return pl.ds(_mult(i * TM, 8), TM)
    return pl.ds(_mult(i * TM + rb * RU, 8), RU)


def _prows(i, rb=None):
    if rb is None:
        return pl.ds(_mult(i * (TM // 2), 8), TM // 2)
    return pl.ds(_mult(i * (TM // 2) + rb * (RU // 2), 8), RU // 2)


def _pk0(i):
    return (i // NT) * (TP // 2) + (i % NT) * (TM // 2)


def _pkrows(i):
    return pl.ds(_mult(_pk0(i), 8), TM // 2)


def _grow(i):
    return (i // NT) * (T + 2 * HALO) + (i % NT) * TM


def rsl(rb):
    return slice(rb * RU, (rb + 1) * RU)


def csl(n):
    return slice(n * 128, (n + 1) * 128)


def kernel(x_hbm, w1a_h, w1b_h, wq_h, wk_h, wv_h, wo_h, wp1_h, dw_h, wp2_h, w2a_h, w2b_h, o_hbm,
           w1a, w1b, wq, wk, wv, wo, wp1, wp2, w2a, w2b, dw_ref,
           xs, hs, qs, vs, gs, dcs, us, hb, accs, ls, zs, mqv, dwt, st, bn,
           wsem, csem, xsem, osem):
    def wcopy(k):
        srcs = (w1a_h, w1b_h, wq_h, wk_h, wv_h, wo_h, wp1_h, wp2_h, w2a_h, w2b_h, dw_h)
        dsts = (w1a, w1b, wq, wk, wv, wo, wp1, wp2, w2a, w2b)
        dst = dw_ref if k == 10 else dsts[k].bitcast(BF)
        return pltpu.make_async_copy(srcs[k], dst, wsem.at[k])

    def w1a_copy(c):
        return pltpu.make_async_copy(w1a_h.at[:, c * 512:(c + 1) * 512], w1a.bitcast(BF).at[:, c * 512:(c + 1) * 512], csem.at[c])

    def w1b_copy(c):
        return pltpu.make_async_copy(w1b_h.at[c * 512:(c + 1) * 512, :], w1b.bitcast(BF).at[c * 512:(c + 1) * 512, :], csem.at[4 + c])

    def xcopy(i):
        rows = pl.ds(_mult(i * TM, 16), TM)
        return pltpu.make_async_copy(x_hbm.at[rows, :], qs.bitcast(BF).at[rows, :], xsem.at[i])

    def ocopy(i):
        rows = pl.ds(_mult(i * TM, 16), TM)
        return pltpu.make_async_copy(qs.bitcast(BF).at[rows, :], o_hbm.at[rows, :], osem.at[0])

    def make_pin():
        nv = jnp.abs(bn[2:3, :])

        def pin(val, dep):
            never = jnp.broadcast_to(nv[:, :val.shape[1]], val.shape) < 0.0
            return jnp.where(never, dep, val)
        return pin

    def memo(fn):
        cache = {}

        def get(rb, rel=None):
            if rb not in cache:
                cache[rb] = fn(rb, rel)
            return cache[rb]
        return get

    def stash(rb, h32):
        hb[rb * (RU // 2):(rb + 1) * (RU // 2), :] = h32
        return hb[rb * (RU // 2):(rb + 1) * (RU // 2), :]

    def all_units(get):
        for rb in range(NRB):
            get(rb)

    def pin_rhs(w32, pin, tokens):
        if not tokens:
            return w32
        cols = []
        for n in range(4):
            col = w32[:, csl(n)]
            if n in tokens:
                tk = tokens[n]()
                k = tk.shape[0]
                col = jnp.concatenate([pin(col[:k], tk), col[k:]], axis=0)
            cols.append(col)
        return jnp.concatenate(cols, axis=1)

    def spread(first, count, unit, res, lead):
        out = {}
        for rb in range(NRB):
            p = first + rb * count // NRB
            pr = -1 if lead is None else min(p - lead, 4 * (p // 4) - 1)

            def token(rb=rb, pr=pr):
                rel = None
                if lead is not None and pr >= 0:
                    rel = jnp.concatenate([res[pr // 4][rsl(rb), csl(pr % 4)]] * 4, axis=1)
                u_ = unit(rb, rel)
                return jnp.concatenate([u_[:, csl(n)] for n in range(4)], axis=0)
            assert p < 16 and (p // 4, p % 4) not in out
            out[p // 4, p % 4] = token
        return out

    def tok(deadlines, c):
        return {n: f for (cc, n), f in deadlines.items() if cc == c}

    def acc_matmul(lhs, w, pin, deadlines, res, pre=None):
        acc = None
        for kg in range(4):
            if pre:
                pre(kg)
            part = _dot(lhs[:, kg * 512:(kg + 1) * 512], pin_rhs(w[kg * 256:(kg + 1) * 256, :], pin, tok(deadlines, kg)))
            res.append(part)
            if acc is None:
                acc = [part[rsl(rb), :] for rb in range(NRB)]
            else:
                acc = [acc[rb] + part[rsl(rb), :] for rb in range(NRB)]
        return acc

    def ffa(h32, wa, pin, deadlines, res, pre=None):
        for c in range(F // 512):
            if pre:
                pre(c)
            u = _dot(h32, pin_rhs(wa[:, c * 512:(c + 1) * 512], pin, tok(deadlines, c)))
            res.append(u)
            us[:, c * 512:(c + 1) * 512] = pack(_silu(u))

    def held(val, rel, pin):
        if rel is None:
            return val
        if val.dtype == U32:
            return pin(val, pltpu.bitcast(rel[:val.shape[0]], U32))
        return pin(val, rel)

    def ff1_tail_unit(i, yacc, pin):
        def unit(rb, rel):
            x1 = unpack(held(qs[_prows(i, rb), :], rel, pin)).astype(F32) + 0.5 * yacc[rb]
            xs[_rows(i, rb), :] = x1
            h1 = pack(_ln(x1))
            rows = pl.ds(_mult(_pk0(i) + rb * (RU // 2), 8), RU // 2)
            hs[rows, :] = h1
            return hs[rows, :]
        return memo(unit)

    def qv_matmul(i):
        return _dot(hs[_pkrows(i), :], mqv[...])

    def a_step(i, do_prev, pre_a=None, pre_b=None, mode="steady"):
        pin = make_pin()
        lnx = memo(lambda rb, rel: stash(rb, pack(_ln(unpack(held(qs[_prows(i, rb), :], rel, pin)).astype(F32)))))
        dl, r1, r2 = {}, [], []
        lhs = hb
        if mode == "first":
            def nxt(rb, rel):
                rows = slice(rb * (RU // 2), (rb + 1) * (RU // 2))
                zs[rows, :] = pack(_ln(unpack(held(qs[_prows(i + 1, rb), :], rel, pin)).astype(F32)))
                return zs[rows, :]
            dl = spread(9, 5, memo(nxt), r2, 4)
        if do_prev:
            yacc = acc_matmul(us, w1b, pin, {} if mode == "second" else spread(4, 10, lnx, r1, 3), r1, pre_b)
            tail = ff1_tail_unit(i - 1, yacc, pin)
            dl = spread(2, 10, tail, r2, 4)
        if mode == "second":
            lhs = zs
        else:
            all_units(lnx)
        ffa(lhs[...], w1a, pin, dl, r2, pre_a)
        if do_prev:
            all_units(tail)
            qv = qv_matmul(i - 1)
            qs[_prows(i - 1), :] = pack(qv[:, :D])
            vs[_pkrows(i - 1), :] = pack(qv[:, D:])

    def conv_stream(n_old, pin):
        cs = [dict(cnt=0) for _ in range(4)]
        sub = lax.broadcasted_iota(jnp.int32, (8, 128), 0)

        def rot(v):
            return [v] + [pltpu.roll(v, 8 - s_, 0) for s_ in range(1, 8)]

        def shift(ra, rb_):
            return [ra[0]] + [jnp.where(sub < 8 - s_, ra[s_], rb_[s_]) for s_ in range(1, 8)]

        def step(cb, t, j, dep, key, valid=None):
            c_ = cs[cb]
            g0 = _grow(t)
            rel = (lambda v: v) if dep is None else (lambda v: pin(v, dep))
            ld = lambda jj: rel(gs[pl.ds(_mult(g0 + cb * GR + 8 * jj, 8), 8), :])
            if c_.get("next") != (key, j):
                ra, rb_ = rot(ld(j)), rot(ld(j + 1))
                c_["G"], c_["R"] = shift(ra, rb_), rb_
            if "w" not in c_:
                c_["w"] = [dwt[(kk * 4 + cb) * 8:(kk * 4 + cb + 1) * 8, :] for kk in range(KW)]
            rn = rot(ld(j + 2))
            gn = shift(c_["R"], rn)
            terms = [c_["G"][s_] * c_["w"][s_ - 1] for s_ in range(1, 8)] + [gn[s_] * c_["w"][7 + s_] for s_ in range(8)]
            c_["G"], c_["R"], c_["next"] = gn, rn, (key, j + 1)
            while len(terms) > 1:
                terms = [terms[q] + terms[q + 1] for q in range(0, len(terms) - 1, 2)] + ([terms[-1]] if len(terms) % 2 else [])
            o = terms[0]
            dcs[pl.ds(_mult(t * TM + 8 * j, 8), 8), csl(cb)] = o
            if c_["cnt"] == 0:
                c_["c"] = o
            else:
                d = o - c_["c"]
                if valid is not None:
                    d = jnp.where(valid, d, 0.0)
                c_["s1"] = d if c_["cnt"] == 1 else c_["s1"] + d
                c_["s2"] = d * d if c_["cnt"] == 1 else c_["s2"] + d * d
            c_["cnt"] += 1
            return o

        def flush(cb, valid=None):
            c_ = cs[cb]
            k = jnp.full((8, 128), c_["cnt"], F32)
            if valid is not None:
                k = jnp.where(valid, k, k - 1.0)
            cols = csl(cb)
            rk = 1.0 / k
            tmean = c_["c"] + c_["s1"] * rk
            tm2 = c_["s2"] - c_["s1"] * c_["s1"] * rk
            n = jnp.zeros((8, 128), F32) + jnp.asarray(n_old, F32)
            f = k / (n + k)
            mean_old = st[0, :, cols]
            delta = tmean - mean_old
            st[0, :, cols] = mean_old + delta * f
            st[1, :, cols] = st[1, :, cols] + tm2 + delta * delta * (n * f)
            c_["cnt"] = 0
        return step, flush

    def attn_tail_unit(i, pin):
        def unit(rb, rel):
            lsum = ls[rsl(rb), :]
            if rel is not None:
                lsum = pin(lsum, rel[:, 0:128])
            inv = 1.0 / jnp.sum(lsum, axis=-1, keepdims=True)
            x2 = held(xs[_rows(i, rb), :], rel, pin) + accs[rsl(rb), :] * inv
            xs[_rows(i, rb), :] = x2
            return stash(rb, pack(_ln(x2)))
        return memo(unit)

    def glu_block(i, y2, n):
        g = y2[:, csl(n)] * _sigmoid(y2[:, D + n * 128:D + (n + 1) * 128])
        gs[pl.ds(_mult(_grow(i) + (n * GR + HALO), 8), TM), :] = g
        return g

    def b_step(i, prev, conv_mode):
        pin = make_pin()
        kb = _mult((i // NT) * (TP // 2), TP // 2)
        if prev == "ff1":
            tail = ff1_tail_unit(NTILE - 1, acc_matmul(us, w1b, pin, {}, []), pin)
        else:
            tail = attn_tail_unit(i - 1, pin)
        q = qs[_prows(i), :]
        m = [None] * NRB
        mhist = []
        sp = {}
        MD, LN0 = 2, 2
        late = []
        if conv_mode:
            has_old = i >= 2
            conv, flush = conv_stream(jnp.where(has_old, (NV - 1) + NV * (i - 2), 0), pin)
            for cb in range(4):
                late += [(cb, i - 1, j, 1) for j in range(NV - 1)]
                late.append((cb, jnp.maximum(i - 2, 0), NV - 1, 0))
        for c in range(NKC):
            kt = hs[pl.ds(kb + c * (KC // 2), KC // 2), :]
            rowsets = [kt[n * 64:(n + 1) * 64, :] for n in range(4)]
            if c >= MD:
                d = None
                for rb in range(NRB):
                    for v in range(RU // 8):
                        t_ = mhist[c - MD][rb][v * 8:(v + 1) * 8, :]
                        d = t_ if d is None else jnp.maximum(d, t_)
                r2 = rowsets[3]
                rowsets[3] = jnp.concatenate(
                    [jnp.concatenate([pin(r2[0:8, 0:128], pltpu.bitcast(d, U32)), r2[0:8, 128:]], axis=1), r2[8:]], axis=0)
            if LN0 <= c < LN0 + NRB:
                r1 = rowsets[0]
                rowsets[0] = jnp.concatenate([pin(r1[:RU // 2], tail(c - LN0)), r1[RU // 2:]], axis=0)
            kt = jnp.concatenate(rowsets, axis=0)
            sc = _dot_nt(q, kt)
            for rb in range(NRB):
                parts = [sc[rsl(rb), csl(j)] for j in range(4)]
                if c == NKC - 1:
                    lane = lax.broadcasted_iota(jnp.int32, (RU, 128), 1)
                    parts[3] = jnp.where(lane < T - (c * KC + 384), parts[3], -jnp.inf)
                mm = jnp.maximum(jnp.maximum(parts[0], parts[1]), jnp.maximum(parts[2], parts[3]))
                m[rb] = mm if m[rb] is None else jnp.maximum(m[rb], mm)
                for j in range(4):
                    sp[c, rb, j] = parts[j]
            mhist.append(list(m))
        all_units(tail)
        if prev == "ff1":
            mid = qv_matmul(NTILE - 1)
        else:
            mid = _dot(hb[...], wp1[...])
        mxb = [jnp.broadcast_to(jnp.max(m[rb], axis=-1, keepdims=True), (RU, 128)) for rb in range(NRB)]
        C0, RL = 2, 31
        slots = [(c * 4 + n) * NV + v for c in range(C0, NKC) for n in range(4) for v in range(NV)]
        where = {slots[k * len(slots) // max(len(late), 1)]: u_ for k, u_ in enumerate(late)}
        acc, l128, pvs = {}, [None] * NRB, []
        for c in range(NKC):
            pbl = []
            for rb in range(NRB):
                mb = mxb[rb]
                if c == 1:
                    mb = pin(mb, mid[rsl(rb), csl(4)])
                elif c >= 2:
                    mb = pin(mb, pvs[c - 1][rsl(rb), csl(1)])
                pj = [jnp.exp2(sp[c, rb, j] - mb) for j in range(4)]
                lsum = (pj[0] + pj[1]) + (pj[2] + pj[3])
                l128[rb] = lsum if l128[rb] is None else l128[rb] + lsum
                pbl.append(jnp.concatenate(pj, axis=1))
            pv = jnp.dot(jnp.concatenate(pbl, axis=0).astype(BF), unpack(vs[pl.ds(kb + c * (KC // 2), KC // 2), :]),
                         preferred_element_type=F32)
            pvs.append(pv)
            for n in range(4):
                side = None
                if c == 1:
                    if prev == "ff1":
                        qs[_prows(NTILE - 1), csl(n)] = pack(mid[:, csl(n)])
                        vs[_pkrows(NTILE - 1), csl(n)] = pack(mid[:, D + n * 128:D + (n + 1) * 128])
                    else:
                        side = glu_block(i - 1, mid, n)
                for v in range(NV):
                    blk = pv[v * 8:(v + 1) * 8, csl(n)]
                    if c == 0:
                        acc[n, v] = blk
                        continue
                    a = acc[n, v]
                    if side is not None:
                        a = pin(a, side[v * 8:(v + 1) * 8, :])
                    slot = (c * 4 + n) * NV + v
                    if slot in where:
                        s0 = slot - RL
                        dep = pvs[s0 // (4 * NV)][(s0 % NV) * 8:(s0 % NV) * 8 + 8, csl((s0 // NV) % 4)]
                        cb_, t_, j_, key_ = where[slot]
                        a = pin(a, conv(cb_, t_, j_, dep, key_, has_old if key_ == 0 else None))
                        if key_ == 0:
                            flush(cb_, has_old)
                    if n == 1:
                        rb, vv = divmod(v, RU // 8)
                        a = pin(a, l128[rb][vv * 8:(vv + 1) * 8, :])
                    acc[n, v] = a + blk
        for n in range(4):
            for v in range(NV):
                accs[v * 8:(v + 1) * 8, csl(n)] = acc[n, v]
        for rb in range(NRB):
            ls[rsl(rb), :] = l128[rb]

    def bn_silu_unit(i, pin):
        def unit(rb, rel):
            z = pack(_silu((held(dcs[_rows(i, rb), :], rel, pin) - bn[0:1, :]) * bn[1:2, :]))
            zs[rb * (RU // 2):(rb + 1) * (RU // 2), :] = z
            return zs[rb * (RU // 2):(rb + 1) * (RU // 2), :]
        return memo(unit)

    def c_step(i, do_prev, do_cur, do_next):
        pin = make_pin()
        if do_cur:
            y3 = _dot(zs[...], wp2[...])

            def x3u(rb, rel):
                x3 = held(xs[_rows(i, rb), :], rel, pin) + y3[rsl(rb), :]
                xs[_rows(i, rb), :] = x3
                return stash(rb, pack(_ln(x3)))
            x3u = memo(x3u)
        if do_prev:
            r1 = []
            yacc = acc_matmul(us, w2b, pin, spread(5, 10, x3u, r1, 3) if do_cur else {}, r1)

            def out_unit(rb, rel):
                o = pack(_ln(held(xs[_rows(i - 1, rb), :], rel, pin) + 0.5 * yacc[rb]))
                qs[_prows(i - 1, rb), :] = o
                return qs[_prows(i - 1, rb), :]
            out_unit = memo(out_unit)
        if do_cur:
            dl, r2 = {}, []
            if do_prev:
                dl.update(spread(6, 5, out_unit, r2, 4))
            if do_next:
                nd = len(dl)
                dl.update(spread(11, 5, bn_silu_unit(jnp.minimum(i + 1, NTILE - 1), pin), r2, None if do_prev else 3))
                assert len(dl) == nd + NRB
            all_units(x3u)
            ffa(hb[...], w2a, pin, dl, r2)
        elif do_prev:
            all_units(out_unit)

    WQ, WK, WV, WO, WP1, WP2, W2A, W2B, DW = range(2, 11)
    xcopy(0).start()
    w1a_copy(0).start()
    xcopy(1).start()
    for c in range(1, 4):
        w1a_copy(c).start()
    for c in range(4):
        w1b_copy(c).start()
    for k in (DW, WQ, WK, WV, WO):
        wcopy(k).start()
    for t in range(2, NTILE):
        xcopy(t).start()
    for k in (WP1, WP2, W2A, W2B):
        wcopy(k).start()
    for b in range(B):
        hs[(b * TP + T) // 2:(b + 1) * TP // 2, :] = jnp.zeros(((TP - T) // 2, D), U32)
        vs[(b * TP + T) // 2:(b + 1) * TP // 2, :] = jnp.zeros(((TP - T) // 2, D), U32)
        for cb in range(4):
            g0 = cb * GR + b * (T + 2 * HALO)
            gs[g0:g0 + HALO, :] = jnp.zeros((HALO, 128), F32)
            gs[g0 + HALO + T:g0 + T + 2 * HALO, :] = jnp.zeros((HALO, 128), F32)
    for cb in range(4):
        gs[cb * GR + HALO + TM:cb * GR + HALO + TM + 16, :] = jnp.zeros((16, 128), F32)
    st[...] = jnp.zeros(st.shape, F32)
    bn[...] = jnp.zeros(bn.shape, F32)
    xcopy(0).wait()
    bn[2:3, :] = unpack(qs[0:8, :]).astype(F32)[0:1, :]

    def first_a(c):
        w1a_copy(c).wait()
        if c == 1:
            xcopy(1).wait()
    a_step(0, False, pre_a=first_a, mode="first")

    def first_b(kg):
        if kg == 2:
            w1b_copy(2).wait()
            w1b_copy(3).wait()

    def fold_weights(c):
        if c != 0:
            return
        for k in (DW, WQ, WK, WV, WO):
            wcopy(k).wait()
        for kk in range(KW):
            for cb in range(4):
                dwt[(kk * 4 + cb) * 8:(kk * 4 + cb + 1) * 8, :] = jnp.broadcast_to(
                    dw_ref[kk:kk + 1, csl(cb)].astype(F32), (8, 128))
        mqv[:, :D] = pack(_dot_nt(wq[...], wk[...]) * (D ** -0.5 * LOG2E))
        mqv[:, D:] = pack(_dot(wv[...], wo[...]))
    w1b_copy(0).wait()
    w1b_copy(1).wait()
    a_step(1, True, pre_a=fold_weights, pre_b=first_b, mode="second")

    def a_body(j, c):
        xcopy(2 * j).wait()
        xcopy(2 * j + 1).wait()
        a_step(2 * j, True)
        a_step(2 * j + 1, True)
        return c
    lax.fori_loop(1, NTILE // 2 - 1, a_body, 0)
    a_body(NTILE // 2 - 1, 0)

    for k in (WP1, WP2, W2A, W2B):
        wcopy(k).wait()
    b_step(0, "ff1", 0)

    def b_body(i, c):
        b_step(i, "attn", 2)
        return c
    lax.fori_loop(1, NTILE, b_body, 0)

    pin = make_pin()
    all_units(attn_tail_unit(NTILE - 1, pin))
    conv, flush = conv_stream((NV - 1) + NV * (NTILE - 2), pin)
    for n in range(4):
        wab = jnp.concatenate([wp1[:, csl(n)], wp1[:, D + n * 128:D + (n + 1) * 128]], axis=1)
        yab = _dot(hb[...], wab)
        gs[pl.ds(_grow(NTILE - 1) + n * GR + HALO, TM), :] = yab[:, :128] * _sigmoid(yab[:, 128:])
        conv(n, NTILE - 2, NV - 1, None, 0)
        for j in range(NV):
            conv(n, NTILE - 1, j, None, 1)
        flush(n)
    mean8, m28 = st[0], st[1]
    mu = jnp.mean(mean8, axis=0, keepdims=True)
    dm = mean8 - mu
    var = (jnp.sum(m28, axis=0, keepdims=True) + (B * T // 8) * jnp.sum(dm * dm, axis=0, keepdims=True)) * (1.0 / (B * T))
    bn[0:1, :] = mu
    bn[1:2, :] = lax.rsqrt(var + EPS)
    all_units(bn_silu_unit(0, pin))
    c_step(0, False, True, True)
    c_step(1, True, True, True)
    ocopy(0).start()

    def c_body(j, c):
        c_step(2 * j, True, True, True)
        c_step(2 * j + 1, True, True, True)
        ocopy(2 * j - 1).start()
        ocopy(2 * j).start()
        return c
    lax.fori_loop(1, NTILE // 2, c_body, 0)
    c_step(NTILE, True, False, False)
    ocopy(NTILE - 1).start()
    for t in range(NTILE):
        ocopy(t).wait()


@jax.jit
def pallas_standalone__conformer_family_conformer__speech_kernel(
        x, w_ff1_a, w_ff1_b, w_q, w_k, w_v, w_o, w_pw1, dw, w_pw2, w_ff2_a, w_ff2_b):
    assert x.shape == (B, T, D) and w_ff1_a.shape == (D, F) and dw.shape == (KW, D)
    xf = x.reshape(B * T, D)
    ws = (w_ff1_a, w_ff1_b, w_q, w_k, w_v, w_o, w_pw1, dw, w_pw2, w_ff2_a, w_ff2_b)
    packed = lambda w: pltpu.VMEM((w.shape[0] // 2, w.shape[1]), U32)
    hbm = pl.BlockSpec(memory_space=pl.ANY)
    out = pl.pallas_call(
        kernel,
        in_specs=[hbm] * 12,
        out_specs=hbm,
        out_shape=jax.ShapeDtypeStruct((B * T, D), x.dtype),
        scratch_shapes=[packed(w) for w in (w_ff1_a, w_ff1_b, w_q, w_k, w_v, w_o, w_pw1, w_pw2, w_ff2_a, w_ff2_b)] + [
            pltpu.VMEM((KW, D), BF),
            pltpu.VMEM((B * T, D), F32),
            pltpu.VMEM((B * TP // 2, D), U32),
            pltpu.VMEM((B * T // 2, D), U32),
            pltpu.VMEM((B * TP // 2, D), U32),
            pltpu.VMEM((4 * GR, 128), F32),
            pltpu.VMEM((B * T, D), F32),
            pltpu.VMEM((TM // 2, F), U32),
            pltpu.VMEM((TM // 2, D), U32),
            pltpu.VMEM((TM, D), F32),
            pltpu.VMEM((TM, 128), F32),
            pltpu.VMEM((TM // 2, D), U32),
            pltpu.VMEM((D // 2, 2 * D), U32),
            pltpu.VMEM((KW * 4 * 8, 128), F32),
            pltpu.VMEM((2, 8, D), F32),
            pltpu.VMEM((8, D), F32),
            pltpu.SemaphoreType.DMA((11,)),
            pltpu.SemaphoreType.DMA((8,)),
            pltpu.SemaphoreType.DMA((NTILE,)),
            pltpu.SemaphoreType.DMA((1,)),
        ],
        compiler_params=pltpu.CompilerParams(vmem_limit_bytes=124 * 1024 * 1024),
    )(xf, *ws)
    return out.reshape(B, T, D)
```

```python
import jax
import jax.numpy as jnp
from jax import lax
from jax.experimental import pallas as pl
from jax.experimental.pallas import tpu as pltpu

B, T, D, F, KW = 2, 4000, 512, 2048, 15
TP = 4096
TM = 400
NT = T // TM
NTILE = B * NT
KC = 512
NKC = TP // KC
RU = 80
NRB = TM // RU
NV = TM // 8
EPS = 1e-5
LOG2E = 1.4426950408889634
BF = jnp.bfloat16
F32 = jnp.float32
U32 = jnp.uint32
HALO = 8
GR = B * (T + 2 * HALO)


def _ln(x):
    m = jnp.mean(x, axis=-1, keepdims=True)
    xc = x - m
    v = jnp.mean(xc * xc, axis=-1, keepdims=True)
    return xc * lax.rsqrt(v + EPS)


def pack(x):
    return pltpu.bitcast(x.astype(BF), U32)


def unpack(w):
    return pltpu.bitcast(w, BF)


def _dot(a32, b32):
    return jnp.dot(unpack(a32), unpack(b32), preferred_element_type=F32)


def _dot_nt(a32, b32):
    return lax.dot_general(unpack(a32), unpack(b32), (((1,), (1,)), ((), ())), preferred_element_type=F32)


def _sigmoid(x):
    return 0.5 * jnp.tanh(0.5 * x) + 0.5


def _silu(x):
    hx = 0.5 * x
    return hx * jnp.tanh(hx) + hx


def _mult(v, n):
    return v if isinstance(v, int) else pl.multiple_of(v, n)


def _rows(i, rb=None):
    if rb is None:
        return pl.ds(_mult(i * TM, 8), TM)
    return pl.ds(_mult(i * TM + rb * RU, 8), RU)


def _prows(i, rb=None):
    if rb is None:
        return pl.ds(_mult(i * (TM // 2), 8), TM // 2)
    return pl.ds(_mult(i * (TM // 2) + rb * (RU // 2), 8), RU // 2)


def _pk0(i):
    return (i // NT) * (TP // 2) + (i % NT) * (TM // 2)


def _pkrows(i):
    return pl.ds(_mult(_pk0(i), 8), TM // 2)


def _grow(i):
    return (i // NT) * (T + 2 * HALO) + (i % NT) * TM


def rsl(rb):
    return slice(rb * RU, (rb + 1) * RU)


def csl(n):
    return slice(n * 128, (n + 1) * 128)


def kernel(x_hbm, w1a_h, w1b_h, wq_h, wk_h, wv_h, wo_h, wp1_h, dw_h, wp2_h, w2a_h, w2b_h, o_hbm,
           w1a, w1b, wq, wk, wv, wo, wp1, wp2, w2a, w2b, dw_ref,
           xs, hs, qs, vs, gs, dcs, us, hb, accs, ls, zs, mqv, dwt, st, bn,
           wsem, csem, xsem, osem):
    def wcopy(k):
        srcs = (w1a_h, w1b_h, wq_h, wk_h, wv_h, wo_h, wp1_h, wp2_h, w2a_h, w2b_h, dw_h)
        dsts = (w1a, w1b, wq, wk, wv, wo, wp1, wp2, w2a, w2b)
        dst = dw_ref if k == 10 else dsts[k].bitcast(BF)
        return pltpu.make_async_copy(srcs[k], dst, wsem.at[k])

    def w1a_copy(c):
        return pltpu.make_async_copy(w1a_h.at[:, c * 512:(c + 1) * 512], w1a.bitcast(BF).at[:, c * 512:(c + 1) * 512], csem.at[c])

    def w1b_copy(c):
        return pltpu.make_async_copy(w1b_h.at[c * 512:(c + 1) * 512, :], w1b.bitcast(BF).at[c * 512:(c + 1) * 512, :], csem.at[4 + c])

    def xcopy(i):
        rows = pl.ds(_mult(i * TM, 16), TM)
        return pltpu.make_async_copy(x_hbm.at[rows, :], qs.bitcast(BF).at[rows, :], xsem.at[i])

    def ocopy(i):
        rows = pl.ds(_mult(i * TM, 16), TM)
        return pltpu.make_async_copy(qs.bitcast(BF).at[rows, :], o_hbm.at[rows, :], osem.at[0])

    def make_pin():
        nv = jnp.abs(bn[2:3, :])

        def pin(val, dep):
            never = jnp.broadcast_to(nv[:, :val.shape[1]], val.shape) < 0.0
            return jnp.where(never, dep, val)
        return pin

    def memo(fn):
        cache = {}

        def get(rb, rel=None):
            if rb not in cache:
                cache[rb] = fn(rb, rel)
            return cache[rb]
        return get

    def stash(rb, h32):
        hb[rb * (RU // 2):(rb + 1) * (RU // 2), :] = h32
        return hb[rb * (RU // 2):(rb + 1) * (RU // 2), :]

    def all_units(get):
        for rb in range(NRB):
            get(rb)

    def pin_rhs(w32, pin, tokens):
        if not tokens:
            return w32
        cols = []
        for n in range(4):
            col = w32[:, csl(n)]
            if n in tokens:
                tk = tokens[n]()
                k = tk.shape[0]
                col = jnp.concatenate([pin(col[:k], tk), col[k:]], axis=0)
            cols.append(col)
        return jnp.concatenate(cols, axis=1)

    def spread(first, count, unit, res, lead):
        out = {}
        for rb in range(NRB):
            p = first + rb * count // NRB
            pr = -1 if lead is None else min(p - lead, 4 * (p // 4) - 1)

            def token(rb=rb, pr=pr):
                rel = None
                if lead is not None and pr >= 0:
                    rel = jnp.concatenate([res[pr // 4][rsl(rb), csl(pr % 4)]] * 4, axis=1)
                u_ = unit(rb, rel)
                return jnp.concatenate([u_[:, csl(n)] for n in range(4)], axis=0)
            assert p < 16 and (p // 4, p % 4) not in out
            out[p // 4, p % 4] = token
        return out

    def tok(deadlines, c):
        return {n: f for (cc, n), f in deadlines.items() if cc == c}

    def acc_matmul(lhs, w, pin, deadlines, res, pre=None):
        acc = None
        for kg in range(4):
            if pre:
                pre(kg)
            part = _dot(lhs[:, kg * 512:(kg + 1) * 512], pin_rhs(w[kg * 256:(kg + 1) * 256, :], pin, tok(deadlines, kg)))
            res.append(part)
            if acc is None:
                acc = [part[rsl(rb), :] for rb in range(NRB)]
            else:
                acc = [acc[rb] + part[rsl(rb), :] for rb in range(NRB)]
        return acc

    def ffa(h32, wa, pin, deadlines, res, pre=None):
        for c in range(F // 512):
            if pre:
                pre(c)
            u = _dot(h32, pin_rhs(wa[:, c * 512:(c + 1) * 512], pin, tok(deadlines, c)))
            res.append(u)
            us[:, c * 512:(c + 1) * 512] = pack(_silu(u))

    def held(val, rel, pin):
        if rel is None:
            return val
        if val.dtype == U32:
            return pin(val, pltpu.bitcast(rel[:val.shape[0]], U32))
        return pin(val, rel)

    def ff1_tail_unit(i, yacc, pin):
        def unit(rb, rel):
            x1 = unpack(held(qs[_prows(i, rb), :], rel, pin)).astype(F32) + 0.5 * yacc[rb]
            xs[_rows(i, rb), :] = x1
            h1 = pack(_ln(x1))
            rows = pl.ds(_mult(_pk0(i) + rb * (RU // 2), 8), RU // 2)
            hs[rows, :] = h1
            return hs[rows, :]
        return memo(unit)

    def qv_matmul(i):
        return _dot(hs[_pkrows(i), :], mqv[...])

    def a_step(i, do_prev, pre_a=None, pre_b=None, mode="steady"):
        pin = make_pin()
        lnx = memo(lambda rb, rel: stash(rb, pack(_ln(unpack(held(qs[_prows(i, rb), :], rel, pin)).astype(F32)))))
        dl, r1, r2 = {}, [], []
        lhs = hb
        if mode == "first":
            def nxt(rb, rel):
                rows = slice(rb * (RU // 2), (rb + 1) * (RU // 2))
                zs[rows, :] = pack(_ln(unpack(held(qs[_prows(i + 1, rb), :], rel, pin)).astype(F32)))
                return zs[rows, :]
            dl = spread(9, 5, memo(nxt), r2, 4)
        if do_prev:
            yacc = acc_matmul(us, w1b, pin, {} if mode == "second" else spread(4, 10, lnx, r1, 3), r1, pre_b)
            tail = ff1_tail_unit(i - 1, yacc, pin)
            dl = spread(2, 10, tail, r2, 4)
        if mode == "second":
            lhs = zs
        else:
            all_units(lnx)
        ffa(lhs[...], w1a, pin, dl, r2, pre_a)
        if do_prev:
            all_units(tail)
            qv = qv_matmul(i - 1)
            qs[_prows(i - 1), :] = pack(qv[:, :D])
            vs[_pkrows(i - 1), :] = pack(qv[:, D:])

    def conv_stream(n_old, pin):
        cs = [dict(cnt=0) for _ in range(4)]
        sub = lax.broadcasted_iota(jnp.int32, (8, 128), 0)

        def rot(v):
            return [v] + [pltpu.roll(v, 8 - s_, 0) for s_ in range(1, 8)]

        def shift(ra, rb_):
            return [ra[0]] + [jnp.where(sub < 8 - s_, ra[s_], rb_[s_]) for s_ in range(1, 8)]

        def step(cb, t, j, dep, key, valid=None, direct=False):
            c_ = cs[cb]
            g0 = _grow(t)
            rel = (lambda v: v) if dep is None else (lambda v: pin(v, dep))
            ld = lambda jj: rel(gs[pl.ds(_mult(g0 + cb * GR + 8 * jj, 8), 8), :])
            if c_.get("next") != (key, j):
                ra, rb_ = rot(ld(j)), rot(ld(j + 1))
                c_["G"], c_["R"] = shift(ra, rb_), rb_
            if "w" not in c_:
                c_["w"] = [dwt[(kk * 4 + cb) * 8:(kk * 4 + cb + 1) * 8, :] for kk in range(KW)]
            if direct:
                rn = None
                gn = [gs[pl.ds(g0 + (cb * GR + 8 * (j + 1) + s_), 8), :] for s_ in range(8)]
            else:
                rn = rot(ld(j + 2))
                gn = shift(c_["R"], rn)
            terms = [c_["G"][s_] * c_["w"][s_ - 1] for s_ in range(1, 8)] + [gn[s_] * c_["w"][7 + s_] for s_ in range(8)]
            c_["G"], c_["R"], c_["next"] = gn, rn, (key, j + 1)
            while len(terms) > 1:
                terms = [terms[q] + terms[q + 1] for q in range(0, len(terms) - 1, 2)] + ([terms[-1]] if len(terms) % 2 else [])
            o = terms[0]
            dcs[pl.ds(_mult(t * TM + 8 * j, 8), 8), csl(cb)] = o
            if c_["cnt"] == 0:
                c_["c"] = o
            else:
                d = o - c_["c"]
                if valid is not None:
                    d = jnp.where(valid, d, 0.0)
                c_["s1"] = d if c_["cnt"] == 1 else c_["s1"] + d
                c_["s2"] = d * d if c_["cnt"] == 1 else c_["s2"] + d * d
            c_["cnt"] += 1
            return o

        def flush(cb, valid=None):
            c_ = cs[cb]
            k = jnp.full((8, 128), c_["cnt"], F32)
            if valid is not None:
                k = jnp.where(valid, k, k - 1.0)
            cols = csl(cb)
            rk = 1.0 / k
            tmean = c_["c"] + c_["s1"] * rk
            tm2 = c_["s2"] - c_["s1"] * c_["s1"] * rk
            n = jnp.zeros((8, 128), F32) + jnp.asarray(n_old, F32)
            f = k / (n + k)
            mean_old = st[0, :, cols]
            delta = tmean - mean_old
            st[0, :, cols] = mean_old + delta * f
            st[1, :, cols] = st[1, :, cols] + tm2 + delta * delta * (n * f)
            c_["cnt"] = 0
        return step, flush

    def attn_tail_unit(i, pin):
        def unit(rb, rel):
            lsum = ls[rsl(rb), :]
            if rel is not None:
                lsum = pin(lsum, rel[:, 0:128])
            inv = 1.0 / jnp.sum(lsum, axis=-1, keepdims=True)
            x2 = held(xs[_rows(i, rb), :], rel, pin) + accs[rsl(rb), :] * inv
            xs[_rows(i, rb), :] = x2
            return stash(rb, pack(_ln(x2)))
        return memo(unit)

    def glu_block(i, y2, n):
        g = y2[:, csl(n)] * _sigmoid(y2[:, D + n * 128:D + (n + 1) * 128])
        gs[pl.ds(_mult(_grow(i) + (n * GR + HALO), 8), TM), :] = g
        return g

    def b_step(i, prev, conv_mode):
        pin = make_pin()
        kb = _mult((i // NT) * (TP // 2), TP // 2)
        if prev == "ff1":
            tail = ff1_tail_unit(NTILE - 1, acc_matmul(us, w1b, pin, {}, []), pin)
        else:
            tail = attn_tail_unit(i - 1, pin)
        q = qs[_prows(i), :]
        m = [None] * NRB
        mhist = []
        sp = {}
        MD, LN0 = 2, 2
        late = []
        if conv_mode:
            has_old = i >= 2
            conv, flush = conv_stream(jnp.where(has_old, (NV - 1) + NV * (i - 2), 0), pin)
            for cb in range(4):
                late += [(cb, i - 1, j, 1) for j in range(NV - 1)]
                late.append((cb, jnp.maximum(i - 2, 0), NV - 1, 0))
        for c in range(NKC):
            kt = hs[pl.ds(kb + c * (KC // 2), KC // 2), :]
            rowsets = [kt[n * 64:(n + 1) * 64, :] for n in range(4)]
            if c >= MD:
                d = None
                for rb in range(NRB):
                    for v in range(RU // 8):
                        t_ = mhist[c - MD][rb][v * 8:(v + 1) * 8, :]
                        d = t_ if d is None else jnp.maximum(d, t_)
                r2 = rowsets[3]
                rowsets[3] = jnp.concatenate(
                    [jnp.concatenate([pin(r2[0:8, 0:128], pltpu.bitcast(d, U32)), r2[0:8, 128:]], axis=1), r2[8:]], axis=0)
            if LN0 <= c < LN0 + NRB:
                r1 = rowsets[0]
                rowsets[0] = jnp.concatenate([pin(r1[:RU // 2], tail(c - LN0)), r1[RU // 2:]], axis=0)
            kt = jnp.concatenate(rowsets, axis=0)
            sc = _dot_nt(q, kt)
            for rb in range(NRB):
                parts = [sc[rsl(rb), csl(j)] for j in range(4)]
                if c == NKC - 1:
                    lane = lax.broadcasted_iota(jnp.int32, (RU, 128), 1)
                    parts[3] = jnp.where(lane < T - (c * KC + 384), parts[3], -jnp.inf)
                mm = jnp.maximum(jnp.maximum(parts[0], parts[1]), jnp.maximum(parts[2], parts[3]))
                m[rb] = mm if m[rb] is None else jnp.maximum(m[rb], mm)
                for j in range(4):
                    sp[c, rb, j] = parts[j]
            mhist.append(list(m))
        all_units(tail)
        if prev == "ff1":
            mid = qv_matmul(NTILE - 1)
        else:
            mid = _dot(hb[...], wp1[...])
        mxb = [jnp.broadcast_to(jnp.max(m[rb], axis=-1, keepdims=True), (RU, 128)) for rb in range(NRB)]
        C0, RL = 2, 31
        slots = [(c * 4 + n) * NV + v for c in range(C0, NKC) for n in range(4) for v in range(NV)]
        where = {slots[k * len(slots) // max(len(late), 1)]: u_ for k, u_ in enumerate(late)}
        acc, l128, pvs = {}, [None] * NRB, []
        for c in range(NKC):
            pbl = []
            for rb in range(NRB):
                mb = mxb[rb]
                if c == 1:
                    mb = pin(mb, mid[rsl(rb), csl(4)])
                elif c >= 2:
                    mb = pin(mb, pvs[c - 1][rsl(rb), csl(1)])
                pj = [jnp.exp2(sp[c, rb, j] - mb) for j in range(4)]
                lsum = (pj[0] + pj[1]) + (pj[2] + pj[3])
                l128[rb] = lsum if l128[rb] is None else l128[rb] + lsum
                pbl.append(jnp.concatenate(pj, axis=1))
            pv = jnp.dot(jnp.concatenate(pbl, axis=0).astype(BF), unpack(vs[pl.ds(kb + c * (KC // 2), KC // 2), :]),
                         preferred_element_type=F32)
            pvs.append(pv)
            for n in range(4):
                side = None
                if c == 1:
                    if prev == "ff1":
                        qs[_prows(NTILE - 1), csl(n)] = pack(mid[:, csl(n)])
                        vs[_pkrows(NTILE - 1), csl(n)] = pack(mid[:, D + n * 128:D + (n + 1) * 128])
                    else:
                        side = glu_block(i - 1, mid, n)
                for v in range(NV):
                    blk = pv[v * 8:(v + 1) * 8, csl(n)]
                    if c == 0:
                        acc[n, v] = blk
                        continue
                    a = acc[n, v]
                    if side is not None:
                        a = pin(a, side[v * 8:(v + 1) * 8, :])
                    slot = (c * 4 + n) * NV + v
                    if slot in where:
                        s0 = slot - RL
                        dep = pvs[s0 // (4 * NV)][(s0 % NV) * 8:(s0 % NV) * 8 + 8, csl((s0 // NV) % 4)]
                        cb_, t_, j_, key_ = where[slot]
                        a = pin(a, conv(cb_, t_, j_, dep, key_, has_old if key_ == 0 else None))
                        if key_ == 0:
                            flush(cb_, has_old)
                    if n == 1:
                        rb, vv = divmod(v, RU // 8)
                        a = pin(a, l128[rb][vv * 8:(vv + 1) * 8, :])
                    acc[n, v] = a + blk
        for n in range(4):
            for v in range(NV):
                accs[v * 8:(v + 1) * 8, csl(n)] = acc[n, v]
        for rb in range(NRB):
            ls[rsl(rb), :] = l128[rb]

    def bn_silu_unit(i, pin):
        def unit(rb, rel):
            z = pack(_silu((held(dcs[_rows(i, rb), :], rel, pin) - bn[0:1, :]) * bn[1:2, :]))
            zs[rb * (RU // 2):(rb + 1) * (RU // 2), :] = z
            return zs[rb * (RU // 2):(rb + 1) * (RU // 2), :]
        return memo(unit)

    def c_step(i, do_prev, do_cur, do_next):
        pin = make_pin()
        if do_cur:
            y3 = _dot(zs[...], wp2[...])

            def x3u(rb, rel):
                x3 = held(xs[_rows(i, rb), :], rel, pin) + y3[rsl(rb), :]
                xs[_rows(i, rb), :] = x3
                return stash(rb, pack(_ln(x3)))
            x3u = memo(x3u)
        if do_prev:
            r1 = []
            yacc = acc_matmul(us, w2b, pin, spread(5, 10, x3u, r1, 3) if do_cur else {}, r1)

            def out_unit(rb, rel):
                o = pack(_ln(held(xs[_rows(i - 1, rb), :], rel, pin) + 0.5 * yacc[rb]))
                qs[_prows(i - 1, rb), :] = o
                return qs[_prows(i - 1, rb), :]
            out_unit = memo(out_unit)
        if do_cur:
            dl, r2 = {}, []
            if do_prev:
                dl.update(spread(6, 5, out_unit, r2, 4))
            if do_next:
                nd = len(dl)
                dl.update(spread(11, 5, bn_silu_unit(jnp.minimum(i + 1, NTILE - 1), pin), r2, None if do_prev else 3))
                assert len(dl) == nd + NRB
            all_units(x3u)
            ffa(hb[...], w2a, pin, dl, r2)
        elif do_prev:
            all_units(out_unit)

    WQ, WK, WV, WO, WP1, WP2, W2A, W2B, DW = range(2, 11)
    xcopy(0).start()
    w1a_copy(0).start()
    xcopy(1).start()
    for c in range(1, 4):
        w1a_copy(c).start()
    for c in range(4):
        w1b_copy(c).start()
    for k in (DW, WQ, WK, WV, WO):
        wcopy(k).start()
    for t in range(2, NTILE):
        xcopy(t).start()
    for k in (WP1, WP2, W2A, W2B):
        wcopy(k).start()
    for b in range(B):
        hs[(b * TP + T) // 2:(b + 1) * TP // 2, :] = jnp.zeros(((TP - T) // 2, D), U32)
        vs[(b * TP + T) // 2:(b + 1) * TP // 2, :] = jnp.zeros(((TP - T) // 2, D), U32)
        for cb in range(4):
            g0 = cb * GR + b * (T + 2 * HALO)
            gs[g0:g0 + HALO, :] = jnp.zeros((HALO, 128), F32)
            gs[g0 + HALO + T:g0 + T + 2 * HALO, :] = jnp.zeros((HALO, 128), F32)
    for cb in range(4):
        gs[cb * GR + HALO + TM:cb * GR + HALO + TM + 16, :] = jnp.zeros((16, 128), F32)
    st[...] = jnp.zeros(st.shape, F32)
    bn[...] = jnp.zeros(bn.shape, F32)
    xcopy(0).wait()
    bn[2:3, :] = unpack(qs[0:8, :]).astype(F32)[0:1, :]

    def first_a(c):
        w1a_copy(c).wait()
        if c == 1:
            xcopy(1).wait()
    a_step(0, False, pre_a=first_a, mode="first")

    def first_b(kg):
        if kg == 2:
            w1b_copy(2).wait()
            w1b_copy(3).wait()

    def fold_weights(c):
        if c != 0:
            return
        for k in (DW, WQ, WK, WV, WO):
            wcopy(k).wait()
        for kk in range(KW):
            for cb in range(4):
                dwt[(kk * 4 + cb) * 8:(kk * 4 + cb + 1) * 8, :] = jnp.broadcast_to(
                    dw_ref[kk:kk + 1, csl(cb)].astype(F32), (8, 128))
        mqv[:, :D] = pack(_dot_nt(wq[...], wk[...]) * (D ** -0.5 * LOG2E))
        mqv[:, D:] = pack(_dot(wv[...], wo[...]))
    w1b_copy(0).wait()
    w1b_copy(1).wait()
    a_step(1, True, pre_a=fold_weights, pre_b=first_b, mode="second")

    def a_body(j, c):
        xcopy(2 * j).wait()
        xcopy(2 * j + 1).wait()
        a_step(2 * j, True)
        a_step(2 * j + 1, True)
        return c
    lax.fori_loop(1, NTILE // 2 - 1, a_body, 0)
    a_body(NTILE // 2 - 1, 0)

    for k in (WP1, WP2, W2A, W2B):
        wcopy(k).wait()
    b_step(0, "ff1", 0)

    def b_body(i, c):
        b_step(i, "attn", 2)
        return c
    lax.fori_loop(1, NTILE, b_body, 0)

    pin = make_pin()
    all_units(attn_tail_unit(NTILE - 1, pin))
    conv, flush = conv_stream((NV - 1) + NV * (NTILE - 2), pin)
    for n in range(4):
        wab = jnp.concatenate([wp1[:, csl(n)], wp1[:, D + n * 128:D + (n + 1) * 128]], axis=1)
        yab = _dot(hb[...], wab)
        gs[pl.ds(_grow(NTILE - 1) + n * GR + HALO, TM), :] = yab[:, :128] * _sigmoid(yab[:, 128:])
        conv(n, NTILE - 2, NV - 1, None, 0)
        for j in range(NV):
            conv(n, NTILE - 1, j, None, 1, None, True)
        flush(n)
    mean8, m28 = st[0], st[1]
    mu = jnp.mean(mean8, axis=0, keepdims=True)
    dm = mean8 - mu
    var = (jnp.sum(m28, axis=0, keepdims=True) + (B * T // 8) * jnp.sum(dm * dm, axis=0, keepdims=True)) * (1.0 / (B * T))
    bn[0:1, :] = mu
    bn[1:2, :] = lax.rsqrt(var + EPS)
    all_units(bn_silu_unit(0, pin))
    c_step(0, False, True, True)
    c_step(1, True, True, True)
    ocopy(0).start()

    def c_body(j, c):
        c_step(2 * j, True, True, True)
        c_step(2 * j + 1, True, True, True)
        ocopy(2 * j - 1).start()
        ocopy(2 * j).start()
        return c
    lax.fori_loop(1, NTILE // 2, c_body, 0)
    c_step(NTILE, True, False, False)
    ocopy(NTILE - 1).start()
    for t in range(NTILE):
        ocopy(t).wait()


@jax.jit
def pallas_standalone__conformer_family_conformer__speech_kernel(
        x, w_ff1_a, w_ff1_b, w_q, w_k, w_v, w_o, w_pw1, dw, w_pw2, w_ff2_a, w_ff2_b):
    assert x.shape == (B, T, D) and w_ff1_a.shape == (D, F) and dw.shape == (KW, D)
    xf = x.reshape(B * T, D)
    ws = (w_ff1_a, w_ff1_b, w_q, w_k, w_v, w_o, w_pw1, dw, w_pw2, w_ff2_a, w_ff2_b)
    packed = lambda w: pltpu.VMEM((w.shape[0] // 2, w.shape[1]), U32)
    hbm = pl.BlockSpec(memory_space=pl.ANY)
    out = pl.pallas_call(
        kernel,
        in_specs=[hbm] * 12,
        out_specs=hbm,
        out_shape=jax.ShapeDtypeStruct((B * T, D), x.dtype),
        scratch_shapes=[packed(w) for w in (w_ff1_a, w_ff1_b, w_q, w_k, w_v, w_o, w_pw1, w_pw2, w_ff2_a, w_ff2_b)] + [
            pltpu.VMEM((KW, D), BF),
            pltpu.VMEM((B * T, D), F32),
            pltpu.VMEM((B * TP // 2, D), U32),
            pltpu.VMEM((B * T // 2, D), U32),
            pltpu.VMEM((B * TP // 2, D), U32),
            pltpu.VMEM((4 * GR, 128), F32),
            pltpu.VMEM((B * T, D), F32),
            pltpu.VMEM((TM // 2, F), U32),
            pltpu.VMEM((TM // 2, D), U32),
            pltpu.VMEM((TM, D), F32),
            pltpu.VMEM((TM, 128), F32),
            pltpu.VMEM((TM // 2, D), U32),
            pltpu.VMEM((D // 2, 2 * D), U32),
            pltpu.VMEM((KW * 4 * 8, 128), F32),
            pltpu.VMEM((2, 8, D), F32),
            pltpu.VMEM((8, D), F32),
            pltpu.SemaphoreType.DMA((11,)),
            pltpu.SemaphoreType.DMA((8,)),
            pltpu.SemaphoreType.DMA((NTILE,)),
            pltpu.SemaphoreType.DMA((1,)),
        ],
        compiler_params=pltpu.CompilerParams(vmem_limit_bytes=124 * 1024 * 1024),
    )(xf, *ws)
    return out.reshape(B, T, D)
```
